```python
import jax
import jax.numpy as jnp

def _softmax(x, axis=-1):
    return jax.nn.softmax(x, axis=axis)
def _gelu(x):
    return jax.nn.gelu(x, approximate=True)
def _silu(x):
    return jax.nn.silu(x)
def _sigmoid(x):
    return jax.nn.sigmoid(x)
def _layernorm(x, axis=-1, eps=1e-5):
    m = jnp.mean(x, axis=axis, keepdims=True)
    v = jnp.var(x, axis=axis, keepdims=True)
    return (x - m) / jnp.sqrt(v + eps)
def _scatter_add(tgt, idx, src, axis=0):
    return tgt.at[idx].add(src)
def _segment_sum(src, seg, n):
    return jax.ops.segment_sum(src, seg, n)
class _Rng:
    def __init__(self, key):
        self._k = key
    def _next(self):
        self._k, sub = jax.random.split(self._k)
        return sub
    def normal(self, shape):
        return jax.random.normal(self._next(), shape, dtype=jnp.bfloat16)
    def randint(self, lo, hi, shape):
        return jax.random.randint(self._next(), shape, lo, hi, dtype=jnp.int32)
    def uniform(self, shape, lo=0.0, hi=1.0):
        return jax.random.uniform(self._next(), shape, jnp.bfloat16, lo, hi)
    def permutation(self, n):
        return jax.random.permutation(self._next(), n)


kernel_name = 'parallel_sum__ssm_conv_h3__dense_activation_gelu__prompt'

def setup_inputs():
    _rng = _Rng(jax.random.key(int.from_bytes(__import__("os").urandom(4), "little")))
    _w = (lambda a: (lambda t: t.astype(jnp.bfloat16) if jnp.issubdtype(t.dtype, jnp.floating) else t)(jnp.asarray(a)))
    def _A_setup():
        B, S, D = 1, 2048, 640
        ks = 4
        return {
            "q": _w((lambda *s: _rng.normal(s) * 0.05)(B, S, D)),
            "k": _w((lambda *s: _rng.normal(s) * 0.05)(B, S, D)),
            "v": _w((lambda *s: _rng.normal(s) * 0.05)(B, S, D)),
            "shift_k": _w((lambda *s: _rng.normal(s) * 0.05)(D, ks) * 0.5),
            "ssm_k": _w((lambda *s: _rng.normal(s) * 0.05)(D, S) * (1.0 / S ** 0.5)),
            "ssm_D": _w((lambda *s: _rng.normal(s) * 0.05)(D)),
        }
    _A_in = _A_setup()

    def _B_setup():
        B, S, D, F = 1, 2048, 640, 1728
        return {
            "x": _w((lambda *s: _rng.normal(s) * 0.05)(B, S, D)),
            "w1": _w((lambda *s: _rng.normal(s) * 0.05)(D, F) * (D ** -0.5)),
            "b1": _w((lambda *s: _rng.normal(s) * 0.05)(F) * 0.01),
            "w2": _w((lambda *s: _rng.normal(s) * 0.05)(F, D) * (F ** -0.5)),
            "b2": _w((lambda *s: _rng.normal(s) * 0.05)(D) * 0.01),
        }
    _B_in = _B_setup()

    return {
        "A_q": _A_in["q"],
        "A_k": _A_in["k"],
        "A_v": _A_in["v"],
        "A_shift_k": _A_in["shift_k"],
        "A_ssm_k": _A_in["ssm_k"],
        "A_ssm_D": _A_in["ssm_D"],
        "B_x": _B_in["x"],
        "B_w1": _B_in["w1"],
        "B_b1": _B_in["b1"],
        "B_w2": _B_in["w2"],
        "B_b2": _B_in["b2"],
    }

def reference(A_q, A_k, A_v, A_shift_k, A_ssm_k, A_ssm_D, B_x, B_w1, B_b1, B_w2, B_b2):
    def _A_ref(q, k, v, shift_k, ssm_k, ssm_D):
        B, S, D = q.shape
        ks = shift_k.shape[-1]
        k_pad = jnp.pad(k, ((0, 0), (ks - 1, 0), (0, 0)))
        k_shift = jnp.zeros_like(k)
        for t in range(ks):
            k_shift = k_shift + k_pad[:, t:t + S, :] * shift_k[:, ks - 1 - t][None, None, :]
        kv = k_shift * v
        L = 2 * S
        kv_pad = jnp.pad(kv, ((0, 0), (0, S), (0, 0)))
        kf_pad = jnp.pad(ssm_k, ((0, 0), (0, S)))
        kv_f = (lambda x, axes=(-2,-1): jnp.fft.rfft2(x.astype(jnp.float32), axes=axes))(kv_pad[:, None, :, :], axes=(1, 2))
        kf_f = (lambda x, axes=(-2,-1): jnp.fft.rfft2(x.astype(jnp.float32), axes=axes))(kf_pad[:, None, :], axes=(1, 2))
        kf_f = (lambda x, *d: x.transpose(*d))(kf_f, 1, 2, 0)
        y_f = kv_f * kf_f[None, :, :, :]
        y = (lambda x, s, axes=(-2,-1): jnp.fft.irfft2(x, s=s, axes=axes).astype(jnp.bfloat16))(y_f, (1, L), axes=(1, 2))[:, 0, :S, :]
        y = y + kv * ssm_D[None, None, :]
        return q * y

    def _B_ref(x, w1, b1, w2, b2):
        h = jnp.einsum("bsd,df->bsf", x, w1) + b1
        h = _gelu(h)
        return jnp.einsum("bsf,fd->bsd", h, w2) + b2

    x = A_q
    xn = _layernorm(x, axis=-1)
    return x + _A_ref(xn, A_k, A_v, A_shift_k, A_ssm_k, A_ssm_D) + _B_ref(xn, B_w1, B_b1, B_w2, B_b2)
```

```python
import numpy as np
import jax
import jax.numpy as jnp
from jax.experimental import pallas as pl
from jax.experimental.pallas import tpu as pltpu

S, D, F = 2048, 640, 1728
C = 128
NC = S // C
TM = 256
NB = S // TM
NL = D // 128
NG = C // 8
f32, bf16, u32 = jnp.float32, jnp.bfloat16, jnp.uint32
pk = lambda v: pltpu.bitcast(v, u32)
upk = lambda v: pltpu.bitcast(v, bf16)
RATE = int('104')
W1 = float('0.3')
W2 = (14 - 14 * W1) / 70
DENS = float('2.3')
F1 = int('7')
FB = int('100')
INVD = int('4')
PTS = [float(v) for v in '1.12,1.4,1.8,2.3,3,5,7.55'.split(',')]
LAG = int('3')
KG = [int(v) for v in '0,4,8,11,14'.split(',')]
FWD_AT = {0: [], 1: [0, 1, 2, 3], 2: [4, 5, 6, 7], 3: [8, 9, 10], 4: [11, 12, 13], 5: [14, 15], 6: [], 7: []}
QB = 2 * NC
PB = QB + 6


def _dft_mats():
    n = np.arange(C)[None, :]
    th = 2 * np.pi * (np.arange(C)[:, None] + 0.25) / C
    co, si = np.cos(th * n), np.sin(th * n)
    il = lambda a, b: np.stack([a.reshape(NG, 8, C), b.reshape(NG, 8, C)], 1).reshape(2 * C, C)
    return il(co, si), il(si - co, si + co), il(co, si).T / C


def _pack(m):
    b = m.astype(np.float32).astype(jnp.bfloat16).view(np.uint16).astype(np.uint32)
    return b[0::2] | (b[1::2] << 16)


def kern(z_ref, x_h, k_h, v_h, sk_ref, ssm_h, dd_ref, w1_h, b1_ref, w2_h, b2_ref, fu_ref, fk_ref, inv_ref, o_h,
         x_v, k_v, v_v, ssm_v, w1_v, w2_v, o_v, kf, xn_v, xb_v, kvd_v, kvb_v, ff_v, g_v, acc_v, zs,
         sem, wsem, ssem, osem):
    z0 = z_ref[0]
    keep = jax.lax.broadcasted_iota(jnp.int32, (8, 128), 0) >= z0

    def after(v, mark):
        if v.dtype != f32:
            mark = pltpu.bitcast(mark, v.dtype)
        return jnp.where(keep, v, mark)

    def lanes(c):
        return pl.ds(c * 128, 128)

    x_u, k_u, v_u, o_u = (r.bitcast(u32) for r in (x_h, k_h, v_h, o_h))
    ssm_u, w1_u, w2_u = (r.bitcast(u32) for r in (ssm_h, w1_h, w2_h))
    cp = {}
    for s in range(NB):
        rr = pl.ds(s * TM // 2, TM // 2)
        cp["x", s] = pltpu.make_async_copy(x_u.at[rr], x_v.at[rr], sem.at[0, s])
        cp["k", s] = pltpu.make_async_copy(k_u.at[rr], k_v.at[rr], sem.at[1, s])
        cp["v", s] = pltpu.make_async_copy(v_u.at[rr], v_v.at[rr], sem.at[2, s])
        cp["o", s] = pltpu.make_async_copy(o_v.at[rr], o_u.at[rr], osem.at[s])
    for a in range(NC):
        cp["s", a] = pltpu.make_async_copy(ssm_u.at[:, lanes(a)], ssm_v.at[a], ssem.at[a])
    for i in range(7):
        rr = pl.ds(i * 128, min(128, F // 2 - i * 128))
        cp["w1", i] = pltpu.make_async_copy(w1_u.at[rr], w1_v.at[rr], wsem.at[0, i])
    for c in range(NL):
        cp["w2", c] = pltpu.make_async_copy(w2_u.at[:, lanes(c)], w2_v.at[c], wsem.at[1, c])

    skt = sk_ref[...].astype(f32)
    dd = dd_ref[...].astype(f32)[None, :]
    b2 = b2_ref[...].astype(f32)[None, :]

    def ln(s, h, mark=None):
        r0 = s * TM + h * 16
        xs = [x_v[pl.ds(r0 // 2, 8), lanes(c)] for c in range(NL)]
        if mark is not None:
            xs = [after(v, mark) for v in xs]
        x = upk(jnp.concatenate(xs, 1)).astype(f32)
        m = jnp.mean(x, axis=-1, keepdims=True)
        xc = x - m
        var = jnp.mean(xc * xc, axis=-1, keepdims=True)
        xn = xc * jax.lax.rsqrt(var + 1e-5)
        xn_v[pl.ds(r0, 16), :] = xn
        xb_v[pl.ds(r0 // 2, 8), :] = pk(xn.astype(bf16))

    def kload(a, c, mark):
        u = (a * NL + c) % NKF
        if a == 0:
            kf[u, 0:8, :] = jnp.zeros((8, 128), f32)
        for r in range(-8 if a else 0, C // 2, 8):
            k2 = upk(after(k_v[pl.ds(a * C // 2 + r, 8), lanes(c)], mark)).astype(f32)
            if r < 0:
                kf[u, 0:8, :] = k2[8:16]
            else:
                kf[u, pl.ds(8 + 2 * r, 16), :] = k2

    def kvp(a, c, hf, mark):
        u = (a * NL + c) % NKF
        n = C // 2
        r0 = hf * n
        cs = slice(c * 128, (c + 1) * 128)
        w0 = after(jnp.broadcast_to(skt[0:1, cs], (8, 128)), mark)
        ksh = (kf[u, pl.ds(8 + r0, n), :].reshape(n // 8, 8, 128) * w0[None]).reshape(n, 128)
        for t in range(1, 4):
            ksh = ksh + kf[u, pl.ds(8 + r0 - t, n), :] * skt[t:t + 1, cs]
        kv = ksh * upk(v_v[pl.ds((a * C + r0) // 2, n // 2), lanes(c)]).astype(f32)
        kvd_v[pl.ds(a * C + r0, n), lanes(c)] = kv * dd[:, cs]
        kvb_v[a, c, pl.ds(r0 // 2, n // 2), :] = pk(kv.astype(bf16))

    def fwd(a, c):
        kk = jax.lax.dot_general(upk(fk_ref[...]), upk(ssm_v[a, pl.ds(c * 64, 64), :]), (((1,), (1,)), ((), ())),
                                 preferred_element_type=f32).reshape(NG, 2, 8, 128)
        zs[z0 + NC + a, c, :, 0] = kk[:, 1] - kk[:, 0]
        zs[z0 + NC + a, c, :, 1] = kk[:, 0]
        zs[z0 + NC + a, c, :, 2] = kk[:, 1]
        uu = jnp.dot(upk(fu_ref[...]), upk(kvb_v[a, c]), preferred_element_type=f32).reshape(NG, 2, 8, 128)
        zs[z0 + a, c, :, 0] = uu[:, 0] + uu[:, 1]
        zs[z0 + a, c, :, 1] = uu[:, 0]
        zs[z0 + a, c, :, 2] = uu[:, 1]
        return [uu[i, 1] for i in range(NG)]

    part = {}

    def prod(s, c, g, t, mark):
        a0 = 2 * s
        acc = [None, None]
        ucur = zs[z0 + a0 + 1, c, g, t]
        for j in range(a0 + 2):
            kj = zs[z0 + NC + j, c, g, t]
            if j == 0:
                kj = after(kj, mark)
            p = kj * ucur
            acc[1] = p if acc[1] is None else acc[1] + p
            if a0 - j >= 0:
                ucur = zs[z0 + a0 - j, c, g, t]
                p = kj * ucur
                acc[0] = p if acc[0] is None else acc[0] + p
        part[t] = acc
        if t < 2:
            return
        pr, pi = [], []
        for o in range(2):
            hs = 0.5 * part[0][o]
            pr.append(hs - part[2][o])
            pi.append(hs + part[1][o])
        if s > 0:
            q0r, q0i = pr[0] + zs[z0 + PB, c, g, 1], pi[0] - zs[z0 + PB, c, g, 0]
        else:
            q0r, q0i = pr[0], pi[0]
        q1r, q1i = pr[1] + pi[0], pi[1] - pr[0]
        if s + 1 < NB:
            zs[z0 + PB, c, g, 0] = pr[1]
            zs[z0 + PB, c, g, 1] = pi[1]
        for a, qr, qi in ((a0, q0r, q0i), (a0 + 1, q1r, q1i)):
            zs[z0 + QB + a // 3, c, g, a % 3] = pltpu.bitcast(jnp.concatenate([qr, qi], 0).astype(bf16), f32)

    def mm1(s, i, sync):
        f0 = i * 128
        fn = min(128, F - f0)
        xb = upk(xb_v[pl.ds(s * TM // 2, TM // 2), :])
        w = upk(w1_v[pl.ds(f0 // 2, fn // 2), :])
        h = jax.lax.dot_general(xb, w, (((1,), (1,)), ((), ())), preferred_element_type=f32)
        sync()
        h = h + b1_ref[pl.ds(f0, fn)].astype(f32)[None, :]
        c0 = np.float32(np.sqrt(2 / np.pi))
        c1 = np.float32(np.sqrt(2 / np.pi) * 0.044715)
        t = jnp.tanh(h * (c0 + c1 * (h * h)))
        g_v[i, :, 0:fn] = pk((h + h * t).astype(bf16))
        return [h[r:r + 8] for r in range(0, TM, 8)] if fn == 128 else []

    def mm2(s, c, m, sync):
        t0, t1 = KG[m], KG[m + 1]
        k0, k1 = t0 * 128, min(t1 * 128, F)
        g = upk(jnp.concatenate([g_v[i, :, 0:min(128, F - i * 128)] for i in range(t0, t1)], 1))
        o = jnp.dot(g, upk(w2_v[c, k0 // 2:k1 // 2, :]), preferred_element_type=f32)
        sync()
        if m > 0:
            o = o + acc_v[z0]
        if m < len(KG) - 2:
            acc_v[z0] = o
        else:
            ff_v[s % 2, :, lanes(c)] = 0.5 * o + b2[:, c * 128:(c + 1) * 128]
        return [o[r:r + 8] for r in range(0, TM, 8)]

    def inv(a, c):
        rr = pl.ds(a * C, C)
        y = jnp.dot(upk(inv_ref[...]), upk(zs[z0 + QB + a // 3, c, :, a % 3].reshape(C, 128)), preferred_element_type=f32)
        x = upk(x_v[pl.ds(a * C // 2, C // 2), lanes(c)]).astype(f32)
        r = xn_v[rr, lanes(c)] * (y + kvd_v[rr, lanes(c)]) + x + ff_v[a // 2 % 2, pl.ds((a % 2) * C, C), lanes(c)]
        o_v[pl.ds(a * C // 2, C // 2), lanes(c)] = pk(r.astype(bf16))
        return [y[i:i + 8] for i in range(0, C, 8)]

    NM = len(KG) - 1
    NP = 14 + NL * NM
    fwd_slot, inv_slot, side_slot, need = {}, {}, {}, {}

    def first_use(key, t):
        need[key] = min(need.get(key, t), t)

    for s in range(NB):
        items = [(a, c) for a in FWD_AT[s] for c in range(NL)]
        lo = F1 if s == 1 else 0
        for i, (a, c) in enumerate(items):
            t = s * NP + lo + i * (NP - lo) // len(items)
            fwd_slot.setdefault(t, []).append((a, c))
            side_slot.setdefault(t - LAG - 1, []).append((kload, (a, c), 30))
            for hf in range(2):
                side_slot.setdefault(t - LAG, []).append((kvp, (a, c, hf), 90))
            first_use(("k", a // 2), t - LAG - 1)
            first_use(("v", a // 2), t - LAG - 1)
            first_use(("s", a), t)
        if s > 0:
            for h in range(16):
                lo1 = 14 + 3 * NM if s == 1 else 15
                t = (s - 1) * NP + lo1 + h * (NP - 2 - lo1) // 16
                side_slot.setdefault(t, []).append((ln, (s, h), 80))
                first_use(("x", s), t)
        for c in range(NL):
            t = s * NP + 14 + NM * (c + 1) - 1 + (NP if s < INVD else 0)
            inv_slot.setdefault(t, []).extend([(2 * s, c), (2 * s + 1, c)])
    for i in range(2, 7):
        first_use(("w1", i), 2 * i)
    for c in range(NL):
        first_use(("w2", c), 14 + NM * c)
    order = [("x", 0)] + [("w1", i) for i in range(7)] + [("w2", 0), ("w2", 1), ("w2", 2), ("x", 1), ("w2", 3), ("w2", 4)]
    order += sorted((k for k in need if k not in order), key=lambda k: need[k])
    tiles, even = 0, []
    for t in range(NB * NP):
        i = t % NP
        tiles += 5 if i < 14 else KG[(i - 14) % NM + 1] - KG[(i - 14) % NM]
        if tiles % 4 == 0:
            even.append(t)
        tiles += 2 * len(fwd_slot.get(t, [])) + 2 * len(inv_slot.get(t, []))
    points = [3, 7, 11, 13 + NM, 13 + 3 * NM, 13 + 4 * NM]
    points += [max(t for t in even if t <= int(p * NP)) for p in PTS]
    waits, ostart = {}, {}
    for k, t in need.items():
        waits.setdefault(max(p for p in points if p < t), []).append(k)
    for s in range(NB - 1):
        done = max(t for t, its in inv_slot.items() if (2 * s, NL - 1) in its)
        ostart.setdefault(min(p for p in points if p > done), []).append(s)

    queue = [(s, c, g) for s in range(NB) for c in range(NL) for g in range(NG)]
    fwd_done = set()
    state = dict(pos=0, credit=0.0)

    def products(budget, force, side):
        state["credit"] += budget
        while state["pos"] < len(queue):
            s, c, g = queue[state["pos"]]
            if (2 * s + 1, c) not in fwd_done:
                assert (s, c) > force
                state["credit"] = min(state["credit"], 0.0)
                break
            if state["credit"] <= 0 and (s, c) > force:
                break
            if state["credit"] <= 0:
                state["forced"] = state.get("forced", 0) + 1
            side.extend((prod, (s, c, g, t), 8 * s + 6 + 12 * (t == 2)) for t in range(3))
            state["credit"] -= 24 * s + 30
            state["pos"] += 1

    for key in order:
        cp[key].start()
    cp["x", 0].wait()
    for h in range(16):
        ln(0, h)
    cp["w1", 0].wait()
    cp["w1", 1].wait()
    carry = []
    force = (-1, 0)
    for s in range(NB):
        for i in range(NP):
            t = s * NP + i

            def sync():
                for key in waits.get(t, []):
                    cp[key].wait()
                for b in ostart.get(t, []):
                    cp["o", b].start()

            c, m = divmod(i - 14, NM)
            side = carry + side_slot.get(t, [])
            marks = []
            load = dict(dur=0.0, base=sum(p[-1] for p in side_slot.get(t, [])))

            def add(vals, dur, base):
                marks.extend((v, dur / len(vals)) for v in vals)
                load["dur"] += dur
                load["base"] += base

            if i < 14:
                add(mm1(s, i, sync), 320, 400 if i < 13 else 200)
            else:
                add(mm2(s, c, m, sync), 64 * (KG[m + 1] - KG[m]), 32 * (KG[m + 1] - KG[m]) + 32 * (m == NM - 1))
            for it in inv_slot.get(t, []):
                add(inv(*it), 64, 104)
            for it in fwd_slot.get(t, []):
                add(fwd(*it), 128, FB)
            for a, cc in inv_slot.get(t + LAG, []):
                force = max(force, (a // 2, cc))
            products(max(0.0, DENS * load["dur"] - load["base"]), force, side)
            if state["pos"] == len(queue) and "end" not in state:
                state["end"] = t
            fwd_done.update(fwd_slot.get(t, []))
            carry = []
            if not marks:
                carry = side
                continue
            tot, span = sum(p[-1] for p in side), sum(d for _, d in marks)
            cum, pos, j = 0.0, 0.0, 0
            for fn, args, w in side:
                while j < len(marks) - 1 and pos < span * cum / tot:
                    pos += marks[j][1]
                    j += 1
                fn(*args, marks[j][0])
                cum += w
    cp["o", NB - 1].start()
    for s in range(NB):
        cp["o", s].wait()


NKF = 24


@jax.jit
def pallas_parallel_sum__ssm_conv_h3__dense_activation_gelu__prompt_kernel(A_q, A_k, A_v, A_shift_k, A_ssm_k, A_ssm_D, B_x, B_w1, B_b1, B_w2, B_b2):
    fu, fk, inv = _dft_mats()
    hbm = pl.BlockSpec(memory_space=pl.ANY)
    vm = pl.BlockSpec(memory_space=pltpu.VMEM)
    V = pltpu.VMEM
    out = pl.pallas_call(
        kern,
        in_specs=[pl.BlockSpec(memory_space=pltpu.SMEM), hbm, hbm, hbm, vm, hbm, vm, hbm, vm, hbm, vm, vm, vm, vm],
        out_specs=hbm,
        out_shape=jax.ShapeDtypeStruct((S, D), bf16),
        scratch_shapes=[
            V((S // 2, D), u32), V((S // 2, D), u32), V((S // 2, D), u32),
            V((NC, D // 2, C), u32), V((F // 2, D), u32), V((NL, F // 2, 128), u32), V((S // 2, D), u32),
            V((NKF, C + 8, 128), f32), V((S, D), f32), V((S // 2, D), u32), V((S, D), f32),
            V((NC, NL, C // 2, 128), u32), V((2, TM, D), f32), V((14, TM // 2, 128), u32), V((1, TM, 128), f32),
            V((PB + 1, NL, NG, 3, 8, 128), f32),
            pltpu.SemaphoreType.DMA((3, 8)), pltpu.SemaphoreType.DMA((2, 8)), pltpu.SemaphoreType.DMA((NC,)),
            pltpu.SemaphoreType.DMA((NB,)),
        ],
        compiler_params=pltpu.CompilerParams(vmem_limit_bytes=110 * 1024 * 1024),
    )(jnp.asarray(np.zeros((1,), np.int32)), A_q.reshape(S, D), A_k.reshape(S, D), A_v.reshape(S, D), A_shift_k.T,
      A_ssm_k, A_ssm_D, B_w1.T, B_b1, B_w2, B_b2, _pack(fu), _pack(fk), _pack(inv))
    return out.reshape(1, S, D)
```

```python
import numpy as np
import jax
import jax.numpy as jnp
from jax.experimental import pallas as pl
from jax.experimental.pallas import tpu as pltpu

S, D, F = 2048, 640, 1728
C = 128
NC = S // C
TM = 256
NB = S // TM
NL = D // 128
NG = C // 8
f32, bf16, u32 = jnp.float32, jnp.bfloat16, jnp.uint32
pk = lambda v: pltpu.bitcast(v, u32)
upk = lambda v: pltpu.bitcast(v, bf16)
RATE = int('104')
W1 = float('0.3')
W2 = (14 - 14 * W1) / 70
DENS = float('2.4')
F1 = int('8')
FB = int('140')
INVD = int('4')
PTS = [float(v) for v in '1.45,2.1,3.1,7.15'.split(',')]
JS = int('6')
PAD = int('1')
LAG = int('2')
KG = [int(v) for v in '0,4,8,11,14'.split(',')]
FWD = eval('[(1.5, 2, [0, 1]), (2, 3, [2, 3, 4, 5, 6]), (3, 4, [7, 8, 9, 10]), (4, 5, [11, 12, 13]), (5, 6, [14, 15])]')
GB = int('400')
QB = 2 * NC
PB = QB + 6


def _dft_mats():
    n = np.arange(C)[None, :]
    th = 2 * np.pi * (np.arange(C)[:, None] + 0.25) / C
    co, si = np.cos(th * n), np.sin(th * n)
    il = lambda a, b: np.stack([a.reshape(NG, 8, C), b.reshape(NG, 8, C)], 1).reshape(2 * C, C)
    return il(co, si), il(si - co, si + co), np.stack([co, si], 1).reshape(2 * C, C).T / C


def _pack(m):
    b = m.astype(np.float32).astype(jnp.bfloat16).view(np.uint16).astype(np.uint32)
    return b[0::2] | (b[1::2] << 16)


def kern(z_h, x_h, k_h, v_h, sk_h, ssm_h, dd_h, w1_h, b1_h, w2_h, b2_h, dft_h, o_h,
         x_v, k_v, v_v, ssm_v, w1_v, w2_v, o_v, kf, xn_v, xb_v, kvd_v, kvb_v, ff_v, g_v, acc_v, zs,
         dft_ref, z_ref, sk_ref, dd_ref, b1_ref, b2_ref,
         sem, wsem, ssem, osem, csem):
    def after(v, mark):
        if v.dtype != f32:
            mark = pltpu.bitcast(mark, v.dtype)
        return jnp.where(keep, v, mark)

    def lanes(c):
        return pl.ds(c * 128, 128)

    x_u, k_u, v_u, o_u = (r.bitcast(u32) for r in (x_h, k_h, v_h, o_h))
    ssm_u, w1_u, w2_u = (r.bitcast(u32) for r in (ssm_h, w1_h, w2_h))
    cp = {}
    for s in range(NB):
        rr = pl.ds(s * TM // 2, TM // 2)
        cp["x", s] = pltpu.make_async_copy(x_u.at[rr], x_v.at[rr], sem.at[0, s])
        cp["k", s] = pltpu.make_async_copy(k_u.at[rr], k_v.at[rr], sem.at[1, s])
        cp["v", s] = pltpu.make_async_copy(v_u.at[rr], v_v.at[rr], sem.at[2, s])
        cp["o", s] = pltpu.make_async_copy(o_v.at[rr], o_u.at[rr], osem.at[s])
    for a in range(NC):
        cp["s", a] = pltpu.make_async_copy(ssm_u.at[:, lanes(a)], ssm_v.at[a], ssem.at[a])
    for i in range(7):
        rr = pl.ds(i * 128, min(128, F // 2 - i * 128))
        cp["w1", i] = pltpu.make_async_copy(w1_u.at[rr], w1_v.at[rr], wsem.at[0, i])
    for c in range(NL):
        cp["w2", c] = pltpu.make_async_copy(w2_u.at[:, lanes(c)], w2_v.at[c], wsem.at[1, c])

    for i, (src, dst) in enumerate(((z_h, z_ref), (b1_h, b1_ref), (b2_h, b2_ref), (sk_h, sk_ref), (dd_h, dd_ref),
                                    (dft_h, dft_ref))):
        cp["c", i] = pltpu.make_async_copy(src, dst, csem.at[i])

    def ln(s, h, mark=None):
        r0 = s * TM + h * 16
        xs = [x_v[pl.ds(r0 // 2, 8), lanes(c)] for c in range(NL)]
        if mark is not None:
            xs = [after(v, mark) for v in xs]
        x = upk(jnp.concatenate(xs, 1)).astype(f32)
        m = jnp.mean(x, axis=-1, keepdims=True)
        xc = x - m
        var = jnp.mean(xc * xc, axis=-1, keepdims=True)
        xn = xc * jax.lax.rsqrt(var + 1e-5)
        xn_v[pl.ds(r0, 16), :] = xn
        xb_v[pl.ds(r0 // 2, 8), :] = pk(xn.astype(bf16))

    def kload(a, c, mark):
        u = (a * NL + c) % NKF
        if a == 0:
            kf[u, 0:8, :] = jnp.zeros((8, 128), f32)
        for r in range(-8 if a else 0, C // 2, 8):
            k2 = upk(after(k_v[pl.ds(a * C // 2 + r, 8), lanes(c)], mark)).astype(f32)
            if r < 0:
                kf[u, 0:8, :] = k2[8:16]
            else:
                kf[u, pl.ds(8 + 2 * r, 16), :] = k2

    def kvp(a, c, hf, mark):
        u = (a * NL + c) % NKF
        n = C // 2
        r0 = hf * n
        cs = slice(c * 128, (c + 1) * 128)
        skt = sk_ref[:, cs].astype(f32)
        w0 = after(jnp.broadcast_to(skt[0:1], (8, 128)), mark)
        ksh = (kf[u, pl.ds(8 + r0, n), :].reshape(n // 8, 8, 128) * w0[None]).reshape(n, 128)
        for t in range(1, 4):
            ksh = ksh + kf[u, pl.ds(8 + r0 - t, n), :] * skt[t:t + 1]
        kv = ksh * upk(v_v[pl.ds((a * C + r0) // 2, n // 2), lanes(c)]).astype(f32)
        kvd_v[pl.ds(a * C + r0, n), lanes(c)] = kv * dd_ref[lanes(c)].astype(f32)[None, :]
        kvb_v[a, pl.ds(r0 // 2, n // 2), lanes(c)] = pk(kv.astype(bf16))

    def fwd(a, c):
        kk = jax.lax.dot_general(upk(dft_ref[:, 128:256]), upk(ssm_v[a, pl.ds(c * 64, 64), :]), (((1,), (1,)), ((), ())),
                                 preferred_element_type=f32).reshape(NG, 2, 8, 128)
        zs[z0 + NC + a, c, 0:NG, 0] = kk[:, 1] - kk[:, 0]
        zs[z0 + NC + a, c, 0:NG, 1] = kk[:, 0]
        zs[z0 + NC + a, c, 0:NG, 2] = kk[:, 1]
        uu = jnp.dot(upk(dft_ref[:, 0:128]), upk(kvb_v[a, :, lanes(c)]), preferred_element_type=f32).reshape(NG, 2, 8, 128)
        zs[z0 + a, c, 0:NG, 0] = uu[:, 0] + uu[:, 1]
        zs[z0 + a, c, 0:NG, 1] = uu[:, 0]
        zs[z0 + a, c, 0:NG, 2] = uu[:, 1]
        return [uu[i, 1] for i in range(NG)]

    part = {}

    def prod(s, c, g, t, j0, j1, mark):
        a0 = 2 * s
        if j0 == 0:
            part[t], part["u"] = [None, None], zs[z0 + a0 + 1, c, g, t]
        acc = part[t]
        for j in range(j0, j1):
            kj = zs[z0 + NC + j, c, g, t]
            if j == j0:
                kj = after(kj, mark)
            p = kj * part["u"]
            acc[1] = p if acc[1] is None else acc[1] + p
            if a0 - j >= 0:
                part["u"] = zs[z0 + a0 - j, c, g, t]
                p = kj * part["u"]
                acc[0] = p if acc[0] is None else acc[0] + p
        if t < 2 or j1 < a0 + 2:
            return
        pr, pi = [], []
        for o in range(2):
            hs = 0.5 * part[0][o]
            pr.append(hs - part[2][o])
            pi.append(hs + part[1][o])
        if s > 0:
            q0r, q0i = pr[0] + zs[z0 + PB, c, g, 1], pi[0] - zs[z0 + PB, c, g, 0]
        else:
            q0r, q0i = pr[0], pi[0]
        q1r, q1i = pr[1] + pi[0], pi[1] - pr[0]
        if s + 1 < NB:
            zs[z0 + PB, c, g, 0] = pr[1]
            zs[z0 + PB, c, g, 1] = pi[1]
        for a, qr, qi in ((a0, q0r, q0i), (a0 + 1, q1r, q1i)):
            zs[z0 + QB + a // 3, c, g, a % 3] = pltpu.bitcast(pltpu.pack_elementwise([qr, qi], packed_dtype=bf16), f32)

    def mm1(s, i, sync):
        f0 = i * 128
        fn = min(128, F - f0)
        xb = upk(xb_v[pl.ds(s * TM // 2, TM // 2), :])
        w = upk(w1_v[pl.ds(f0 // 2, fn // 2), :])
        h = jax.lax.dot_general(xb, w, (((1,), (1,)), ((), ())), preferred_element_type=f32)
        sync()
        h = h + b1_ref[pl.ds(f0, fn)].astype(f32)[None, :]
        c0 = np.float32(np.sqrt(2 / np.pi))
        c1 = np.float32(np.sqrt(2 / np.pi) * 0.044715)
        t = jnp.tanh(h * (c0 + c1 * (h * h)))
        g_v[s % 2, :, pl.ds(f0, fn)] = pk((h + h * t).astype(bf16))
        return [h[r:r + 8] for r in range(0, TM, 8)] if fn == 128 else []

    def mm2(s, c, m, sync):
        t0, t1 = KG[m], KG[m + 1]
        k0, k1 = t0 * 128, min(t1 * 128, F)
        g = upk(g_v[s % 2, :, k0:k1])
        o = jnp.dot(g, upk(w2_v[c, k0 // 2:k1 // 2, :]), preferred_element_type=f32)
        sync()
        if m > 0:
            o = o + acc_v[z0]
        if m < len(KG) - 2:
            acc_v[z0] = o
        else:
            ff_v[s % 3, :, lanes(c)] = 0.5 * o + b2_ref[lanes(c)].astype(f32)[None, :]
        return [o[r:r + 8] for r in range(0, TM, 8)]

    def inv(a, c):
        rr = pl.ds(a * C, C)
        y = jnp.dot(upk(dft_ref[0:C // 2, 256:512]), upk(zs[z0 + QB + a // 3, c, 0:NG, a % 3].reshape(C, 128)), preferred_element_type=f32)
        x = upk(x_v[pl.ds(a * C // 2, C // 2), lanes(c)]).astype(f32)
        r = xn_v[rr, lanes(c)] * (y + kvd_v[rr, lanes(c)]) + x + ff_v[a // 2 % 3, pl.ds((a % 2) * C, C), lanes(c)]
        o_v[pl.ds(a * C // 2, C // 2), lanes(c)] = pk(r.astype(bf16))
        return [y[i:i + 8] for i in range(0, C, 8)]

    NM = len(KG) - 1
    NP = 14 + NL * NM
    up = lambda s: [(mm1, s, i) for i in range(14)]
    down = lambda s: [(mm2, s, c, m) for c in range(NL) for m in range(NM)]
    slots = [(mm1, s, 2 * p + i) for p in range(7) for s in (0, 1) for i in (0, 1)] + down(0) + down(1)
    for s in range(2, NB):
        slots += up(s) + down(s)
    at = {sl: t for t, sl in enumerate(slots)}
    fwd_slot, inv_slot, side_slot, need = {}, {}, {}, {}

    def first_use(key, t):
        need[key] = min(need.get(key, t), t)

    for lo, hi, chunks in FWD:
        items = [(a, c) for a in chunks for c in range(NL)]
        for i, (a, c) in enumerate(items):
            t = int((lo + (hi - lo) * i / len(items)) * NP)
            fwd_slot.setdefault(t, []).append((a, c))
            side_slot.setdefault(t - LAG - 1, []).append((kload, (a, c), 30))
            for hf in range(2):
                side_slot.setdefault(t - LAG, []).append((kvp, (a, c, hf), 90))
            first_use(("k", a // 2), t - LAG - 1)
            first_use(("v", a // 2), t - LAG - 1)
            first_use(("s", a), t)
            first_use(("c", 3), t - LAG)
            first_use(("c", 4), t - LAG)
            first_use(("c", 5), t)
    for s in range(NB):
        if s > 1:
            for h in range(16):
                t = (s - 1) * NP + 15 + h * (NP - 17) // 16
                side_slot.setdefault(t, []).append((ln, (s, h), 80))
                first_use(("x", s), t)
        for c in range(NL):
            t = at[mm2, max(s + 1, 2) if s < INVD else s, c, NM - 1] - (NM if s < INVD else 0)
            inv_slot.setdefault(t, []).extend([(2 * s, c), (2 * s + 1, c)])
    for i in range(1, 7):
        first_use(("w1", i), at[mm1, 0, 2 * i])
    for c in range(NL):
        first_use(("w2", c), at[mm2, 0, c, 0])
    first_use(("c", 2), at[mm2, 0, 0, 0])
    tiles, even = 0, []
    for t, sl in enumerate(slots):
        tiles += 5 if sl[0] is mm1 else KG[sl[3] + 1] - KG[sl[3]]
        if tiles % 4 == 0:
            even.append(t)
        tiles += 2 * len(fwd_slot.get(t, [])) + len(inv_slot.get(t, []))
    points = [3, 11, 27] + [max(t for t in even if t <= int(p * NP)) for p in PTS]
    waits, ostart = {}, {}
    for k, t in need.items():
        waits.setdefault(max(p for p in points if p < t), []).append(k)
    for s in range(NB - 1):
        done = max(t for t, its in inv_slot.items() if (2 * s, NL - 1) in its)
        ostart.setdefault(min(p for p in points if p > done), []).append(s)

    queue = [(s, c, g) for s in range(NB) for c in range(NL) for g in range(NG)]
    fwd_done = set()
    state = dict(pos=0, credit=0.0)

    def products(budget, force, side):
        state["credit"] += budget
        while state["pos"] < len(queue):
            s, c, g = queue[state["pos"]]
            if (2 * s + 1, c) not in fwd_done:
                assert (s, c) > force
                state["credit"] = min(state["credit"], 0.0)
                break
            if state["credit"] <= 0 and (s, c) > force:
                break
            if state["credit"] <= 0:
                state["forced"] = state.get("forced", 0) + 1
            n = -(-(2 * s + 2) // JS)
            cuts = [(2 * s + 2) * i // n for i in range(n + 1)]
            side.extend((prod, (s, c, g, t, j0, j1), 4 * (j1 - j0) + 12 * (t == 2 and j1 == cuts[-1]))
                        for t in range(3) for j0, j1 in zip(cuts, cuts[1:]))
            state["credit"] -= 24 * s + 30
            state["pos"] += 1

    for key in [("c", 0), ("c", 1), ("x", 0), ("x", 1), ("w1", 0)] + sorted(need, key=lambda k: need[k]):
        cp[key].start()
    for s in (0, 1):
        cp["x", s].wait()
        for h in range(16):
            ln(s, h)
    for key in (("w1", 0), ("c", 0), ("c", 1)):
        cp[key].wait()
    z0 = z_ref[0]
    keep = jax.lax.broadcasted_iota(jnp.int32, (8, 128), 0) >= z0
    carry = []
    force = (-1, 0)
    for t, sl in enumerate(slots):
        def sync():
            for key in waits.get(t, []):
                cp[key].wait()
            for b in ostart.get(t, []):
                cp["o", b].start()

        side = carry + side_slot.get(t, [])
        marks = []
        load = dict(dur=0.0, base=sum(p[-1] for p in side_slot.get(t, [])))

        def add(vals, dur, base):
            marks.extend((v, dur / len(vals)) for v in vals)
            load["dur"] += dur
            load["base"] += base

        if sl[0] is mm1:
            add(mm1(*sl[1:], sync), 320, GB if sl[2] < 13 else GB // 2)
        else:
            n = KG[sl[3] + 1] - KG[sl[3]]
            add(mm2(*sl[1:], sync), 64 * n, 32 * n + 32 * (sl[3] == NM - 1))
        for it in inv_slot.get(t, []):
            add(inv(*it), 64, 104)
        for it in fwd_slot.get(t, []):
            add(fwd(*it), 128, FB)
        for a, cc in inv_slot.get(t + LAG, []):
            force = max(force, (a // 2, cc))
        products(max(0.0, DENS * load["dur"] - load["base"]), force, side)
        if state["pos"] == len(queue) and "end" not in state:
            state["end"] = t
        fwd_done.update(fwd_slot.get(t, []))
        carry = []
        if not marks:
            carry = side
            continue
        tot, span = sum(p[-1] for p in side), sum(d for _, d in marks)
        cum, pos, j = 0.0, 0.0, 0
        for fn, args, w in side:
            while j < len(marks) - 1 and pos < span * cum / tot:
                pos += marks[j][1]
                j += 1
            fn(*args, marks[j][0])
            cum += w
    cp["o", NB - 1].start()
    for s in range(NB):
        cp["o", s].wait()


NKF = 24


@jax.jit
def pallas_parallel_sum__ssm_conv_h3__dense_activation_gelu__prompt_kernel(A_q, A_k, A_v, A_shift_k, A_ssm_k, A_ssm_D, B_x, B_w1, B_b1, B_w2, B_b2):
    fu, fk, inv = _dft_mats()
    hbm = pl.BlockSpec(memory_space=pl.ANY)
    V = pltpu.VMEM
    out = pl.pallas_call(
        kern,
        in_specs=[hbm] * 12,
        out_specs=hbm,
        out_shape=jax.ShapeDtypeStruct((S, D), bf16),
        scratch_shapes=[
            V((S // 2, D), u32), V((S // 2, D), u32), V((S // 2, D), u32),
            V((NC, D // 2, C), u32), V((F // 2, D), u32), V((NL, F // 2, 128), u32), V((S // 2, D), u32),
            V((NKF, C + 8, 128), f32), V((S, D), f32), V((S // 2, D), u32), V((S, D), f32),
            V((NC, C // 2, D), u32), V((3, TM, D), f32), V((2, TM // 2, 14 * 128), u32), V((1, TM, 128), f32),
            V((PB + 1, NL, NG + PAD, 3, 8, 128), f32),
            V((C, 4 * C), u32), pltpu.SMEM((1,), jnp.int32), V((4, D), bf16), V((D,), bf16), V((F,), bf16), V((D,), bf16),
            pltpu.SemaphoreType.DMA((3, 8)), pltpu.SemaphoreType.DMA((2, 8)), pltpu.SemaphoreType.DMA((NC,)),
            pltpu.SemaphoreType.DMA((NB,)), pltpu.SemaphoreType.DMA((6,)),
        ],
        compiler_params=pltpu.CompilerParams(vmem_limit_bytes=110 * 1024 * 1024),
    )(jnp.asarray(np.zeros((1,), np.int32)), A_q.reshape(S, D), A_k.reshape(S, D), A_v.reshape(S, D), A_shift_k.T,
      A_ssm_k, A_ssm_D, B_w1.T, B_b1, B_w2, B_b2, np.concatenate([_pack(fu), _pack(fk), np.pad(_pack(inv), ((0, C // 2), (0, 0)))], 1))
    return out.reshape(1, S, D)
```

```python
import functools
import numpy as np
import jax
import jax.numpy as jnp
from jax.experimental import pallas as pl
from jax.experimental.pallas import tpu as pltpu

S, D, F = 2048, 640, 1728
C = 128
NC = S // C
TM = 256
NB = S // TM
NL = D // 128
NG = C // 8
f32, bf16, u32 = jnp.float32, jnp.bfloat16, jnp.uint32
pk = lambda v: pltpu.bitcast(v, u32)
upk = lambda v: pltpu.bitcast(v, bf16)
RATE = int('104')
W1 = float('0.3')
W2 = (14 - 14 * W1) / 70
DENS = eval('[2.36]')
U0 = float('0.45')
F1 = int('8')
FB = int('80')
PTS = [float(v) for v in '1.45,2.1,2.95,7.15'.split(',')]
JS = int('5')
PAD = int('1')
LS = int('12')
HZ = int('0')
KQ = int('4')
IW = int('0')
MIX = int('1')
KN = int('3')
UN = int('3')
KO = int('1')
G2 = int('0')
I6 = int('2')
LAG = int('2')
KG = [int(v) for v in '0,4,8,11,14'.split(',')]
FWD = eval('[(1.6, 2.1, [0, 1], True), (2.22, 3, [2, 3, 4, 5, 6], True), (3.1, 4, [7, 8, 9, 10], True), (4, 5, [11, 12, 13], True), (5, 6, [14, 15], True)]')
GB = int('340')
UB = 0
NM = len(KG) - 1
NP = 14 + NL * NM


def _dft_mats():
    n = np.arange(C)[None, :]
    th = 2 * np.pi * (np.arange(C)[:, None] + 0.25) / C
    co, si = np.cos(th * n), np.sin(th * n)
    il = lambda a, b: np.stack([a.reshape(NG, 8, C), b.reshape(NG, 8, C)], 1).reshape(2 * C, C)
    return il(co, si), il(si - co, si + co), np.stack([co, si], 1).reshape(2 * C, C).T / C


def _pack(m):
    b = m.astype(np.float32).astype(jnp.bfloat16).view(np.uint16).astype(np.uint32)
    return b[0::2] | (b[1::2] << 16)


def kern(z_h, x_h, k_h, v_h, sk_h, ssm_h, dd_h, w1_h, b1_h, w2_h, b2_h, dft_h, o_h,
         x_v, k_v, v_v, ssm_v, w1_v, w2_v, o_v, kf, xn_v, xb_v, kvd_v, kvb_v, ff_v, g_v, acc_v, us, ks, qs, pp,
         dft_ref, z_ref, sk_ref, dd_ref, b1_ref, b2_ref,
         sem, wsem, ssem, osem, csem):
    def after(v, mark):
        if v.dtype != f32:
            mark = pltpu.bitcast(mark, v.dtype)
        return jnp.where(keep, v, mark)

    def lanes(c):
        return pl.ds(c * 128, 128)

    x_u, k_u, v_u, o_u = (r.bitcast(u32) for r in (x_h, k_h, v_h, o_h))
    ssm_u, w1_u, w2_u = (r.bitcast(u32) for r in (ssm_h, w1_h, w2_h))
    cp = {}
    for s in range(NB):
        rr = pl.ds(s * TM // 2, TM // 2)
        cp["x", s] = pltpu.make_async_copy(x_u.at[rr], x_v.at[rr], sem.at[0, s])
        cp["k", s] = pltpu.make_async_copy(k_u.at[rr], k_v.at[rr], sem.at[1, s])
        cp["v", s] = pltpu.make_async_copy(v_u.at[rr], v_v.at[rr], sem.at[2, s])
    for a in range(NC):
        cp["s", a] = pltpu.make_async_copy(ssm_u.at[:, lanes(a)], ssm_v.at[a], ssem.at[a])
    for i in range(7):
        rr = pl.ds(i * 128, min(128, F // 2 - i * 128))
        cp["w1", i] = pltpu.make_async_copy(w1_u.at[rr], w1_v.at[rr], wsem.at[0, i])
    for c in range(NL):
        cp["w2", c] = pltpu.make_async_copy(w2_u.at[:, lanes(c)], w2_v.at[c], wsem.at[1, c])

    for i, (src, dst) in enumerate(((z_h, z_ref), (b1_h, b1_ref), (b2_h, b2_ref), (sk_h, sk_ref), (dd_h, dd_ref),
                                    (dft_h, dft_ref))):
        cp["c", i] = pltpu.make_async_copy(src, dst, csem.at[i])

    class Pos:
        def __init__(self, blk):
            static = isinstance(blk, int)
            self.half = blk * (TM // 2) if static else pl.multiple_of(blk * (TM // 2), TM // 2)
            self.full = blk * TM if static else pl.multiple_of(blk * TM, TM)
            self.chunk = 2 * blk
            self.z = z0 + 2 * blk if z0 is not None else None

    norm = {}

    def ln(p, s, h, stage, mark=None):
        r0 = s * TM + h * 16
        later = lambda v: v if mark is None else after(v.reshape(2, 8, 128), mark[None]).reshape(16, 128)
        wide = lambda v: jnp.broadcast_to(v, (16, 128))
        if stage == 0:
            xs = [x_v[pl.ds(p.half + r0 // 2, 8), lanes(c)] for c in range(NL)]
            xs = [upk(v if mark is None else after(v, mark)).astype(f32) for v in xs]
            norm[s, h] = xs, wide(jnp.sum(functools.reduce(jnp.add, xs), axis=-1, keepdims=True))
        elif stage == 1:
            xs, total = norm[s, h]
            m = later(total) * (1.0 / D)
            xc = [x - m for x in xs]
            norm[s, h] = xc, wide(jnp.sum(functools.reduce(jnp.add, [v * v for v in xc]), axis=-1, keepdims=True))
        else:
            xc, total = norm.pop((s, h))
            r = jax.lax.rsqrt(later(total) * (1.0 / D) + 1e-5)
            for c in range(NL):
                xn = xc[c] * r
                xn_v[pl.ds(p.full + r0, 16), lanes(c)] = xn
                xb_v[pl.ds(p.half + r0 // 2, 8), lanes(c)] = pk(xn.astype(bf16))

    def kload(p, a, c, mark):
        u = (a * NL + c) % NKF
        first = isinstance(p.chunk, int) and p.chunk + a == 0
        if first:
            kf[u, 0:8, :] = jnp.zeros((8, 128), f32)
        for r in range(0 if first else -8, C // 2, 8):
            k2 = upk(after(k_v[pl.ds(p.half + (a * C // 2 + r), 8), lanes(c)], mark)).astype(f32)
            if r < 0:
                kf[u, 0:8, :] = k2[8:16]
            else:
                kf[u, pl.ds(8 + 2 * r, 16), :] = k2

    def kvp(p, a, c, hf, mark):
        u = (a * NL + c) % NKF
        n = C // KQ
        r0 = hf * n
        skt = sk_ref[:, lanes(c)].astype(f32)
        w0 = after(jnp.broadcast_to(skt[0:1], (8, 128)), mark)
        ksh = (kf[u, pl.ds(8 + r0, n), :].reshape(n // 8, 8, 128) * w0[None]).reshape(n, 128)
        for t in range(1, 4):
            ksh = ksh + kf[u, pl.ds(8 + r0 - t, n), :] * skt[t:t + 1]
        rows = pl.ds(p.half + (a * C + r0) // 2, n // 2)
        kv = ksh * upk(v_v[rows, lanes(c)]).astype(f32)
        kvd_v[pl.ds(p.full + (a * C + r0), n), lanes(c)] = kv * dd_ref[lanes(c)].astype(f32)[None, :]
        kvb_v[rows, lanes(c)] = pk(kv.astype(bf16))

    def clear(p, ref, j, c, mark):
        zero = after(jnp.zeros((8, 128), f32), mark)
        ref[j, c] = jnp.broadcast_to(zero, ref.shape[2:])

    def fwd_k(p, a, c):
        kk = jax.lax.dot_general(upk(dft_ref[:, 128:256]), upk(ssm_v[p.chunk + a, pl.ds(c * 64, 64), :]),
                                 (((1,), (1,)), ((), ())), preferred_element_type=f32).reshape(NG, 2, 8, 128)
        ks[p.z + a, c, 0:NG, KO % KN] = kk[:, 1] - kk[:, 0]
        ks[p.z + a, c, 0:NG, (KO + 1) % KN] = kk[:, 0]
        ks[p.z + a, c, 0:NG, (KO + 2) % KN] = kk[:, 1]
        return [kk[i, 1] for i in range(NG)]

    def fwd_u(p, a, c):
        kv = upk(kvb_v[pl.ds(p.half + a * C // 2, C // 2), lanes(c)])
        uu = jnp.dot(upk(dft_ref[:, 0:128]), kv, preferred_element_type=f32).reshape(NG, 2, 8, 128)
        us[p.z + (UB + a), c, 0:NG, 0] = uu[:, 0] + uu[:, 1]
        us[p.z + (UB + a), c, 0:NG, 1] = uu[:, 0]
        us[p.z + (UB + a), c, 0:NG, 2] = uu[:, 1]
        return [uu[i, 1] for i in range(NG)]

    part = {}

    def prod(p, a0, lags, c, g, t, j0, j1, mark):
        if j0 == 0:
            part[t], part["u"] = [None, None], us[p.z + (UB + a0 + 1), c, g, t]
        acc = part[t]
        for j in range(j0, j1):
            kj = ks[z0 + j, c, g, (KO + t) % KN]
            if j == j0:
                kj = after(kj, mark)
            pr = kj * part["u"]
            acc[1] = pr if acc[1] is None else acc[1] + pr
            if j < lags - 1:
                part["u"] = us[p.z + (UB + a0 - j), c, g, t]
                pr = kj * part["u"]
                acc[0] = pr if acc[0] is None else acc[0] + pr
        if t < 2 or j1 < lags:
            return
        last = (pp[z0, c, g, 0], pp[z0, c, g, 1]) if lags > 2 else None
        for o in range(2):
            hs = 0.5 * part[0][o]
            re, im = hs - part[2][o], hs + part[1][o]
            q = [re, im] if last is None else [re + last[1], im - last[0]]
            qs[p.z + (a0 + o), c, g] = pltpu.pack_elementwise(q, packed_dtype=bf16)
            last = (re, im)
        if lags < NC:
            pp[z0, c, g, 0] = last[0]
            pp[z0, c, g, 1] = last[1]

    def mm1(p, s, i, sync):
        f0 = i * 128
        fn = min(128, F - f0)
        xb = upk(xb_v[pl.ds(p.half + s * TM // 2, TM // 2), :])
        w = upk(w1_v[pl.ds(f0 // 2, 64), :])
        h = jax.lax.dot_general(xb, w, (((1,), (1,)), ((), ())), preferred_element_type=f32)
        sync()
        marks = [h[r:r + 8] for r in range(0, TM, 8)]
        h = h[:, :fn] + b1_ref[pl.ds(f0, fn)].astype(f32)[None, :]
        c0 = np.float32(np.sqrt(2 / np.pi))
        c1 = np.float32(np.sqrt(2 / np.pi) * 0.044715)
        t = jnp.tanh(h * (c0 + c1 * (h * h)))
        g_v[s % 2, :, pl.ds(f0, fn)] = pk((h + h * t).astype(bf16))
        return marks

    def mm2(p, s, c, m, sync):
        k0, k1 = KG[m] * 128, min(KG[m + 1] * 128, F)
        o = jnp.dot(upk(g_v[s % 2, :, k0:k1]), upk(w2_v[c, k0 // 2:k1 // 2, :]), preferred_element_type=f32)
        sync()
        if m > 0:
            o = o + acc_v[z0]
        if m < NM - 1:
            acc_v[z0] = o
        else:
            ff_v[pl.ds(p.full + s * TM, TM), lanes(c)] = 0.5 * o + b2_ref[lanes(c)].astype(f32)[None, :]
        return [o[r:r + 8] for r in range(0, TM, 8)]

    def inv(p, a, c):
        rr, rh = pl.ds(p.full + a * C, C), pl.ds(p.half + a * C // 2, C // 2)
        q = pltpu.bitcast(qs[p.z + a, c].reshape(C, 128), bf16)
        y = jnp.dot(upk(dft_ref[0:C // 2, 256:512]), q, preferred_element_type=f32)
        x = upk(x_v[rh, lanes(c)]).astype(f32)
        r = xn_v[rr, lanes(c)] * (y + kvd_v[rr, lanes(c)]) + x + ff_v[rr, lanes(c)]
        o_v[rh, lanes(c)] = pk(r.astype(bf16))
        return [y[i:i + 8] for i in range(0, C, 8)] if IW else []

    up = lambda s: [(mm1, s, i) for i in range(14)]
    down = lambda s: [(mm2, s, c, m) for c in range(NL) for m in range(NM)]
    tiles = lambda sl: 5 if sl[0] is mm1 else KG[sl[3] + 1] - KG[sl[3]]

    def plan(slots, head, fwds, lns, invs, prods, dens, extra=()):
        at = {sl: t for t, sl in enumerate(slots)}
        mxu, side, need, done = {}, {}, {}, {}
        for t, piece in extra:
            side.setdefault(t, []).append(piece)
        for lo, hi, chunks, with_k in fwds:
            items = [(a, c) for a in chunks for c in range(NL)]
            for i, (a, c) in enumerate(items):
                t = int((lo + (hi - lo) * i / len(items)) * NP)
                mxu.setdefault(t, []).extend([(fwd_k, a, c)] * with_k + [(fwd_u, a, c)])
                done[a, c] = t
                side.setdefault(t - LAG - 2, []).append((kload, (a, c), 30))
                for hf in range(KQ):
                    side.setdefault(t - LAG - (hf < KQ // 2), []).append((kvp, (a, c, hf), 180 // KQ))
                for key in (("k", a // 2), ("v", a // 2), ("c", 3), ("c", 4)):
                    need.setdefault(key, t - LAG - 2)
                for key in [("s", a)] * with_k + [("c", 5)]:
                    need.setdefault(key, t)
        for s, t0 in lns:
            need["x", s] = t0
            for h in range(TM // 16):
                for stage, w in enumerate((25, 32, 40)):
                    side.setdefault(t0 + h * LS // 16 + stage, []).append((ln, (s, h, stage), w))
        for s, host in invs:
            for c in range(NL):
                t = at[mm2, host, c, NM - 1] - NM * (host > s)
                mxu[t] = [(inv, 2 * s, c), (inv, 2 * s + 1, c)] + mxu.get(t, [])
        queue = [(a0, lags, c, g) for a0, lags in prods for c in range(NL) for g in range(NG)]
        credit = 0.0
        for t, sl in enumerate(slots):
            more = [it[0] for it in mxu.get(t, [])]
            busy = (GB if sl[2] < 13 else GB // 2) if sl[0] is mm1 else 32 * tiles(sl) + 32 * (sl[3] == NM - 1)
            busy += sum(104 if fn is inv else FB for fn in more) + sum(w for _, _, w in side.get(t, []))
            credit += (t < len(slots) - HZ) * max(0.0, dens * 64 * (tiles(sl) + len(more)) - busy)
            due = [(it[1], it[2]) for u in range(t, t + LAG + 1) for it in mxu.get(u, []) if it[0] is inv]
            while queue:
                a0, lags, c, g = queue[0]
                urgent = (a0, c) in due or t == len(slots) - 1 - HZ
                if done.get((a0 + 1, c), -1) >= t:
                    assert not urgent
                    credit = min(credit, 0.0)
                    break
                if credit <= 0 and not urgent:
                    break
                queue.pop(0)
                n = -(-lags // JS)
                cuts = [lags * i // n for i in range(n + 1)]
                side.setdefault(t, []).extend(
                    (prod, (a0, lags, c, g, comp, j0, j1), 4 * (j1 - j0) + 12 * (comp == 2 and j1 == lags))
                    for comp in range(3) for j0, j1 in zip(cuts, cuts[1:]))
                credit -= 12 * lags + 6
        print("compile", credit)
        return dict(slots=slots, head=head, mxu=mxu, side=side, need=need)

    def emit(p, pln, syncs):
        carry = []
        for t, sl in enumerate([None] + pln["slots"], -1):
            if sl is None:
                groups = [(fwd_k(p, a, c), 1) for a in pln["head"] for c in range(NL)]
            else:
                groups = [(sl[0](p, *sl[1:], syncs.get(t, lambda: None)), tiles(sl))]
                groups += [(it[0](p, *it[1:]), 1) for it in pln["mxu"].get(t, [])]
            marks = [(v, n / len(vals)) for vals, n in groups for v in vals]
            side = carry + pln["side"].get(t, [])
            if MIX:
                lists = [[it for it in side if it[0] is prod], [it for it in side if it[0] is not prod]]
                side = [it for _, it in sorted((((i + 0.5) / len(l), it) for l in lists for i, it in enumerate(l)),
                                               key=lambda e: e[0])]
            carry = [] if marks else side
            if not marks:
                continue
            tot, span = sum(w for _, _, w in side), sum(d for _, d in marks)
            cum, pos, j = 0.0, 0.0, 0
            for fn, args, w in side:
                while j < len(marks) - 1 and pos < span * cum / tot:
                    pos += marks[j][1]
                    j += 1
                fn(p, *args, marks[j][0])
                cum += w

    slots = [(mm1, s, 2 * q + i) for q in range(7) for s in (0, 1) for i in (0, 1)] + down(0) + down(1)
    for s in range(2, NB):
        slots += up(s) + down(s)
    first = plan(slots, [], FWD, [(s, (s - 1) * NP + 15) for s in range(2, NB)],
                 [(0, 2), (1, 3), (2, 3), (3, 4), (4, 4), (5, 5), (6, 6), (7, 7)],
                 [(2 * s, 2 * s + 2) for s in range(NB)], DENS[0])

    need = first["need"]
    need.update({("w1", i): 4 * i for i in range(1, 7)})
    need.update({key: 28 for key in [("c", 2)] + [("w2", c) for c in range(NL)]})

    def even_slots(pln):
        n, out = NL * len(pln["head"]), []
        for t, sl in enumerate(pln["slots"]):
            n += tiles(sl)
            if n % 4 == 0:
                out.append(t)
            n += len(pln["mxu"].get(t, []))
        return out

    points = [3, 11, 27] + [max(t for t in even_slots(first) if t <= int(q * NP)) for q in PTS]
    waits = {}
    for key, t in need.items():
        waits.setdefault(max(q for q in points if q < t), []).append(key)
    early = [("c", 0), ("c", 1), ("x", 0), ("x", 1), ("w1", 0)]
    late = [key for key in cp if key not in need and key not in early]
    for key in early + sorted(need, key=lambda k: need[k]) + late:
        cp[key].start()
    w1_v[F // 2:14 * 64, :] = jnp.zeros((14 * 64 - F // 2, D), u32)
    z0 = None
    for s in (0, 1):
        cp["x", s].wait()
        for h in range(TM // 16):
            for stage in range(3):
                ln(Pos(0), s, h, stage)
    for key in (("w1", 0), ("c", 0), ("c", 1)):
        cp[key].wait()
    z0 = z_ref[0]
    keep = jax.lax.broadcasted_iota(jnp.int32, (8, 128), 0) >= z0

    def out_copy(blk, cols=slice(None), sem=None):
        rr = pl.ds(Pos(blk).half, TM // 2)
        return pltpu.make_async_copy(o_v.at[rr, cols], o_u.at[rr, cols], osem.at[blk if sem is None else sem])

    outs = {points[-2]: [out_copy(0)], points[-1]: [out_copy(s) for s in range(1, NB - 1)],
            len(slots) - 2: [out_copy(7, pl.ds(0, D - 128))]}

    def sync(t):
        for key in waits.get(t, []):
            cp[key].wait()
        for d in outs.get(t, []):
            d.start()

    emit(Pos(0), first, {t: functools.partial(sync, t) for t in list(waits) + list(outs)})
    last = out_copy(7, pl.ds(D - 128, 128), NB)
    last.start()
    for d in [d for ds in outs.values() for d in ds] + [last]:
        d.wait()


NKF = 24


@jax.jit
def pallas_parallel_sum__ssm_conv_h3__dense_activation_gelu__prompt_kernel(A_q, A_k, A_v, A_shift_k, A_ssm_k, A_ssm_D, B_x, B_w1, B_b1, B_w2, B_b2):
    fu, fk, inv = _dft_mats()
    hbm = pl.BlockSpec(memory_space=pl.ANY)
    V = pltpu.VMEM
    out = pl.pallas_call(
        kern,
        in_specs=[hbm] * 12,
        out_specs=hbm,
        out_shape=jax.ShapeDtypeStruct((S, D), bf16),
        scratch_shapes=[
            V((S // 2, D), u32), V((S // 2, D), u32), V((S // 2, D), u32),
            V((NC, D // 2, C), u32), V((14 * 64, D), u32), V((NL, F // 2, 128), u32), V((S // 2, D), u32),
            V((NKF, C + 8, 128), f32), V((S, D), f32), V((S // 2, D), u32), V((S, D), f32),
            V((S // 2, D), u32), V((S, D), f32), V((2, TM // 2, 14 * 128), u32), V((1, TM, 128), f32),
            V((UB + NC, NL, NG + 1, UN, 8, 128), f32), V((NC, NL, NG + 1, KN, 8, 128), f32),
            V((NC, NL, NG, 8, 128), u32), V((1, NL, NG, 2, 8, 128), f32),
            V((C, 4 * C), u32), pltpu.SMEM((1,), jnp.int32), V((4, D), bf16), V((D,), bf16), V((F,), bf16), V((D,), bf16),
            pltpu.SemaphoreType.DMA((3, 8)), pltpu.SemaphoreType.DMA((2, 8)), pltpu.SemaphoreType.DMA((NC,)),
            pltpu.SemaphoreType.DMA((NB + 1,)), pltpu.SemaphoreType.DMA((6,)),
        ],
        compiler_params=pltpu.CompilerParams(vmem_limit_bytes=110 * 1024 * 1024),
    )(jnp.asarray(np.zeros((1,), np.int32)), A_q.reshape(S, D), A_k.reshape(S, D), A_v.reshape(S, D), A_shift_k.T,
      A_ssm_k, A_ssm_D, B_w1.T, B_b1, B_w2, B_b2, np.concatenate([_pack(fu), _pack(fk), np.pad(_pack(inv), ((0, C // 2), (0, 0)))], 1))
    return out.reshape(1, S, D)
```

```python
import functools
import numpy as np
import jax
import jax.numpy as jnp
from jax.experimental import pallas as pl
from jax.experimental.pallas import tpu as pltpu

S, D, F = 2048, 640, 1728
C = 128
NC = S // C
TM = 256
NB = S // TM
NL = D // 128
NG = C // 8
f32, bf16, u32 = jnp.float32, jnp.bfloat16, jnp.uint32
pk = lambda v: pltpu.bitcast(v, u32)
upk = lambda v: pltpu.bitcast(v, bf16)
RATE = int('104')
W1 = float('0.3')
W2 = (14 - 14 * W1) / 70
DENS = eval('[2.41]')
U0 = float('0.45')
F1 = int('8')
FB = int('80')
PTS = [float(v) for v in '1.45,2.1,3.05,7.05'.split(',')]
JS = int('5')
PAD = int('1')
LS = int('12')
HZ = int('0')
KQ = int('8')
IW = int('0')
MIX = int('1')
KN = int('3')
UN = int('3')
KO = int('1')
G2 = int('0')
I6 = int('2')
FL = int('1')
IB = int('150')
LAG = int('2')
KG = [int(v) for v in '0,4,8,12,14'.split(',')]
FWD = eval('[(1.6, 2.1, [0, 1], True), (2.22, 3, [2, 3, 4, 5, 6], True), (3.1, 4, [7, 8, 9, 10], True), (4, 5, [11, 12, 13], True), (5, 6, [14, 15], True)]')
GB = int('340')
UB = 0
NM = len(KG) - 1
NP = 14 + NL * NM


def _dft_mats():
    n = np.arange(C)[None, :]
    th = 2 * np.pi * (np.arange(C)[:, None] + 0.25) / C
    co, si = np.cos(th * n), np.sin(th * n)
    il = lambda a, b: np.stack([a.reshape(NG, 8, C), b.reshape(NG, 8, C)], 1).reshape(2 * C, C)
    return il(co, si), il(si - co, si + co), np.stack([co, si], 1).reshape(2 * C, C).T / C


def _pack(m):
    b = m.astype(np.float32).astype(jnp.bfloat16).view(np.uint16).astype(np.uint32)
    return b[0::2] | (b[1::2] << 16)


def kern(z_h, x_h, k_h, v_h, sk_h, ssm_h, dd_h, w1_h, b1_h, w2_h, b2_h, dft_h, o_h,
         x_v, k_v, v_v, ssm_v, w1_v, w2_v, o_v, kf, xb_v, kvb_v, ff_v, g_v, acc_v, us, ks, qs, pp,
         dft_ref, z_ref, sk_ref, dd_ref, b1_ref, b2_ref,
         sem, wsem, ssem, osem, csem):
    def after(v, mark):
        if v.dtype != f32:
            mark = pltpu.bitcast(mark, v.dtype)
        return jnp.where(keep, v, mark)

    def lanes(c):
        return pl.ds(c * 128, 128)

    x_u, k_u, v_u, o_u = (r.bitcast(u32) for r in (x_h, k_h, v_h, o_h))
    ssm_u, w1_u, w2_u = (r.bitcast(u32) for r in (ssm_h, w1_h, w2_h))
    cp = {}
    for s in range(NB):
        rr = pl.ds(s * TM // 2, TM // 2)
        cp["x", s] = pltpu.make_async_copy(x_u.at[rr], x_v.at[rr], sem.at[0, s])
        cp["k", s] = pltpu.make_async_copy(k_u.at[rr], k_v.at[rr], sem.at[1, s])
        cp["v", s] = pltpu.make_async_copy(v_u.at[rr], v_v.at[rr], sem.at[2, s])
    for a in range(NC):
        cp["s", a] = pltpu.make_async_copy(ssm_u.at[:, lanes(a)], ssm_v.at[a], ssem.at[a])
    for i in range(7):
        rr = pl.ds(i * 128, min(128, F // 2 - i * 128))
        cp["w1", i] = pltpu.make_async_copy(w1_u.at[rr], w1_v.at[rr], wsem.at[0, i])
    for c in range(NL):
        cp["w2", c] = pltpu.make_async_copy(w2_u.at[:, lanes(c)], w2_v.at[c], wsem.at[1, c])

    for i, (src, dst) in enumerate(((z_h, z_ref), (b1_h, b1_ref), (b2_h, b2_ref), (sk_h, sk_ref), (dd_h, dd_ref),
                                    (dft_h, dft_ref))):
        cp["c", i] = pltpu.make_async_copy(src, dst, csem.at[i])

    class Pos:
        def __init__(self, blk):
            static = isinstance(blk, int)
            self.half = blk * (TM // 2) if static else pl.multiple_of(blk * (TM // 2), TM // 2)
            self.full = blk * TM if static else pl.multiple_of(blk * TM, TM)
            self.chunk = 2 * blk
            self.z = z0 + 2 * blk if z0 is not None else None

    norm = {}

    def ln(p, s, h, stage, mark=None):
        r0 = s * TM + h * 16
        later = lambda v: v if mark is None else after(v.reshape(2, 8, 128), mark[None]).reshape(16, 128)
        wide = lambda v: jnp.broadcast_to(v, (16, 128))
        if stage == 0:
            xs = [x_v[pl.ds(p.half + r0 // 2, 8), lanes(c)] for c in range(NL)]
            xs = [upk(v if mark is None else after(v, mark)).astype(f32) for v in xs]
            norm[s, h] = xs, wide(jnp.sum(functools.reduce(jnp.add, xs), axis=-1, keepdims=True))
        elif stage == 1:
            xs, total = norm[s, h]
            m = later(total) * (1.0 / D)
            xc = [x - m for x in xs]
            norm[s, h] = xc, wide(jnp.sum(functools.reduce(jnp.add, [v * v for v in xc]), axis=-1, keepdims=True))
        else:
            xc, total = norm.pop((s, h))
            r = jax.lax.rsqrt(later(total) * (1.0 / D) + 1e-5)
            for c in range(NL):
                xb_v[pl.ds(p.half + r0 // 2, 8), lanes(c)] = pk((xc[c] * r).astype(bf16))

    def kload(p, a, c, mark):
        u = (a * NL + c) % NKF
        first = isinstance(p.chunk, int) and p.chunk + a == 0
        if first:
            kf[u, 0:8, :] = jnp.zeros((8, 128), f32)
        for r in range(0 if first else -8, C // 2, 8):
            k2 = upk(after(k_v[pl.ds(p.half + (a * C // 2 + r), 8), lanes(c)], mark)).astype(f32)
            if r < 0:
                kf[u, 0:8, :] = k2[8:16]
            else:
                kf[u, pl.ds(8 + 2 * r, 16), :] = k2

    def kvp(p, a, c, hf, mark):
        u = (a * NL + c) % NKF
        n = C // KQ
        r0 = hf * n
        skt = sk_ref[:, lanes(c)].astype(f32)
        w0 = after(jnp.broadcast_to(skt[0:1], (8, 128)), mark)
        ksh = (kf[u, pl.ds(8 + r0, n), :].reshape(n // 8, 8, 128) * w0[None]).reshape(n, 128)
        for t in range(1, 4):
            ksh = ksh + kf[u, pl.ds(8 + r0 - t, n), :] * skt[t:t + 1]
        rows = pl.ds(p.half + (a * C + r0) // 2, n // 2)
        kv = ksh * upk(v_v[rows, lanes(c)]).astype(f32)
        kvb_v[rows, lanes(c)] = pk(kv.astype(bf16))

    def clear(p, ref, j, c, mark):
        zero = after(jnp.zeros((8, 128), f32), mark)
        ref[j, c] = jnp.broadcast_to(zero, ref.shape[2:])

    def fwd_k(p, a, c):
        kk = jax.lax.dot_general(upk(dft_ref[:, 128:256]), upk(ssm_v[p.chunk + a, pl.ds(c * 64, 64), :]),
                                 (((1,), (1,)), ((), ())), preferred_element_type=f32).reshape(NG, 2, 8, 128)
        ks[p.z + a, c, 0:NG, KO % KN] = kk[:, 1] - kk[:, 0]
        ks[p.z + a, c, 0:NG, (KO + 1) % KN] = kk[:, 0]
        ks[p.z + a, c, 0:NG, (KO + 2) % KN] = kk[:, 1]
        return [kk[i, 1] for i in range(NG)]

    def fwd_u(p, a, c):
        kv = upk(kvb_v[pl.ds(p.half + a * C // 2, C // 2), lanes(c)])
        uu = jnp.dot(upk(dft_ref[:, 0:128]), kv, preferred_element_type=f32).reshape(NG, 2, 8, 128)
        us[p.z + (UB + a), c, 0:NG, 0] = uu[:, 0] + uu[:, 1]
        us[p.z + (UB + a), c, 0:NG, 1] = uu[:, 0]
        us[p.z + (UB + a), c, 0:NG, 2] = uu[:, 1]
        return [uu[i, 1] for i in range(NG)]

    part = {}

    def prod(p, a0, lags, c, g, t, j0, j1, mark):
        if j0 == 0:
            part[t], part["u"] = [None, None], us[p.z + (UB + a0 + 1), c, g, t]
        acc = part[t]
        for j in range(j0, j1):
            kj = ks[z0 + j, c, g, (KO + t) % KN]
            if j == j0:
                kj = after(kj, mark)
            pr = kj * part["u"]
            acc[1] = pr if acc[1] is None else acc[1] + pr
            if j < lags - 1:
                part["u"] = us[p.z + (UB + a0 - j), c, g, t]
                pr = kj * part["u"]
                acc[0] = pr if acc[0] is None else acc[0] + pr
        if t < 2 or j1 < lags:
            return
        last = (pp[z0, c, g, 0], pp[z0, c, g, 1]) if lags > 2 else None
        for o in range(2):
            hs = 0.5 * part[0][o]
            re, im = hs - part[2][o], hs + part[1][o]
            q = [re, im] if last is None else [re + last[1], im - last[0]]
            qs[p.z + (a0 + o), c, g] = pltpu.pack_elementwise(q, packed_dtype=bf16)
            last = (re, im)
        if lags < NC:
            pp[z0, c, g, 0] = last[0]
            pp[z0, c, g, 1] = last[1]

    def mm1(p, s, i, sync):
        f0 = i * 128
        fn = min(128, F - f0)
        xb = upk(xb_v[pl.ds(p.half + s * TM // 2, TM // 2), :])
        w = upk(w1_v[pl.ds(f0 // 2, 64), :])
        h = jax.lax.dot_general(xb, w, (((1,), (1,)), ((), ())), preferred_element_type=f32)
        sync()
        marks = [h[r:r + 8] for r in range(0, TM, 8)]
        h = h[:, :fn] + b1_ref[pl.ds(f0, fn)].astype(f32)[None, :]
        c0 = np.float32(np.sqrt(2 / np.pi))
        c1 = np.float32(np.sqrt(2 / np.pi) * 0.044715)
        t = jnp.tanh(h * (c0 + c1 * (h * h)))
        g_v[s % 2, :, pl.ds(f0, fn)] = pk((h + h * t).astype(bf16))
        return marks

    def mm2(p, s, c, m, sync):
        k0, k1 = KG[m] * 128, min(KG[m + 1] * 128, F)
        o = jnp.dot(upk(g_v[s % 2, :, k0:k1]), upk(w2_v[c, k0 // 2:k1 // 2, :]), preferred_element_type=f32)
        sync()
        if m > 0:
            o = o + acc_v[z0]
        if m < NM - 1:
            acc_v[z0] = o
        else:
            ff_v[pl.ds(p.full + s * TM, TM), lanes(c)] = 0.5 * o + b2_ref[lanes(c)].astype(f32)[None, :]
        return [o[r:r + 8] for r in range(0, TM, 8)]

    def inv(p, a, c):
        rr, rh = pl.ds(p.full + a * C, C), pl.ds(p.half + a * C // 2, C // 2)
        q = pltpu.bitcast(qs[p.z + a, c].reshape(C, 128), bf16)
        y = jnp.dot(upk(dft_ref[0:C // 2, 256:512]), q, preferred_element_type=f32)
        x, xn, kv = (upk(ref[rh, lanes(c)]).astype(f32) for ref in (x_v, xb_v, kvb_v))
        r = xn * (y + kv * dd_ref[lanes(c)].astype(f32)[None, :]) + x + ff_v[rr, lanes(c)]
        o_v[rh, lanes(c)] = pk(r.astype(bf16))
        return [y[i:i + 8] for i in range(0, C, 8)] if IW else []

    up = lambda s: [(mm1, s, i) for i in range(14)]
    down = lambda s: [(mm2, s, c, m) for c in range(NL) for m in range(NM)]
    tiles = lambda sl: 5 if sl[0] is mm1 else KG[sl[3] + 1] - KG[sl[3]]

    def plan(slots, head, fwds, lns, invs, prods, dens, extra=()):
        at = {sl: t for t, sl in enumerate(slots)}
        mxu, side, need, done = {}, {}, {}, {}
        for t, piece in extra:
            side.setdefault(t, []).append(piece)
        for lo, hi, chunks, with_k in fwds:
            items = [(a, c) for a in chunks for c in range(NL)]
            for i, (a, c) in enumerate(items):
                t = int((lo + (hi - lo) * i / len(items)) * NP)
                mxu.setdefault(t, []).extend([(fwd_k, a, c)] * with_k + [(fwd_u, a, c)])
                done[a, c] = t
                side.setdefault(t - LAG - 2, []).append((kload, (a, c), 30))
                for hf in range(KQ):
                    side.setdefault(t - LAG - (hf < KQ // 2), []).append((kvp, (a, c, hf), 164 // KQ))
                for key in (("k", a // 2), ("v", a // 2), ("c", 3), ("c", 4)):
                    need.setdefault(key, t - LAG - 2)
                for key in [("s", a)] * with_k + [("c", 5)]:
                    need.setdefault(key, t)
        for s, t0 in lns:
            need["x", s] = t0
            for h in range(TM // 16):
                for stage, w in enumerate((25, 32, 40)):
                    side.setdefault(t0 + h * LS // 16 + stage, []).append((ln, (s, h, stage), w))
        for s, host in invs:
            for c in range(NL):
                t = at[mm2, host, c, NM - 1] - NM * (host > s)
                mxu[t] = [(inv, 2 * s, c), (inv, 2 * s + 1, c)] + mxu.get(t, [])
        queue = [(a0, lags, c, g) for a0, lags in prods for c in range(NL) for g in range(NG)]
        credit = 0.0
        for t, sl in enumerate(slots):
            more = [it[0] for it in mxu.get(t, [])]
            busy = (GB if sl[2] < 13 else GB // 2) if sl[0] is mm1 else 32 * tiles(sl) + 32 * (sl[3] == NM - 1)
            busy += sum(IB if fn is inv else FB for fn in more) + sum(w for _, _, w in side.get(t, []))
            credit += (t < len(slots) - HZ) * max(0.0, dens * 64 * (tiles(sl) + len(more)) - busy)
            due = [(it[1], it[2]) for u in range(t, t + LAG + 1) for it in mxu.get(u, []) if it[0] is inv]
            while queue:
                a0, lags, c, g = queue[0]
                urgent = (a0, c) in due or t == len(slots) - 1 - HZ
                if done.get((a0 + 1, c), -9) >= t - FL:
                    assert not urgent
                    credit = min(credit, 0.0)
                    break
                if credit <= 0 and not urgent:
                    break
                queue.pop(0)
                n = -(-lags // JS)
                cuts = [lags * i // n for i in range(n + 1)]
                side.setdefault(t, []).extend(
                    (prod, (a0, lags, c, g, comp, j0, j1), 4 * (j1 - j0) + 12 * (comp == 2 and j1 == lags))
                    for comp in range(3) for j0, j1 in zip(cuts, cuts[1:]))
                credit -= 12 * lags + 6
        print("compile", credit)
        return dict(slots=slots, head=head, mxu=mxu, side=side, need=need)

    def emit(p, pln, syncs):
        carry = []
        for t, sl in enumerate([None] + pln["slots"], -1):
            if sl is None:
                groups = [(fwd_k(p, a, c), 1) for a in pln["head"] for c in range(NL)]
            else:
                groups = [(sl[0](p, *sl[1:], syncs.get(t, lambda: None)), tiles(sl))]
                groups += [(it[0](p, *it[1:]), 1) for it in pln["mxu"].get(t, [])]
            marks = [(v, n / len(vals)) for vals, n in groups for v in vals]
            side = carry + pln["side"].get(t, [])
            if MIX:
                lists = [[it for it in side if it[0] is prod], [it for it in side if it[0] is not prod]]
                side = [it for _, it in sorted((((i + 0.5) / len(l), it) for l in lists for i, it in enumerate(l)),
                                               key=lambda e: e[0])]
            carry = [] if marks else side
            if not marks:
                continue
            tot, span = sum(w for _, _, w in side), sum(d for _, d in marks)
            cum, pos, j = 0.0, 0.0, 0
            for fn, args, w in side:
                while j < len(marks) - 1 and pos < span * cum / tot:
                    pos += marks[j][1]
                    j += 1
                fn(p, *args, marks[j][0])
                cum += w

    slots = [(mm1, s, 2 * q + i) for q in range(7) for s in (0, 1) for i in (0, 1)] + down(0) + down(1)
    for s in range(2, NB):
        slots += up(s) + down(s)
    first = plan(slots, [], FWD, [(s, (s - 1) * NP + 15) for s in range(2, NB)],
                 [(0, 2), (1, 3), (2, 3), (3, 4), (4, 4), (5, 5), (6, 6), (7, 7)],
                 [(2 * s, 2 * s + 2) for s in range(NB)], DENS[0])

    need = first["need"]
    need.update({("w1", i): 4 * i for i in range(1, 7)})
    need.update({key: 28 for key in [("c", 2)] + [("w2", c) for c in range(NL)]})

    def even_slots(pln):
        n, out = NL * len(pln["head"]), []
        for t, sl in enumerate(pln["slots"]):
            n += tiles(sl)
            if n % 4 == 0:
                out.append(t)
            n += len(pln["mxu"].get(t, []))
        return out

    points = [3, 11, 27] + [max(t for t in even_slots(first) if t <= int(q * NP)) for q in PTS]
    waits = {}
    for key, t in need.items():
        waits.setdefault(max(q for q in points if q < t), []).append(key)
    early = [("c", 0), ("c", 1), ("x", 0), ("x", 1), ("w1", 0)]
    late = [key for key in cp if key not in need and key not in early]
    for key in early + sorted(need, key=lambda k: need[k]) + late:
        cp[key].start()
    w1_v[F // 2:14 * 64, :] = jnp.zeros((14 * 64 - F // 2, D), u32)
    z0 = None
    for s in (0, 1):
        cp["x", s].wait()
        for h in range(TM // 16):
            for stage in range(3):
                ln(Pos(0), s, h, stage)
    for key in (("w1", 0), ("c", 0), ("c", 1)):
        cp[key].wait()
    z0 = z_ref[0]
    keep = jax.lax.broadcasted_iota(jnp.int32, (8, 128), 0) >= z0

    def out_copy(blk, cols=slice(None), sem=None):
        rr = pl.ds(Pos(blk).half, TM // 2)
        return pltpu.make_async_copy(o_v.at[rr, cols], o_u.at[rr, cols], osem.at[blk if sem is None else sem])

    outs = {points[-2]: [out_copy(0)], points[-1]: [out_copy(s) for s in range(1, NB - 1)],
            len(slots) - 2: [out_copy(7, pl.ds(0, D - 128))]}

    def sync(t):
        for key in waits.get(t, []):
            cp[key].wait()
        for d in outs.get(t, []):
            d.start()

    emit(Pos(0), first, {t: functools.partial(sync, t) for t in list(waits) + list(outs)})
    last = out_copy(7, pl.ds(D - 128, 128), NB)
    last.start()
    for d in [d for ds in outs.values() for d in ds] + [last]:
        d.wait()


NKF = 24


@jax.jit
def pallas_parallel_sum__ssm_conv_h3__dense_activation_gelu__prompt_kernel(A_q, A_k, A_v, A_shift_k, A_ssm_k, A_ssm_D, B_x, B_w1, B_b1, B_w2, B_b2):
    fu, fk, inv = _dft_mats()
    hbm = pl.BlockSpec(memory_space=pl.ANY)
    V = pltpu.VMEM
    out = pl.pallas_call(
        kern,
        in_specs=[hbm] * 12,
        out_specs=hbm,
        out_shape=jax.ShapeDtypeStruct((S, D), bf16),
        scratch_shapes=[
            V((S // 2, D), u32), V((S // 2, D), u32), V((S // 2, D), u32),
            V((NC, D // 2, C), u32), V((14 * 64, D), u32), V((NL, F // 2, 128), u32), V((S // 2, D), u32),
            V((NKF, C + 8, 128), f32), V((S // 2, D), u32),
            V((S // 2, D), u32), V((S, D), f32), V((2, TM // 2, 14 * 128), u32), V((1, TM, 128), f32),
            V((UB + NC, NL, NG + 1, UN, 8, 128), f32), V((NC, NL, NG + 1, KN, 8, 128), f32),
            V((NC, NL, NG, 8, 128), u32), V((1, NL, NG, 2, 8, 128), f32),
            V((C, 4 * C), u32), pltpu.SMEM((1,), jnp.int32), V((4, D), bf16), V((D,), bf16), V((F,), bf16), V((D,), bf16),
            pltpu.SemaphoreType.DMA((3, 8)), pltpu.SemaphoreType.DMA((2, 8)), pltpu.SemaphoreType.DMA((NC,)),
            pltpu.SemaphoreType.DMA((NB + 1,)), pltpu.SemaphoreType.DMA((6,)),
        ],
        compiler_params=pltpu.CompilerParams(vmem_limit_bytes=110 * 1024 * 1024),
    )(jnp.asarray(np.zeros((1,), np.int32)), A_q.reshape(S, D), A_k.reshape(S, D), A_v.reshape(S, D), A_shift_k.T,
      A_ssm_k, A_ssm_D, B_w1.T, B_b1, B_w2, B_b2, np.concatenate([_pack(fu), _pack(fk), np.pad(_pack(inv), ((0, C // 2), (0, 0)))], 1))
    return out.reshape(1, S, D)
```

```python
import functools
import numpy as np
import jax
import jax.numpy as jnp
from jax.experimental import pallas as pl
from jax.experimental.pallas import tpu as pltpu

S, D, F = 2048, 640, 1728
C = 128
NC = S // C
TM = 256
NB = S // TM
NL = D // 128
NG = C // 8
f32, bf16, u32 = jnp.float32, jnp.bfloat16, jnp.uint32
pk = lambda v: pltpu.bitcast(v, u32)
upk = lambda v: pltpu.bitcast(v, bf16)
RATE = int('104')
W1 = float('0.3')
W2 = (14 - 14 * W1) / 70
DENS = eval('[2.41]')
U0 = float('0.45')
F1 = int('8')
FB = int('80')
PTS = [float(v) for v in '1.45,2.1,3.05,7.05'.split(',')]
JS = int('5')
PAD = int('1')
LS = int('12')
HZ = int('0')
KQ = int('8')
IW = int('0')
MIX = int('1')
KN = int('3')
UN = int('3')
KO = int('1')
G2 = int('0')
I6 = int('2')
FL = int('1')
IB = int('150')
LAG = int('2')
KG = [int(v) for v in '0,4,8,12,14'.split(',')]
FWD = eval('[(1.6, 2.1, [0, 1], True), (2.22, 3, [2, 3, 4, 5, 6], True), (3.1, 4, [7, 8, 9, 10], True), (4, 5, [11, 12, 13], True), (5, 6, [14, 15], True)]')
GB = int('340')
UB = 0
KP = 8
NM = len(KG) - 1
NP = 14 + NL * NM


def _dft_mats():
    n = np.arange(C)[None, :]
    th = 2 * np.pi * (np.arange(C)[:, None] + 0.25) / C
    co, si = np.cos(th * n), np.sin(th * n)
    il = lambda a, b: np.stack([a.reshape(NG, 8, C), b.reshape(NG, 8, C)], 1).reshape(2 * C, C)
    return il(co, si), il(si - co, si + co), np.stack([co, si], 1).reshape(2 * C, C).T / C


def _pack(m):
    b = m.astype(np.float32).astype(jnp.bfloat16).view(np.uint16).astype(np.uint32)
    return b[0::2] | (b[1::2] << 16)


def kern(z_h, x_h, k_h, v_h, sk_h, ssm_h, dd_h, w1_h, b1_h, w2_h, b2_h, dft_h, o_h,
         x_v, k_v, v_v, ssm_v, w1_v, w2_v, o_v, xb_v, kvb_v, ff_v, g_v, acc_v, us, ks, qs, pp,
         dft_ref, z_ref, sk_ref, dd_ref, b1_ref, b2_ref,
         sems):
    def after(v, mark):
        if v.dtype != f32:
            mark = pltpu.bitcast(mark, v.dtype)
        return jnp.where(keep, v, mark)

    def lanes(c):
        return pl.ds(c * 128, 128)

    x_u, k_u, v_u, o_u = (r.bitcast(u32) for r in (x_h, k_h, v_h, o_h))
    ssm_u, w1_u, w2_u = (r.bitcast(u32) for r in (ssm_h, w1_h, w2_h))
    copies = []

    def copy(src, dst):
        copies.append(pltpu.make_async_copy(src, dst, sems.at[len(copies)]))
        return copies[-1]

    def fetch_rows(src, dst, lo, hi):
        rr = pl.ds(lo, hi - lo)
        return copy(src.at[rr], dst.at[rr])

    def fetch_conv(x, kv, s):
        lo, hi = kv[0] * TM // 2, kv[1] * TM // 2
        cols = pl.ds(s[0] * C, (s[1] - s[0]) * C)
        return ([copy(k_u.at[pl.ds(lo, hi - lo), lanes(c)], k_v.at[c, pl.ds(KP + lo, hi - lo)]) for c in range(NL)]
                + [fetch_rows(v_u, v_v, lo, hi), copy(ssm_u.at[:, cols], ssm_v.at[:, cols]),
                   fetch_rows(x_u, x_v, x[0] * TM // 2, x[1] * TM // 2)])

    arrivals = [[copy(z_h, z_ref), copy(b1_h, b1_ref)],
                [fetch_rows(x_u, x_v, 0, TM // 2)], [fetch_rows(x_u, x_v, TM // 2, TM)],
                [fetch_rows(w1_u, w1_v, 0, 128)], [fetch_rows(w1_u, w1_v, 128, 384)],
                [fetch_rows(w1_u, w1_v, 384, F // 2)], [copy(b2_h, b2_ref), copy(w2_u, w2_v)],
                [copy(sk_h, sk_ref), copy(dd_h, dd_ref), copy(dft_h, dft_ref)] + fetch_conv((2, 3), (0, 1), (0, 2)),
                fetch_conv((3, 4), (1, 4), (2, 7)), fetch_conv((4, NB), (4, NB), (7, NC))]

    class Pos:
        def __init__(self, blk):
            static = isinstance(blk, int)
            self.half = blk * (TM // 2) if static else pl.multiple_of(blk * (TM // 2), TM // 2)
            self.full = blk * TM if static else pl.multiple_of(blk * TM, TM)
            self.chunk = 2 * blk
            self.z = z0 + 2 * blk if z0 is not None else None

    norm = {}

    def ln(p, s, h, stage, mark=None):
        r0 = s * TM + h * 16
        later = lambda v: v if mark is None else after(v.reshape(2, 8, 128), mark[None]).reshape(16, 128)
        wide = lambda v: jnp.broadcast_to(v, (16, 128))
        if stage == 0:
            xs = [x_v[pl.ds(p.half + r0 // 2, 8), lanes(c)] for c in range(NL)]
            xs = [upk(v if mark is None else after(v, mark)).astype(f32) for v in xs]
            norm[s, h] = xs, wide(jnp.sum(functools.reduce(jnp.add, xs), axis=-1, keepdims=True))
        elif stage == 1:
            xs, total = norm[s, h]
            m = later(total) * (1.0 / D)
            xc = [x - m for x in xs]
            norm[s, h] = xc, wide(jnp.sum(functools.reduce(jnp.add, [v * v for v in xc]), axis=-1, keepdims=True))
        else:
            xc, total = norm.pop((s, h))
            r = jax.lax.rsqrt(later(total) * (1.0 / D) + 1e-5)
            for c in range(NL):
                xb_v[pl.ds(p.half + r0 // 2, 8), lanes(c)] = pk((xc[c] * r).astype(bf16))

    def kvp(p, a, c, i, mark):
        n = C // 2 // KQ
        r0 = p.half + a * C // 2 + i * n
        even = lambda v: pltpu.unpack_elementwise(v, index=0, packed_dtype=bf16, unpacked_dtype=f32)
        odd = lambda v: pltpu.unpack_elementwise(v, index=1, packed_dtype=bf16, unpacked_dtype=f32)
        k0, k1, k2 = (k_v[c, pl.ds(r0 + (KP - d), n), :] for d in range(3))
        k0 = after(k0.reshape(n // 8, 8, 128), mark[None]).reshape(n, 128)
        w = sk_ref[:, lanes(c)].astype(f32)
        e1, o1 = even(k1), odd(k1)
        ke = even(k0) * w[0:1] + o1 * w[1:2] + e1 * w[2:3] + odd(k2) * w[3:4]
        ko = odd(k0) * w[0:1] + even(k0) * w[1:2] + o1 * w[2:3] + e1 * w[3:4]
        v = v_v[pl.ds(r0, n), lanes(c)]
        kvb_v[pl.ds(r0, n), lanes(c)] = pltpu.pack_elementwise([ke * even(v), ko * odd(v)], packed_dtype=bf16)

    def clear(p, ref, j, c, mark):
        zero = after(jnp.zeros((8, 128), f32), mark)
        ref[j, c] = jnp.broadcast_to(zero, ref.shape[2:])

    def fwd_k(p, a, c):
        kk = jax.lax.dot_general(upk(dft_ref[:, 128:256]), upk(ssm_v[pl.ds(c * 64, 64), lanes(a)]),
                                 (((1,), (1,)), ((), ())), preferred_element_type=f32).reshape(NG, 2, 8, 128)
        ks[p.z + a, c, 0:NG, KO % KN] = kk[:, 1] - kk[:, 0]
        ks[p.z + a, c, 0:NG, (KO + 1) % KN] = kk[:, 0]
        ks[p.z + a, c, 0:NG, (KO + 2) % KN] = kk[:, 1]
        return [kk[i, 1] for i in range(NG)]

    def fwd_u(p, a, c):
        kv = upk(kvb_v[pl.ds(p.half + a * C // 2, C // 2), lanes(c)])
        uu = jnp.dot(upk(dft_ref[:, 0:128]), kv, preferred_element_type=f32).reshape(NG, 2, 8, 128)
        us[p.z + (UB + a), c, 0:NG, 0] = uu[:, 0] + uu[:, 1]
        us[p.z + (UB + a), c, 0:NG, 1] = uu[:, 0]
        us[p.z + (UB + a), c, 0:NG, 2] = uu[:, 1]
        return [uu[i, 1] for i in range(NG)]

    part = {}

    def prod(p, a0, lags, c, g, t, j0, j1, mark):
        if j0 == 0:
            part[t], part["u"] = [None, None], us[p.z + (UB + a0 + 1), c, g, t]
        acc = part[t]
        for j in range(j0, j1):
            kj = ks[z0 + j, c, g, (KO + t) % KN]
            if j == j0:
                kj = after(kj, mark)
            pr = kj * part["u"]
            acc[1] = pr if acc[1] is None else acc[1] + pr
            if j < lags - 1:
                part["u"] = us[p.z + (UB + a0 - j), c, g, t]
                pr = kj * part["u"]
                acc[0] = pr if acc[0] is None else acc[0] + pr
        if t < 2 or j1 < lags:
            return
        last = (pp[z0, c, g, 0], pp[z0, c, g, 1]) if lags > 2 else None
        for o in range(2):
            hs = 0.5 * part[0][o]
            re, im = hs - part[2][o], hs + part[1][o]
            q = [re, im] if last is None else [re + last[1], im - last[0]]
            qs[p.z + (a0 + o), c, g] = pltpu.pack_elementwise(q, packed_dtype=bf16)
            last = (re, im)
        if lags < NC:
            pp[z0, c, g, 0] = last[0]
            pp[z0, c, g, 1] = last[1]

    def mm1(p, s, i, sync):
        f0 = i * 128
        fn = min(128, F - f0)
        xb = upk(xb_v[pl.ds(p.half + s * TM // 2, TM // 2), :])
        w = upk(w1_v[pl.ds(f0 // 2, 64), :])
        h = jax.lax.dot_general(xb, w, (((1,), (1,)), ((), ())), preferred_element_type=f32)
        sync()
        marks = [h[r:r + 8] for r in range(0, TM, 8)]
        h = h[:, :fn] + b1_ref[pl.ds(f0, fn)].astype(f32)[None, :]
        c0 = np.float32(np.sqrt(2 / np.pi))
        c1 = np.float32(np.sqrt(2 / np.pi) * 0.044715)
        t = jnp.tanh(h * (c0 + c1 * (h * h)))
        g_v[s % 2, :, pl.ds(f0, fn)] = pk((h + h * t).astype(bf16))
        return marks

    def mm2(p, s, c, m, sync):
        k0, k1 = KG[m] * 128, min(KG[m + 1] * 128, F)
        o = jnp.dot(upk(g_v[s % 2, :, k0:k1]), upk(w2_v[k0 // 2:k1 // 2, lanes(c)]), preferred_element_type=f32)
        sync()
        if m > 0:
            o = o + acc_v[z0]
        if m < NM - 1:
            acc_v[z0] = o
        else:
            ff_v[pl.ds(p.full + s * TM, TM), lanes(c)] = 0.5 * o + b2_ref[lanes(c)].astype(f32)[None, :]
        return [o[r:r + 8] for r in range(0, TM, 8)]

    def inv(p, a, c):
        rr, rh = pl.ds(p.full + a * C, C), pl.ds(p.half + a * C // 2, C // 2)
        q = pltpu.bitcast(qs[p.z + a, c].reshape(C, 128), bf16)
        y = jnp.dot(upk(dft_ref[0:C // 2, 256:512]), q, preferred_element_type=f32)
        x, xn, kv = (upk(ref[rh, lanes(c)]).astype(f32) for ref in (x_v, xb_v, kvb_v))
        r = xn * (y + kv * dd_ref[lanes(c)].astype(f32)[None, :]) + x + ff_v[rr, lanes(c)]
        o_v[rh, lanes(c)] = pk(r.astype(bf16))
        return [y[i:i + 8] for i in range(0, C, 8)] if IW else []

    up = lambda s: [(mm1, s, i) for i in range(14)]
    down = lambda s: [(mm2, s, c, m) for c in range(NL) for m in range(NM)]
    tiles = lambda sl: 5 if sl[0] is mm1 else KG[sl[3] + 1] - KG[sl[3]]

    def plan(slots, head, fwds, lns, invs, prods, dens, extra=()):
        at = {sl: t for t, sl in enumerate(slots)}
        mxu, side, done = {}, {}, {}
        for t, piece in extra:
            side.setdefault(t, []).append(piece)
        for lo, hi, chunks, with_k in fwds:
            items = [(a, c) for a in chunks for c in range(NL)]
            for i, (a, c) in enumerate(items):
                t = int((lo + (hi - lo) * i / len(items)) * NP)
                mxu.setdefault(t, []).extend([(fwd_k, a, c)] * with_k + [(fwd_u, a, c)])
                done[a, c] = t
                for hf in range(KQ):
                    side.setdefault(t - LAG - (hf < KQ // 2), []).append((kvp, (a, c, hf), 200 // KQ))
        for s, t0 in lns:
            for h in range(TM // 16):
                for stage, w in enumerate((25, 32, 40)):
                    side.setdefault(t0 + h * LS // 16 + stage, []).append((ln, (s, h, stage), w))
        for s, host in invs:
            for c in range(NL):
                t = at[mm2, host, c, NM - 1] - NM * (host > s)
                mxu[t] = [(inv, 2 * s, c), (inv, 2 * s + 1, c)] + mxu.get(t, [])
        queue = [(a0, lags, c, g) for a0, lags in prods for c in range(NL) for g in range(NG)]
        credit = 0.0
        for t, sl in enumerate(slots):
            more = [it[0] for it in mxu.get(t, [])]
            busy = (GB if sl[2] < 13 else GB // 2) if sl[0] is mm1 else 32 * tiles(sl) + 32 * (sl[3] == NM - 1)
            busy += sum(IB if fn is inv else FB for fn in more) + sum(w for _, _, w in side.get(t, []))
            credit += (t < len(slots) - HZ) * max(0.0, dens * 64 * (tiles(sl) + len(more)) - busy)
            due = [(it[1], it[2]) for u in range(t, t + LAG + 1) for it in mxu.get(u, []) if it[0] is inv]
            while queue:
                a0, lags, c, g = queue[0]
                urgent = (a0, c) in due or t == len(slots) - 1 - HZ
                if done.get((a0 + 1, c), -9) >= t - FL:
                    assert not urgent
                    credit = min(credit, 0.0)
                    break
                if credit <= 0 and not urgent:
                    break
                queue.pop(0)
                n = -(-lags // JS)
                cuts = [lags * i // n for i in range(n + 1)]
                side.setdefault(t, []).extend(
                    (prod, (a0, lags, c, g, comp, j0, j1), 4 * (j1 - j0) + 12 * (comp == 2 and j1 == lags))
                    for comp in range(3) for j0, j1 in zip(cuts, cuts[1:]))
                credit -= 12 * lags + 6
        print("compile", credit)
        return dict(slots=slots, head=head, mxu=mxu, side=side)

    def emit(p, pln, syncs):
        carry = []
        for t, sl in enumerate([None] + pln["slots"], -1):
            if sl is None:
                groups = [(fwd_k(p, a, c), 1) for a in pln["head"] for c in range(NL)]
            else:
                groups = [(sl[0](p, *sl[1:], syncs.get(t, lambda: None)), tiles(sl))]
                groups += [(it[0](p, *it[1:]), 1) for it in pln["mxu"].get(t, [])]
            marks = [(v, n / len(vals)) for vals, n in groups for v in vals]
            side = carry + pln["side"].get(t, [])
            if MIX:
                lists = [[it for it in side if it[0] is prod], [it for it in side if it[0] is not prod]]
                side = [it for _, it in sorted((((i + 0.5) / len(l), it) for l in lists for i, it in enumerate(l)),
                                               key=lambda e: e[0])]
            carry = [] if marks else side
            if not marks:
                continue
            tot, span = sum(w for _, _, w in side), sum(d for _, d in marks)
            cum, pos, j = 0.0, 0.0, 0
            for fn, args, w in side:
                while j < len(marks) - 1 and pos < span * cum / tot:
                    pos += marks[j][1]
                    j += 1
                fn(p, *args, marks[j][0])
                cum += w

    slots = [(mm1, s, 2 * q + i) for q in range(7) for s in (0, 1) for i in (0, 1)] + down(0) + down(1)
    for s in range(2, NB):
        slots += up(s) + down(s)
    first = plan(slots, [], FWD, [(s, (s - 1) * NP + 15) for s in range(2, NB)],
                 [(0, 2), (1, 3), (2, 3), (3, 4), (4, 4), (5, 5), (6, 6), (7, 7)],
                 [(2 * s, 2 * s + 2) for s in range(NB)], DENS[0])


    def even_slots(pln):
        n, out = NL * len(pln["head"]), []
        for t, sl in enumerate(pln["slots"]):
            n += tiles(sl)
            if n % 4 == 0:
                out.append(t)
            n += len(pln["mxu"].get(t, []))
        return out

    points = [3, 11, 27] + [max(t for t in even_slots(first) if t <= int(q * NP)) for q in PTS]
    for d in copies:
        d.start()
    k_v[:, 0:KP, :] = jnp.zeros((NL, KP, 128), u32)
    z0 = None
    for s in (0, 1):
        arrivals[1 + s][0].wait()
        for h in range(TM // 16):
            for stage in range(3):
                ln(Pos(0), s, h, stage)
    for d in arrivals[0] + arrivals[3]:
        d.wait()
    z0 = z_ref[0]
    keep = jax.lax.broadcasted_iota(jnp.int32, (8, 128), 0) >= z0

    def store(lo, hi, cols=slice(None)):
        rr = pl.ds(lo * TM // 2, (hi - lo) * TM // 2)
        return copy(o_v.at[rr, cols], o_u.at[rr, cols])

    waits = dict(zip(points, arrivals[4:]))
    outs = {points[-2]: store(0, 1), points[-1]: store(1, NB - 1), len(slots) - 2: store(NB - 1, NB, pl.ds(0, D - 128))}

    def sync(t):
        for d in waits.get(t, []):
            d.wait()
        if t in outs:
            outs[t].start()

    emit(Pos(0), first, {t: functools.partial(sync, t) for t in list(waits) + list(outs)})
    last = store(NB - 1, NB, pl.ds(D - 128, 128))
    last.start()
    for d in list(outs.values()) + [last]:
        d.wait()


@jax.jit
def pallas_parallel_sum__ssm_conv_h3__dense_activation_gelu__prompt_kernel(A_q, A_k, A_v, A_shift_k, A_ssm_k, A_ssm_D, B_x, B_w1, B_b1, B_w2, B_b2):
    fu, fk, inv = _dft_mats()
    hbm = pl.BlockSpec(memory_space=pl.ANY)
    V = pltpu.VMEM
    out = pl.pallas_call(
        kern,
        in_specs=[hbm] * 12,
        out_specs=hbm,
        out_shape=jax.ShapeDtypeStruct((S, D), bf16),
        scratch_shapes=[
            V((S // 2, D), u32), V((NL, S // 2 + 32, 128), u32), V((S // 2, D), u32),
            V((D // 2, S), u32), V((14 * 64, D), u32), V((F // 2, D), u32), V((S // 2, D), u32),
            V((S // 2, D), u32),
            V((S // 2, D), u32), V((S, D), f32), V((2, TM // 2, 14 * 128), u32), V((1, TM, 128), f32),
            V((UB + NC, NL, NG + 1, UN, 8, 128), f32), V((NC, NL, NG + 1, KN, 8, 128), f32),
            V((NC, NL, NG, 8, 128), u32), V((1, NL, NG, 2, 8, 128), f32),
            V((C, 4 * C), u32), pltpu.SMEM((1,), jnp.int32), V((4, D), bf16), V((D,), bf16), V((F,), bf16), V((D,), bf16),
            pltpu.SemaphoreType.DMA((40,)),
        ],
        compiler_params=pltpu.CompilerParams(vmem_limit_bytes=110 * 1024 * 1024),
    )(jnp.asarray(np.zeros((1,), np.int32)), A_q.reshape(S, D), A_k.reshape(S, D), A_v.reshape(S, D), A_shift_k.T,
      A_ssm_k, A_ssm_D, B_w1.T, B_b1, B_w2, B_b2, np.concatenate([_pack(fu), _pack(fk), np.pad(_pack(inv), ((0, C // 2), (0, 0)))], 1))
    return out.reshape(1, S, D)
```

```python
import functools
import numpy as np
import jax
import jax.numpy as jnp
from jax.experimental import pallas as pl
from jax.experimental.pallas import tpu as pltpu

S, D, F = 2048, 640, 1728
C = 128
NC = S // C
TM = 256
NB = S // TM
NL = D // 128
NG = C // 8
f32, bf16, u32 = jnp.float32, jnp.bfloat16, jnp.uint32
pk = lambda v: pltpu.bitcast(v, u32)
upk = lambda v: pltpu.bitcast(v, bf16)
RATE = int('104')
W1 = float('0.3')
W2 = (14 - 14 * W1) / 70
DENS = eval('[2.55, 2.44, 2.45]')
U0 = float('0.03')
F1 = int('8')
FB = int('80')
PTS = [float(v) for v in '1.5'.split(',')]
JS = int('5')
PAD = int('1')
LS = int('10')
HZ = int('0')
KQ = int('8')
IW = int('0')
MIX = int('1')
KN = int('3')
UN = int('3')
KO = int('1')
G2 = int('0')
I6 = int('2')
FL = int('1')
IB = int('150')
LAG = int('2')
KG = [int(v) for v in '0,4,8,12,14'.split(',')]
FWD = eval('[(1.6, 1.75, [0, 1], True), (1.75, 1.93, [2, 3], True), (1.98, 2.3, [4, 5], True)]')
C0 = int('3')
L1 = int('1')
L2 = int('53')
I0 = int('67')
I1 = int('77')
GC = int('3')
U1 = float('0.45')
U2 = float('0.6')
U3 = float('0.7')
U4 = float('1.4')

GB = int('340')
UB = 4
KP = 8
NM = len(KG) - 1
NP = 14 + NL * NM


def _dft_mats():
    n = np.arange(C)[None, :]
    th = 2 * np.pi * (np.arange(C)[:, None] + 0.25) / C
    co, si = np.cos(th * n), np.sin(th * n)
    il = lambda a, b: np.stack([a.reshape(NG, 8, C), b.reshape(NG, 8, C)], 1).reshape(2 * C, C)
    return il(co, si), il(si - co, si + co), np.stack([co, si], 1).reshape(2 * C, C).T / C


def _pack(m):
    b = m.astype(np.float32).astype(jnp.bfloat16).view(np.uint16).astype(np.uint32)
    return b[0::2] | (b[1::2] << 16)


def kern(z_h, x_h, k_h, v_h, sk_h, ssm_h, dd_h, w1_h, b1_h, w2_h, b2_h, dft_h, o_h,
         x_v, k_v, v_v, ssm_v, w1_v, w2_v, o_v, xb0, xb1, kvb0, kvb1, ff_v, g_v, acc_v, us, ks, qs, pp,
         dft_ref, z_ref, sk_ref, dd_ref, b1_ref, b2_ref,
         sems):
    def after(v, mark):
        if v.dtype != f32:
            mark = pltpu.bitcast(mark, v.dtype)
        return jnp.where(keep, v, mark)

    def lanes(c):
        return pl.ds(c * 128, 128)

    x_u, k_u, v_u, o_u = (r.bitcast(u32) for r in (x_h, k_h, v_h, o_h))
    ssm_u, w1_u, w2_u = (r.bitcast(u32) for r in (ssm_h, w1_h, w2_h))
    xb_v, kvb_v = (xb0, xb1), (kvb0, kvb1)
    copies = []

    def copy(src, dst):
        copies.append(pltpu.make_async_copy(src, dst, sems.at[len(copies)]))
        return copies[-1]

    def fetch_rows(src, dst, lo, hi):
        rr = pl.ds(lo, hi - lo)
        return copy(src.at[rr], dst.at[rr])

    def fetch_conv(x, kv, s):
        lo, hi = kv[0] * TM // 2, kv[1] * TM // 2
        cols = pl.ds(s[0] * C, (s[1] - s[0]) * C)
        return ([copy(k_u.at[pl.ds(lo, hi - lo), lanes(c)], k_v.at[c, pl.ds(KP + lo, hi - lo)]) for c in range(NL)]
                + [fetch_rows(v_u, v_v, lo, hi), copy(ssm_u.at[:, cols], ssm_v.at[:, cols]),
                   fetch_rows(x_u, x_v, x[0] * TM // 2, x[1] * TM // 2)])

    arrivals = [[copy(z_h, z_ref), copy(b1_h, b1_ref)],
                [fetch_rows(x_u, x_v, 0, TM // 2)], [fetch_rows(x_u, x_v, TM // 2, TM)],
                [fetch_rows(w1_u, w1_v, 0, 128)], [fetch_rows(w1_u, w1_v, 128, 384)],
                [fetch_rows(w1_u, w1_v, 384, F // 2)], [copy(b2_h, b2_ref), copy(w2_u, w2_v)],
                [copy(sk_h, sk_ref), copy(dd_h, dd_ref), copy(dft_h, dft_ref)] + fetch_conv((2, 3), (0, 3), (0, 6)),
                fetch_conv((3, 5), (3, 5), (6, 10)), fetch_conv((5, NB), (5, NB), (10, NC))]

    class Pos:
        def __init__(self, blk):
            static = isinstance(blk, int)
            self.half = blk * (TM // 2) if static else pl.multiple_of(blk * (TM // 2), TM // 2)
            self.full = blk * TM if static else pl.multiple_of(blk * TM, TM)
            self.chunk = 2 * blk
            self.z = z0 + 2 * blk if z0 is not None else None
            self.far = z0 if static else z0 + 2 * (blk - 4)

    norm = {}

    def ln(p, s, h, stage, mark=None):
        r0 = s * TM + h * 16
        later = lambda v: v if mark is None else after(v.reshape(2, 8, 128), mark[None]).reshape(16, 128)
        wide = lambda v: jnp.broadcast_to(v, (16, 128))
        if stage == 0:
            xs = [x_v[pl.ds(p.half + r0 // 2, 8), lanes(c)] for c in range(NL)]
            xs = [upk(v if mark is None else after(v, mark)).astype(f32) for v in xs]
            norm[s, h] = xs, wide(jnp.sum(functools.reduce(jnp.add, xs), axis=-1, keepdims=True))
        elif stage == 1:
            xs, total = norm[s, h]
            m = later(total) * (1.0 / D)
            xc = [x - m for x in xs]
            norm[s, h] = xc, wide(jnp.sum(functools.reduce(jnp.add, [v * v for v in xc]), axis=-1, keepdims=True))
        else:
            xc, total = norm.pop((s, h))
            r = jax.lax.rsqrt(later(total) * (1.0 / D) + 1e-5)
            for c in range(NL):
                xb_v[s % 2][pl.ds(p.half + r0 // 2, 8), lanes(c)] = pk((xc[c] * r).astype(bf16))

    def kvp(p, a, c, i, mark):
        n = C // 2 // KQ
        r0 = p.half + a * C // 2 + i * n
        even = lambda v: pltpu.unpack_elementwise(v, index=0, packed_dtype=bf16, unpacked_dtype=f32)
        odd = lambda v: pltpu.unpack_elementwise(v, index=1, packed_dtype=bf16, unpacked_dtype=f32)
        k0, k1, k2 = (k_v[c, pl.ds(r0 + (KP - d), n), :] for d in range(3))
        k0 = after(k0.reshape(n // 8, 8, 128), mark[None]).reshape(n, 128)
        w = sk_ref[:, lanes(c)].astype(f32)
        e1, o1 = even(k1), odd(k1)
        ke = even(k0) * w[0:1] + o1 * w[1:2] + e1 * w[2:3] + odd(k2) * w[3:4]
        ko = odd(k0) * w[0:1] + even(k0) * w[1:2] + o1 * w[2:3] + e1 * w[3:4]
        v = v_v[pl.ds(r0, n), lanes(c)]
        kvb_v[a // 2 % 2][pl.ds(r0, n), lanes(c)] = pltpu.pack_elementwise([ke * even(v), ko * odd(v)], packed_dtype=bf16)

    def fwd_k(p, a, c):
        kk = jax.lax.dot_general(upk(dft_ref[:, 128:256]), upk(ssm_v[pl.ds(c * 64, 64), pl.ds(p.full + a * C, C)]),
                                 (((1,), (1,)), ((), ())), preferred_element_type=f32).reshape(NG, 2, 8, 128)
        ks[p.z + a, c, 0:NG, KO % KN] = kk[:, 1] - kk[:, 0]
        ks[p.z + a, c, 0:NG, (KO + 1) % KN] = kk[:, 0]
        ks[p.z + a, c, 0:NG, (KO + 2) % KN] = kk[:, 1]
        return [kk[i, 1] for i in range(NG)]

    def fwd_u(p, a, c):
        kv = upk(kvb_v[a // 2 % 2][pl.ds(p.half + a * C // 2, C // 2), lanes(c)])
        uu = jnp.dot(upk(dft_ref[:, 0:128]), kv, preferred_element_type=f32).reshape(NG, 2, 8, 128)
        us[p.z + (UB + a), c, 0:NG, 0] = uu[:, 0] + uu[:, 1]
        us[p.z + (UB + a), c, 0:NG, 1] = uu[:, 0]
        us[p.z + (UB + a), c, 0:NG, 2] = uu[:, 1]
        return [uu[i, 1] for i in range(NG)]

    part = {}

    def prod(p, a0, lags, c, g, t, j0, j1, mark):
        if j0 == 0:
            part[t], part["u"] = [None, None], us[p.z + (UB + a0 + 1), c, g, t]
        acc = part[t]
        for j in range(j0, j1):
            kj = ks[(z0 if j < 10 else p.far) + j, c, g, (KO + t) % KN]
            if j == j0:
                kj = after(kj, mark)
            pr = kj * part["u"]
            acc[1] = pr if acc[1] is None else acc[1] + pr
            if j < lags - 1:
                part["u"] = us[p.z + (UB + a0 - j), c, g, t]
                pr = kj * part["u"]
                acc[0] = pr if acc[0] is None else acc[0] + pr
        if t < 2 or j1 < lags:
            return
        last = (pp[z0, c, g, 0], pp[z0, c, g, 1]) if lags > 2 else None
        for o in range(2):
            hs = 0.5 * part[0][o]
            re, im = hs - part[2][o], hs + part[1][o]
            q = [re, im] if last is None else [re + last[1], im - last[0]]
            qs[p.z + (a0 + o), c, g] = pltpu.pack_elementwise(q, packed_dtype=bf16)
            last = (re, im)
        if lags < NC:
            pp[z0, c, g, 0] = last[0]
            pp[z0, c, g, 1] = last[1]

    def mm1(p, s, i, sync):
        f0 = i * 128
        fn = min(128, F - f0)
        xb = upk(xb_v[s % 2][pl.ds(p.half + s * TM // 2, TM // 2), :])
        w = upk(w1_v[pl.ds(f0 // 2, 64), :])
        h = jax.lax.dot_general(xb, w, (((1,), (1,)), ((), ())), preferred_element_type=f32)
        sync()
        marks = [h[r:r + 8] for r in range(0, TM, 8)]
        h = h[:, :fn] + b1_ref[pl.ds(f0, fn)].astype(f32)[None, :]
        c0 = np.float32(np.sqrt(2 / np.pi))
        c1 = np.float32(np.sqrt(2 / np.pi) * 0.044715)
        t = jnp.tanh(h * (c0 + c1 * (h * h)))
        g_v[s % 2, :, pl.ds(f0, fn)] = pk((h + h * t).astype(bf16))
        return marks

    def mm2(p, s, c, m, sync):
        k0, k1 = KG[m] * 128, min(KG[m + 1] * 128, F)
        o = jnp.dot(upk(g_v[s % 2, :, k0:k1]), upk(w2_v[k0 // 2:k1 // 2, lanes(c)]), preferred_element_type=f32)
        sync()
        if m > 0:
            o = o + acc_v[z0]
        if m < NM - 1:
            acc_v[z0] = o
        else:
            ff_v[pl.ds(p.full + s * TM, TM), lanes(c)] = 0.5 * o + b2_ref[lanes(c)].astype(f32)[None, :]
        return [o[r:r + 8] for r in range(0, TM, 8)]

    def inv(p, a, c):
        rr, rh = pl.ds(p.full + a * C, C), pl.ds(p.half + a * C // 2, C // 2)
        q = pltpu.bitcast(qs[p.z + a, c].reshape(C, 128), bf16)
        y = jnp.dot(upk(dft_ref[0:C // 2, 256:512]), q, preferred_element_type=f32)
        x, xn, kv = (upk(ref[rh, lanes(c)]).astype(f32) for ref in (x_v, xb_v[a // 2 % 2], kvb_v[a // 2 % 2]))
        r = xn * (y + kv * dd_ref[lanes(c)].astype(f32)[None, :]) + x + ff_v[rr, lanes(c)]
        o_v[rh, lanes(c)] = pk(r.astype(bf16))
        return [y[i:i + 8] for i in range(0, C, 8)] if IW else []

    up = lambda s: [(mm1, s, i) for i in range(14)]
    down = lambda s: [(mm2, s, c, m) for c in range(NL) for m in range(NM)]
    tiles = lambda sl: 5 if sl[0] is mm1 else KG[sl[3] + 1] - KG[sl[3]]

    def plan(slots, head, fwds, lns, invs, prods, dens, extra=()):
        at = {sl: t for t, sl in enumerate(slots)}
        mxu, side, done = {}, {}, {}
        for t, piece in extra:
            side.setdefault(t, []).append(piece)
        for lo, hi, chunks, with_k in fwds:
            items = [(a, c) for a in chunks for c in range(NL)]
            if len(chunks) == 2:
                items.sort(key=lambda it: it[1])
            for i, (a, c) in enumerate(items):
                t = int((lo + (hi - lo) * i / len(items)) * NP)
                mxu.setdefault(t, []).extend([(fwd_k, a, c)] * with_k + [(fwd_u, a, c)])
                done[a, c] = t
                for hf in range(KQ):
                    side.setdefault(max(t - LAG - (hf < KQ // 2), -1), []).append((kvp, (a, c, hf), 200 // KQ))
        for s, t0, span in lns:
            for h in range(TM // 16):
                for stage, w in enumerate((25, 32, 40)):
                    side.setdefault(t0 + h * span // 16 + stage, []).append((ln, (s, h, stage), w))
        for s, t0 in invs:
            for c in range(NL):
                t = at[mm2, s, c, NM - 1] if t0 is None else t0 + c
                mxu[t] = [(inv, 2 * s, c), (inv, 2 * s + 1, c)] + mxu.get(t, [])
        queue = [(a0, lags, c, g) for a0, lags, cs in prods for c in cs for g in range(NG)]
        credit = 0.0
        for t, sl in enumerate(slots):
            more = [it[0] for it in mxu.get(t, [])]
            busy = (GB if sl[2] < 13 else GB // 2) if sl[0] is mm1 else 32 * tiles(sl) + 32 * (sl[3] == NM - 1)
            busy += sum(IB if fn is inv else FB for fn in more) + sum(w for _, _, w in side.get(t, []))
            credit += (t < len(slots) - HZ) * max(0.0, dens * 64 * (tiles(sl) + len(more)) - busy)
            due = [(it[1], it[2]) for u in range(t, t + LAG + 1) for it in mxu.get(u, []) if it[0] is inv]
            while queue:
                a0, lags, c, g = queue[0]
                urgent = (a0, c) in due or t == len(slots) - 1 - HZ
                if done.get((a0 + 1, c), -9) >= t - FL:
                    assert not urgent
                    credit = min(credit, 0.0)
                    break
                if credit <= 0 and not urgent:
                    break
                queue.pop(0)
                n = -(-lags // JS)
                cuts = [lags * i // n for i in range(n + 1)]
                side.setdefault(t, []).extend(
                    (prod, (a0, lags, c, g, comp, j0, j1), 4 * (j1 - j0) + 12 * (comp == 2 and j1 == lags))
                    for comp in range(3) for j0, j1 in zip(cuts, cuts[1:]))
                credit -= 12 * lags + 6
        print("compile", credit)
        return dict(slots=slots, head=head, mxu=mxu, side=side)

    def emit(p, pln, syncs):
        carry = []
        for t, sl in enumerate([None] + pln["slots"], -1):
            if sl is None:
                groups = [(fwd_k(p, a, c), 1) for a in pln["head"] for c in range(NL)]
            else:
                groups = [(sl[0](p, *sl[1:], syncs.get(t, lambda: None)), tiles(sl))]
                groups += [(it[0](p, *it[1:]), 1) for it in pln["mxu"].get(t, [])]
            marks = [(v, n / len(vals)) for vals, n in groups for v in vals]
            side = carry + pln["side"].get(t, [])
            if MIX:
                lists = [[it for it in side if it[0] is prod], [it for it in side if it[0] is not prod]]
                side = [it for _, it in sorted((((i + 0.5) / len(l), it) for l in lists for i, it in enumerate(l)),
                                               key=lambda e: e[0])]
            carry = [] if marks else side
            if not marks:
                continue
            tot, span = sum(w for _, _, w in side), sum(d for _, d in marks)
            cum, pos, j = 0.0, 0.0, 0
            for fn, args, w in side:
                while j < len(marks) - 1 and pos < span * cum / tot:
                    pos += marks[j][1]
                    j += 1
                fn(p, *args, marks[j][0])
                cum += w

    every, lead, rest = range(NL), range(C0), range(C0, NL)
    first = plan([(mm1, s, 2 * q + i) for q in range(7) for s in (0, 1) for i in (0, 1)] + down(0) + down(1) + up(2),
                 [], FWD, [(2, L2, 8)], [(0, I0), (1, I1)], [(0, 2, every), (2, 4, every), (4, 6, lead)], DENS[0])
    body = plan(down(0) + up(1) + down(1) + up(2), [2, 3, 4, 5], [(U0, U1, [2, 3], False), (U3, U4, [4, 5], False)],
                [(1, L1, LS), (2, NP + L1, LS)], [(0, None), (1, None)], [(0, 10, rest), (2, 12, every), (4, 14, lead)], DENS[1])
    final = plan(down(6) + up(7) + down(7), [], [(0.12, U2, [14, 15], True)], [(7, L1, LS)], [(6, None), (7, None)],
                 [(12, 14, rest), (14, 16, every)], DENS[2])


    def even_slots(pln):
        n, out = NL * len(pln["head"]), []
        for t, sl in enumerate(pln["slots"]):
            n += tiles(sl)
            if n % 4 == 0:
                out.append(t)
            n += len(pln["mxu"].get(t, []))
        return out

    points = [3, 11, 27] + [max(t for t in even_slots(first) if t <= int(q * NP)) for q in PTS]
    for d in copies:
        d.start()
    k_v[:, 0:KP, :] = jnp.zeros((NL, KP, 128), u32)

    def clear(i, carry):
        us[i // NL, i % NL] = jnp.zeros(us.shape[2:], f32)
        return carry

    jax.lax.fori_loop(0, UB * NL, clear, 0)
    z0 = None
    for s in (0, 1):
        arrivals[1 + s][0].wait()
        for h in range(TM // 16):
            for stage in range(3):
                ln(Pos(0), s, h, stage)
    for d in arrivals[0] + arrivals[3]:
        d.wait()
    z0 = z_ref[0]
    keep = jax.lax.broadcasted_iota(jnp.int32, (8, 128), 0) >= z0

    def store(lo, hi, cols=slice(None)):
        rr = pl.ds(lo * TM // 2, (hi - lo) * TM // 2)
        return copy(o_v.at[rr, cols], o_u.at[rr, cols])

    emit(Pos(0), first, {t: (lambda ds=ds: [d.wait() for d in ds]) for t, ds in zip(points, arrivals[4:])})
    outs = [store(0, 2), store(2, 4), store(4, 6), store(6, 7), store(7, NB, pl.ds(0, GC * 128)),
            store(7, NB, pl.ds(GC * 128, D - GC * 128))]

    def step(it, carry):
        for i in range(2):
            @pl.when(it == i)
            def _():
                for d in arrivals[-2 + i]:
                    d.wait()
                outs[i].start()
        emit(Pos(2 * it + 2), body, {})
        return carry

    jax.lax.fori_loop(0, 2, step, 0)
    outs[2].start()
    emit(Pos(0), final, {len(final["slots"]) - (NL - GC) * NM + 1: lambda: [d.start() for d in outs[3:5]]})
    outs[5].start()
    for d in outs:
        d.wait()


@jax.jit
def pallas_parallel_sum__ssm_conv_h3__dense_activation_gelu__prompt_kernel(A_q, A_k, A_v, A_shift_k, A_ssm_k, A_ssm_D, B_x, B_w1, B_b1, B_w2, B_b2):
    fu, fk, inv = _dft_mats()
    hbm = pl.BlockSpec(memory_space=pl.ANY)
    V = pltpu.VMEM
    out = pl.pallas_call(
        kern,
        in_specs=[hbm] * 12,
        out_specs=hbm,
        out_shape=jax.ShapeDtypeStruct((S, D), bf16),
        scratch_shapes=[
            V((S // 2, D), u32), V((NL, S // 2 + 32, 128), u32), V((S // 2, D), u32),
            V((D // 2, S), u32), V((14 * 64, D), u32), V((F // 2, D), u32), V((S // 2, D), u32),
            V((S // 2, D), u32), V((S // 2, D), u32), V((S // 2, D), u32),
            V((S // 2, D), u32), V((S, D), f32), V((2, TM // 2, 14 * 128), u32), V((1, TM, 128), f32),
            V((UB + NC, NL, NG, UN, 8, 128), f32), V((NC, NL, NG, KN, 8, 128), f32),
            V((NC, NL, NG, 8, 128), u32), V((1, NL, NG, 2, 8, 128), f32),
            V((C, 4 * C), u32), pltpu.SMEM((1,), jnp.int32), V((4, D), bf16), V((D,), bf16), V((F,), bf16), V((D,), bf16),
            pltpu.SemaphoreType.DMA((40,)),
        ],
        compiler_params=pltpu.CompilerParams(vmem_limit_bytes=110 * 1024 * 1024),
    )(jnp.asarray(np.zeros((1,), np.int32)), A_q.reshape(S, D), A_k.reshape(S, D), A_v.reshape(S, D), A_shift_k.T,
      A_ssm_k, A_ssm_D, B_w1.T, B_b1, B_w2, B_b2, np.concatenate([_pack(fu), _pack(fk), np.pad(_pack(inv), ((0, C // 2), (0, 0)))], 1))
    return out.reshape(1, S, D)
```

```python
import functools
import numpy as np
import jax
import jax.numpy as jnp
from jax.experimental import pallas as pl
from jax.experimental.pallas import tpu as pltpu

S, D, F = 2048, 640, 1728
C = 128
NC = S // C
TM = 256
NB = S // TM
NL = D // 128
NG = C // 8
f32, bf16, u32 = jnp.float32, jnp.bfloat16, jnp.uint32
pk = lambda v: pltpu.bitcast(v, u32)
upk = lambda v: pltpu.bitcast(v, bf16)
RATE = int('104')
W1 = float('0.3')
W2 = (14 - 14 * W1) / 70
DENS = eval('[2.45,2.47,2.5]')
U0 = float('0.03')
F1 = int('8')
FB = int('80')
PTS = eval('(44,54)')
JS = int('5')
PAD = int('1')
LS = int('16')
HZ = int('0')
KQ = int('8')
IW = int('0')
MIX = int('1')
KN = int('3')
UN = int('3')
KO = int('1')
G2 = int('0')
I6 = int('2')
FL = int('1')
IB = int('150')
LAG = int('2')
KG = [int(v) for v in '0,4,8,12,14'.split(',')]
FWD = eval('[(1.42,1.68,[0,1],True),(1.71,1.95,[2,3],True),(1.95,2.28,[4,5],True)]')
C0 = int('3')
L1 = int('0')
L2 = int('55')
I0 = int('65')
I1 = int('76')
GC = int('3')
U1 = float('0.55')
U2 = float('0.6')
U3 = float('0.85')
U4 = float('1.55')

GB = int('340')
UB = 4
KP = 8
NM = len(KG) - 1
NP = 14 + NL * NM


def _dft_mats():
    n = np.arange(C)[None, :]
    th = 2 * np.pi * (np.arange(C)[:, None] + 0.25) / C
    co, si = np.cos(th * n), np.sin(th * n)
    il = lambda a, b: np.stack([a.reshape(NG, 8, C), b.reshape(NG, 8, C)], 1).reshape(2 * C, C)
    return il(co, si), il(si - co, si + co), np.stack([co, si], 1).reshape(2 * C, C).T / C


def _pack(m):
    b = m.astype(np.float32).astype(jnp.bfloat16).view(np.uint16).astype(np.uint32)
    return b[0::2] | (b[1::2] << 16)


def kern(z_h, x_h, k_h, v_h, sk_h, ssm_h, dd_h, w1_h, b1_h, w2_h, b2_h, fwd_h, inv_h, o_h,
         x_v, k_v, v_v, ssm_v, w1_v, w2_v, o_v, xb0, xb1, kvb0, kvb1, ff_v, g_v, acc_v, us, ks, qs, pp,
         fwd_ref, inv_ref, z_ref, sk_ref, dd_ref, b1_ref, b2_ref,
         sems):
    def after(v, mark):
        if v.dtype != f32:
            mark = pltpu.bitcast(mark, v.dtype)
        return jnp.where(keep, v, mark)

    def lanes(c):
        return pl.ds(c * 128, 128)

    x_u, k_u, v_u, o_u = (r.bitcast(u32) for r in (x_h, k_h, v_h, o_h))
    ssm_u, w1_u, w2_u = (r.bitcast(u32) for r in (ssm_h, w1_h, w2_h))
    xb_v, kvb_v = (xb0, xb1), (kvb0, kvb1)
    copies = []

    def copy(src, dst):
        copies.append(pltpu.make_async_copy(src, dst, sems.at[len(copies)]))
        return copies[-1]

    def fetch_rows(src, dst, lo, hi):
        rr = pl.ds(lo, hi - lo)
        return copy(src.at[rr], dst.at[rr])

    def fetch_conv(x, kv, s):
        lo, hi = kv[0] * TM // 2, kv[1] * TM // 2
        cols = pl.ds(s[0] * C, (s[1] - s[0]) * C)
        return ([copy(k_u.at[pl.ds(lo, hi - lo), lanes(c)], k_v.at[c, pl.ds(KP + lo, hi - lo)]) for c in range(NL)]
                + [fetch_rows(v_u, v_v, lo, hi), copy(ssm_u.at[:, cols], ssm_v.at[:, cols])]
                + [fetch_rows(x_u, x_v, lo * TM // 2, hi * TM // 2) for lo, hi in x])

    arrivals = [[copy(z_h, z_ref), copy(b1_h, b1_ref)],
                [fetch_rows(x_u, x_v, 0, TM // 2)], [fetch_rows(x_u, x_v, TM // 2, TM)],
                [fetch_rows(w1_u, w1_v, 0, 128)]]
    awaited = {4 * q - 1: [fetch_rows(w1_u, w1_v, q * 128, min(q * 128 + 128, F // 2))] for q in range(1, 7)}
    awaited[27] = [copy(b2_h, b2_ref), copy(w2_u.at[:, 0:256], w2_v.at[:, 0:256])]
    awaited[27 + 2 * NM] = [copy(w2_u.at[:, 256:D], w2_v.at[:, 256:D])]
    awaited[PTS[0]] = [copy(sk_h, sk_ref), copy(dd_h, dd_ref), copy(fwd_h, fwd_ref), copy(inv_h, inv_ref)]
    awaited[PTS[0]] += fetch_conv([], (0, 1), (0, 2))
    awaited[PTS[1]] = fetch_conv([(2, 3)], (1, 3), (2, 6))
    arrivals += [fetch_conv([(3, 5)], (3, 5), (6, 11)), fetch_conv([(5, NB)], (5, NB), (11, NC))]

    class Pos:
        def __init__(self, blk):
            static = isinstance(blk, int)
            self.half = blk * (TM // 2) if static else pl.multiple_of(blk * (TM // 2), TM // 2)
            self.full = blk * TM if static else pl.multiple_of(blk * TM, TM)
            self.chunk = 2 * blk
            self.z = z0 + 2 * blk
            self.head = 0 if static else 1 + 5 * (blk // 2)
            self.far = z0 if static else z0 + 2 * (blk - 4)

    norm = {}

    def ln(p, s, h, stage, mark):
        r0 = s * TM + h * 16
        later = lambda v: after(v.reshape(2, 8, 128), mark[None]).reshape(16, 128)
        wide = lambda v: jnp.broadcast_to(v, (16, 128))
        if stage == 0:
            xs = [x_v[pl.ds(p.half + r0 // 2, 8), lanes(c)] for c in range(NL)]
            xs = [upk(after(v, mark)).astype(f32) for v in xs]
            norm[s, h] = xs, wide(jnp.sum(functools.reduce(jnp.add, xs), axis=-1, keepdims=True))
        elif stage == 1:
            xs, total = norm[s, h]
            m = later(total) * (1.0 / D)
            xc = [x - m for x in xs]
            norm[s, h] = xc, wide(jnp.sum(functools.reduce(jnp.add, [v * v for v in xc]), axis=-1, keepdims=True))
        else:
            xc, total = norm.pop((s, h))
            r = jax.lax.rsqrt(later(total) * (1.0 / D) + 1e-5)
            for c in range(NL):
                xb_v[s % 2][pl.ds(p.half + r0 // 2, 8), lanes(c)] = pk((xc[c] * r).astype(bf16))

    def kvp(p, a, c, i, mark):
        n = C // 2 // KQ
        r0 = p.half + a * C // 2 + i * n
        even = lambda v: pltpu.unpack_elementwise(v, index=0, packed_dtype=bf16, unpacked_dtype=f32)
        odd = lambda v: pltpu.unpack_elementwise(v, index=1, packed_dtype=bf16, unpacked_dtype=f32)
        k0, k1, k2 = (k_v[c, pl.ds(r0 + (KP - d), n), :] for d in range(3))
        k0 = after(k0.reshape(n // 8, 8, 128), mark[None]).reshape(n, 128)
        w = sk_ref[:, lanes(c)].astype(f32)
        e1, o1 = even(k1), odd(k1)
        ke = even(k0) * w[0:1] + o1 * w[1:2] + e1 * w[2:3] + odd(k2) * w[3:4]
        ko = odd(k0) * w[0:1] + even(k0) * w[1:2] + o1 * w[2:3] + e1 * w[3:4]
        v = v_v[pl.ds(r0, n), lanes(c)]
        kvb_v[a // 2 % 2][pl.ds(r0, n), lanes(c)] = pltpu.pack_elementwise([ke * even(v), ko * odd(v)], packed_dtype=bf16)

    def hold(p, mark):
        k_v[z0, pl.ds(KP + S // 2, 8), :] = pltpu.bitcast(mark, u32)

    def fwd_k(p, a, c, a0=0):
        kk = jax.lax.dot_general(upk(fwd_ref[:, 128:256]), upk(ssm_v[pl.ds(c * 64, 64), pl.ds(pl.multiple_of((a0 + a) * C, C), C)]),
                                 (((1,), (1,)), ((), ())), preferred_element_type=f32).reshape(NG, 2, 8, 128)
        ks[z0 + a0 + a, c, 0:NG, KO % KN] = kk[:, 1] - kk[:, 0]
        ks[z0 + a0 + a, c, 0:NG, (KO + 1) % KN] = kk[:, 0]
        ks[z0 + a0 + a, c, 0:NG, (KO + 2) % KN] = kk[:, 1]
        return [kk[i, 1] for i in range(NG)]

    def fwd_u(p, a, c):
        kv = upk(kvb_v[a // 2 % 2][pl.ds(p.half + a * C // 2, C // 2), lanes(c)])
        uu = jnp.dot(upk(fwd_ref[:, 0:128]), kv, preferred_element_type=f32).reshape(NG, 2, 8, 128)
        us[p.z + (UB + a), c, 0:NG, 0] = uu[:, 0] + uu[:, 1]
        us[p.z + (UB + a), c, 0:NG, 1] = uu[:, 0]
        us[p.z + (UB + a), c, 0:NG, 2] = uu[:, 1]
        return [uu[i, 1] for i in range(NG)]

    part = {}

    def prod(p, a0, lags, c, g, t, j0, j1, mark):
        if j0 == 0:
            part[t], part["u"] = [None, None], us[p.z + (UB + a0 + 1), c, g, t]
        acc = part[t]
        for j in range(j0, j1):
            kj = ks[(z0 if j < 10 else p.far) + j, c, g, (KO + t) % KN]
            if j == j0:
                kj = after(kj, mark)
            pr = kj * part["u"]
            acc[1] = pr if acc[1] is None else acc[1] + pr
            if j < lags - 1:
                part["u"] = us[p.z + (UB + a0 - j), c, g, t]
                pr = kj * part["u"]
                acc[0] = pr if acc[0] is None else acc[0] + pr
        if t < 2 or j1 < lags:
            return
        last = (pp[z0, c, g, 0], pp[z0, c, g, 1]) if lags > 2 else None
        for o in range(2):
            hs = 0.5 * part[0][o]
            re, im = hs - part[2][o], hs + part[1][o]
            q = [re, im] if last is None else [re + last[1], im - last[0]]
            qs[p.z + (a0 + o), c, g] = pltpu.pack_elementwise(q, packed_dtype=bf16)
            last = (re, im)
        if lags < NC:
            pp[z0, c, g, 0] = last[0]
            pp[z0, c, g, 1] = last[1]

    def mm1(p, s, i, sync):
        f0 = i * 128
        fn = min(128, F - f0)
        xb = upk(xb_v[s % 2][pl.ds(p.half + s * TM // 2, TM // 2), :])
        w = upk(w1_v[pl.ds(f0 // 2, 64), :])
        h = jax.lax.dot_general(xb, w, (((1,), (1,)), ((), ())), preferred_element_type=f32)
        sync()
        marks = [h[r:r + 8] for r in range(0, TM, 8)]
        h = h[:, :fn] + b1_ref[pl.ds(f0, fn)].astype(f32)[None, :]
        c0 = np.float32(np.sqrt(2 / np.pi))
        c1 = np.float32(np.sqrt(2 / np.pi) * 0.044715)
        t = jnp.tanh(h * (c0 + c1 * (h * h)))
        g_v[s % 2, :, pl.ds(f0, fn)] = pk((h + h * t).astype(bf16))
        return marks

    def mm2(p, s, c, m, sync):
        k0, k1 = KG[m] * 128, min(KG[m + 1] * 128, F)
        o = jnp.dot(upk(g_v[s % 2, :, k0:k1]), upk(w2_v[k0 // 2:k1 // 2, lanes(c)]), preferred_element_type=f32)
        sync()
        if m > 0:
            o = o + acc_v[z0]
        if m < NM - 1:
            acc_v[z0] = o
        else:
            ff_v[pl.ds(p.full + s * TM, TM), lanes(c)] = 0.5 * o + b2_ref[lanes(c)].astype(f32)[None, :]
        return [o[r:r + 8] for r in range(0, TM, 8)]

    def inv(p, a, c):
        rr, rh = pl.ds(p.full + a * C, C), pl.ds(p.half + a * C // 2, C // 2)
        q = pltpu.bitcast(qs[p.z + a, c].reshape(C, 128), bf16)
        y = jnp.dot(upk(inv_ref[...]), q, preferred_element_type=f32)
        x, xn, kv = (upk(ref[rh, lanes(c)]).astype(f32) for ref in (x_v, xb_v[a // 2 % 2], kvb_v[a // 2 % 2]))
        r = xn * (y + kv * dd_ref[lanes(c)].astype(f32)[None, :]) + x + ff_v[rr, lanes(c)]
        o_v[rh, lanes(c)] = pk(r.astype(bf16))
        return [y[i:i + 8] for i in range(0, C, 8)] if IW else []

    up = lambda s: [(mm1, s, i) for i in range(14)]
    down = lambda s: [(mm2, s, c, m) for c in range(NL) for m in range(NM)]
    tiles = lambda sl: 5 if sl[0] is mm1 else KG[sl[3] + 1] - KG[sl[3]]

    def plan(slots, head, fwds, lns, invs, prods, dens, extra=()):
        at = {sl: t for t, sl in enumerate(slots)}
        mxu, side, done = {}, {}, {}
        for t, piece in extra:
            side.setdefault(t, []).append(piece)
        for lo, hi, chunks, with_k in fwds:
            items = [(a, c) for a in chunks for c in range(NL)]
            if len(chunks) == 2:
                items.sort(key=lambda it: it[1])
            for i, (a, c) in enumerate(items):
                t = int((lo + (hi - lo) * i / len(items)) * NP)
                mxu.setdefault(t, []).extend([(fwd_k, a, c)] * with_k + [(fwd_u, a, c)])
                done[a, c] = t
                for hf in range(KQ):
                    side.setdefault(max(t - LAG - (hf < KQ // 2), -1), []).append((kvp, (a, c, hf), 200 // KQ))
        for s, t0, span in lns:
            for h in range(TM // 16):
                for stage, w in enumerate((25, 32, 40)):
                    side.setdefault(t0 + h * span // 16 + stage, []).append((ln, (s, h, stage), w))
        for s, t0 in invs:
            for c in range(NL):
                t = at[mm2, s, c, NM - 1] if t0 is None else t0 + c
                mxu[t] = [(inv, 2 * s, c), (inv, 2 * s + 1, c)] + mxu.get(t, [])
        queue = [(a0, lags, c, g) for a0, lags, cs in prods for c in cs for g in range(NG)]
        credit = 0.0
        for t, sl in enumerate(slots):
            more = [it[0] for it in mxu.get(t, [])]
            busy = (GB if sl[2] < 13 else GB // 2) if sl[0] is mm1 else 32 * tiles(sl) + 32 * (sl[3] == NM - 1)
            busy += sum(IB if fn is inv else FB for fn in more) + sum(w for _, _, w in side.get(t, []))
            credit += (t < len(slots) - HZ) * max(0.0, dens * 64 * (tiles(sl) + len(more)) - busy)
            due = [(it[1], it[2]) for u in range(t, t + LAG + 1) for it in mxu.get(u, []) if it[0] is inv]
            while queue:
                a0, lags, c, g = queue[0]
                urgent = (a0, c) in due or t == len(slots) - 1 - HZ
                if done.get((a0 + 1, c), -9) >= t - FL:
                    assert not urgent
                    credit = min(credit, 0.0)
                    break
                if credit <= 0 and not urgent:
                    break
                queue.pop(0)
                n = -(-lags // JS)
                cuts = [lags * i // n for i in range(n + 1)]
                side.setdefault(t, []).extend(
                    (prod, (a0, lags, c, g, comp, j0, j1), 4 * (j1 - j0) + 12 * (comp == 2 and j1 == lags))
                    for comp in range(3) for j0, j1 in zip(cuts, cuts[1:]))
                credit -= 12 * lags + 6
        return dict(slots=slots, head=head, mxu=mxu, side=side)

    def emit(p, pln, syncs):
        carry = []
        for t, sl in enumerate([None] + pln["slots"], -1):
            if sl is None:
                groups = [(fwd_k(p, a, c, p.head), 1) for a in pln["head"] for c in range(NL)]
            else:
                groups = [(sl[0](p, *sl[1:], syncs.get(t, lambda: None)), tiles(sl))]
                groups += [(it[0](p, *it[1:]), 1) for it in pln["mxu"].get(t, [])]
            marks = [(v, n / len(vals)) for vals, n in groups for v in vals]
            side = carry + pln["side"].get(t, [])
            if MIX:
                lists = [[it for it in side if it[0] is prod], [it for it in side if it[0] is not prod]]
                side = [it for _, it in sorted((((i + 0.5) / len(l), it) for l in lists for i, it in enumerate(l)),
                                               key=lambda e: e[0])]
            carry = [] if marks else side
            if not marks:
                continue
            tot, span = sum(w for _, _, w in side), sum(d for _, d in marks)
            cum, pos, j = 0.0, 0.0, 0
            for fn, args, w in side:
                while j < len(marks) - 1 and pos < span * cum / tot:
                    pos += marks[j][1]
                    j += 1
                fn(p, *args, marks[j][0])
                cum += w

    every, lead, rest = range(NL), range(C0), range(C0, NL)
    first = plan([(mm1, s, 2 * q + i) for q in range(7) for s in (0, 1) for i in (0, 1)] + down(0) + down(1) + up(2),
                 [], FWD, [(2, L2, 8)], [(0, I0), (1, I1)], [(0, 2, every), (2, 4, every), (4, 6, lead)], DENS[0], [(PTS[1] - 1, (hold, (), 1))])
    body = plan(down(0) + up(1) + down(1) + up(2), range(5), [(U0, U1, [2, 3], False), (U3, U4, [4, 5], False)],
                [(1, L1, LS), (2, NP + L1, LS)], [(0, None), (1, None)], [(0, 10, rest), (2, 12, every), (4, 14, lead)], DENS[1])
    final = plan(down(6) + up(7) + down(7), [], [(0.12, U2, [14, 15], False)], [(7, L1, LS)], [(6, None), (7, None)],
                 [(12, 14, rest), (14, 16, every)], DENS[2])

    for d in copies:
        d.start()
    k_v[:, 0:KP, :] = jnp.zeros((NL, KP, 128), u32)

    def clear(i, carry):
        us[i // NL, i % NL] = jnp.zeros(us.shape[2:], f32)
        return carry

    jax.lax.fori_loop(0, UB * NL, clear, 0)

    def normalize(i, carry):
        for s in range(2):
            pl.when(i == s)(arrivals[1 + s][0].wait)
        rr = pl.ds(pl.multiple_of(i * (TM // 2), TM // 2), TM // 2)
        x = upk(x_v[rr, :]).astype(f32)
        xc = x - jnp.sum(x, axis=-1, keepdims=True) * (1.0 / D)
        xn = xc * jax.lax.rsqrt(jnp.sum(xc * xc, axis=-1, keepdims=True) * (1.0 / D) + 1e-5)
        xb0[rr, :] = xb1[rr, :] = pk(xn.astype(bf16))
        return carry

    jax.lax.fori_loop(0, 2, normalize, 0)
    for d in arrivals[0] + arrivals[3]:
        d.wait()
    z0 = z_ref[0]
    keep = jax.lax.broadcasted_iota(jnp.int32, (8, 128), 0) >= z0

    def store(lo, hi, cols=slice(None)):
        rr = pl.ds(lo * TM // 2, (hi - lo) * TM // 2)
        return copy(o_v.at[rr, cols], o_u.at[rr, cols])

    emit(Pos(0), first, {t: (lambda ds=ds: [d.wait() for d in ds]) for t, ds in awaited.items()})
    outs = [store(0, 2), store(2, 4), store(4, 6), store(6, 7), store(7, NB, pl.ds(0, GC * 128)),
            store(7, NB, pl.ds(GC * 128, D - GC * 128))]

    def step(it, carry):
        for i in range(2):
            @pl.when(it == i)
            def _():
                for d in arrivals[-2 + i]:
                    d.wait()
                outs[i].start()
        emit(Pos(2 * it + 2), body, {})
        return carry

    jax.lax.fori_loop(0, 2, step, 0)
    outs[2].start()
    emit(Pos(0), final, {len(final["slots"]) - (NL - GC) * NM + 1: lambda: [d.start() for d in outs[3:5]]})
    outs[5].start()
    for d in outs:
        d.wait()


@jax.jit
def pallas_parallel_sum__ssm_conv_h3__dense_activation_gelu__prompt_kernel(A_q, A_k, A_v, A_shift_k, A_ssm_k, A_ssm_D, B_x, B_w1, B_b1, B_w2, B_b2):
    fu, fk, inv = _dft_mats()
    hbm = pl.BlockSpec(memory_space=pl.ANY)
    V = pltpu.VMEM
    out = pl.pallas_call(
        kern,
        in_specs=[hbm] * 13,
        out_specs=hbm,
        out_shape=jax.ShapeDtypeStruct((S, D), bf16),
        scratch_shapes=[
            V((S // 2, D), u32), V((NL, S // 2 + 32, 128), u32), V((S // 2, D), u32),
            V((D // 2, S), u32), V((14 * 64, D), u32), V((F // 2, D), u32), V((S // 2, D), u32),
            V((S // 2, D), u32), V((S // 2, D), u32), V((S // 2, D), u32),
            V((S // 2, D), u32), V((S, D), f32), V((2, TM // 2, 14 * 128), u32), V((1, TM, 128), f32),
            V((UB + NC, NL, NG, UN, 8, 128), f32), V((NC, NL, NG, KN, 8, 128), f32),
            V((NC, NL, NG, 8, 128), u32), V((1, NL, NG, 2, 8, 128), f32),
            V((C, 2 * C), u32), V((C // 2, 2 * C), u32), pltpu.SMEM((1,), jnp.int32), V((4, D), bf16), V((D,), bf16), V((F,), bf16), V((D,), bf16),
            pltpu.SemaphoreType.DMA((64,)),
        ],
        compiler_params=pltpu.CompilerParams(vmem_limit_bytes=110 * 1024 * 1024, flags={"XLA_TPU_RESCHEDULE_DMA_DONES": True}),
    )(jnp.asarray(np.zeros((1,), np.int32)), A_q.reshape(S, D), A_k.reshape(S, D), A_v.reshape(S, D), A_shift_k.T,
      A_ssm_k, A_ssm_D, B_w1.T, B_b1, B_w2, B_b2, np.concatenate([_pack(fu), _pack(fk)], 1), _pack(inv))
    return out.reshape(1, S, D)
```

```python
import functools

import jax
import jax.numpy as jnp
import numpy as np
from jax.experimental import pallas as pl
from jax.experimental.pallas import tpu as pltpu

S, D, F = 2048, 640, 1728
C = 128
NC = S // C
TM = 256
NB = S // TM
NL = D // 128
NF = 14
NG = C // 8
KG = (0, 4, 8, 12, NF)
NM = len(KG) - 1
NP = NF + NL * NM
UB = 4
KP = 8
LAGS = 5
KQ = 8
AHEAD = 2

f32, bf16, u32 = jnp.float32, jnp.bfloat16, jnp.uint32


def _words(v):
    return pltpu.bitcast(v, u32)


def _rows(v):
    return pltpu.bitcast(v, bf16)


def _dft_matrices():
    theta = 2 * np.pi * (np.arange(C)[:, None] + 0.25) / C * np.arange(C)[None, :]
    co, si = np.cos(theta), np.sin(theta)
    by8 = lambda a, b: np.stack([a.reshape(NG, 8, C), b.reshape(NG, 8, C)], 1).reshape(2 * C, C)

    def words(m):
        b = m.astype(np.float32).astype(jnp.bfloat16).view(np.uint16).astype(np.uint32)
        return b[0::2] | (b[1::2] << 16)

    signal = by8(co, si)
    filt = by8(si - co, si + co)
    inverse = np.stack([co, si], 1).reshape(2 * C, C).T / C
    return np.concatenate([words(signal), words(filt)], 1), words(inverse)


def _kernel(z_h, x_h, k_h, v_h, sk_h, ssm_h, dd_h, w1_h, b1_h, w2_h, b2_h, fwd_h, inv_h, o_h,
            x_v, k_v, v_v, ssm_v, w1_v, w2_v, o_v, xb0, xb1, kvb0, kvb1, ff_v, g_v, acc_v, us, ks, qs, pp,
            fwd_v, inv_v, z_v, sk_v, dd_v, b1_v, b2_v, sems):
    def lanes(c):
        return pl.ds(c * 128, 128)

    xb_v, kvb_v = (xb0, xb1), (kvb0, kvb1)

    x_u, k_u, v_u, o_u, ssm_u, w1_u, w2_u = (r.bitcast(u32) for r in (x_h, k_h, v_h, o_h, ssm_h, w1_h, w2_h))
    copies = []

    def copy(src, dst):
        copies.append(pltpu.make_async_copy(src, dst, sems.at[len(copies)]))
        return copies[-1]

    def fetch_rows(src, dst, lo, hi):
        rr = pl.ds(lo, hi - lo)
        return copy(src.at[rr], dst.at[rr])

    def fetch_conv(x, kv, s):
        lo, hi = kv[0] * TM // 2, kv[1] * TM // 2
        cols = pl.ds(s[0] * C, (s[1] - s[0]) * C)
        return ([copy(k_u.at[pl.ds(lo, hi - lo), lanes(c)], k_v.at[c, pl.ds(KP + lo, hi - lo)]) for c in range(NL)]
                + [fetch_rows(v_u, v_v, lo, hi), copy(ssm_u.at[:, cols], ssm_v.at[:, cols])]
                + ([fetch_rows(x_u, x_v, x[0] * TM // 2, x[1] * TM // 2)] if x else []))

    def store(lo, hi, cols=slice(None)):
        rr = pl.ds(lo * TM // 2, (hi - lo) * TM // 2)
        return copy(o_v.at[rr, cols], o_u.at[rr, cols])

    CONV_AT = (44, 54)
    small = [copy(z_h, z_v), copy(b1_h, b1_v)]
    first_rows = [fetch_rows(x_u, x_v, s * TM // 2, (s + 1) * TM // 2) for s in range(2)]
    first_w1 = fetch_rows(w1_u, w1_v, 0, 128)
    awaited = {4 * q - 1: [fetch_rows(w1_u, w1_v, q * 128, min(q * 128 + 128, F // 2))] for q in range(1, NF // 2)}
    awaited[2 * NF - 1] = [copy(b2_h, b2_v), copy(w2_u.at[:, 0:256], w2_v.at[:, 0:256])]
    awaited[2 * NF - 1 + 2 * NM] = [copy(w2_u.at[:, 256:D], w2_v.at[:, 256:D])]
    awaited[CONV_AT[0]] = [copy(sk_h, sk_v), copy(dd_h, dd_v), copy(fwd_h, fwd_v), copy(inv_h, inv_v)]
    awaited[CONV_AT[0]] += fetch_conv(None, (0, 1), (0, 2))
    awaited[CONV_AT[1]] = fetch_conv((2, 3), (1, 3), (2, 6))
    per_pass = [fetch_conv((3, 5), (3, 5), (6, 11)), fetch_conv((5, NB), (5, NB), (11, NC))]
    for d in copies:
        d.start()

    k_v[:, 0:KP, :] = jnp.zeros((NL, KP, 128), u32)

    def clear(i, carry):
        us[i // NL, i % NL] = jnp.zeros(us.shape[2:], f32)
        return carry

    jax.lax.fori_loop(0, UB * NL, clear, 0)
    w1_v[F // 2:NF * 64, :] = jnp.zeros((NF * 64 - F // 2, D), u32)

    def normalize(i, carry):
        for s in range(2):
            pl.when(i == s)(first_rows[s].wait)
        rr = pl.ds(pl.multiple_of(i * (TM // 2), TM // 2), TM // 2)
        x = _rows(x_v[rr, :]).astype(f32)
        xc = x - jnp.sum(x, axis=-1, keepdims=True) * (1.0 / D)
        xn = xc * jax.lax.rsqrt(jnp.sum(xc * xc, axis=-1, keepdims=True) * (1.0 / D) + 1e-5)
        xb0[rr, :] = xb1[rr, :] = _words(xn.astype(bf16))
        return carry

    jax.lax.fori_loop(0, 2, normalize, 0)
    for d in small + [first_w1]:
        d.wait()

    z0 = z_v[0]
    keep = jax.lax.broadcasted_iota(jnp.int32, (8, 128), 0) >= z0

    def after(v, mark):
        if v.dtype != f32:
            mark = pltpu.bitcast(mark, v.dtype)
        return jnp.where(keep, v, mark)

    def hold(p, mark):
        k_v[z0, pl.ds(KP + S // 2, 8), :] = pltpu.bitcast(mark, u32)

    class Pos:
        def __init__(self, blk):
            static = isinstance(blk, int)
            self.half = blk * (TM // 2) if static else pl.multiple_of(blk * (TM // 2), TM // 2)
            self.full = blk * TM if static else pl.multiple_of(blk * TM, TM)
            self.z = z0 + 2 * blk
            self.head = 0 if static else 1 + 5 * (blk // 2)
            self.far = z0 if static else z0 + 2 * (blk - 4)

    norm = {}

    def layernorm(p, s, h, stage, mark):
        r0 = s * TM + h * 16
        later = lambda v: after(v.reshape(2, 8, 128), mark[None]).reshape(16, 128)
        rowsum = lambda vs: jnp.broadcast_to(jnp.sum(functools.reduce(jnp.add, vs), axis=-1, keepdims=True), (16, 128))
        if stage == 0:
            xs = [x_v[pl.ds(p.half + r0 // 2, 8), lanes(c)] for c in range(NL)]
            xs = [_rows(after(v, mark)).astype(f32) for v in xs]
            norm[s, h] = xs, rowsum(xs)
        elif stage == 1:
            xs, total = norm[s, h]
            mean = later(total) * (1.0 / D)
            xc = [x - mean for x in xs]
            norm[s, h] = xc, rowsum([v * v for v in xc])
        else:
            xc, total = norm.pop((s, h))
            r = jax.lax.rsqrt(later(total) * (1.0 / D) + 1e-5)
            for c in range(NL):
                xb_v[s % 2][pl.ds(p.half + r0 // 2, 8), lanes(c)] = _words((xc[c] * r).astype(bf16))

    def short_conv(p, a, c, i, mark):
        n = C // 2 // KQ
        r0 = p.half + a * C // 2 + i * n
        even = lambda v: pltpu.unpack_elementwise(v, index=0, packed_dtype=bf16, unpacked_dtype=f32)
        odd = lambda v: pltpu.unpack_elementwise(v, index=1, packed_dtype=bf16, unpacked_dtype=f32)
        k0, k1, k2 = (k_v[c, pl.ds(r0 + (KP - d), n), :] for d in range(3))
        k0 = after(k0.reshape(n // 8, 8, 128), mark[None]).reshape(n, 128)
        w = sk_v[:, lanes(c)].astype(f32)
        e1, o1 = even(k1), odd(k1)
        ke = even(k0) * w[0:1] + o1 * w[1:2] + e1 * w[2:3] + odd(k2) * w[3:4]
        ko = odd(k0) * w[0:1] + even(k0) * w[1:2] + o1 * w[2:3] + e1 * w[3:4]
        v = v_v[pl.ds(r0, n), lanes(c)]
        kvb_v[a // 2 % 2][pl.ds(r0, n), lanes(c)] = pltpu.pack_elementwise(
            [ke * even(v), ko * odd(v)], packed_dtype=bf16)

    part = {}
    slot_of = lambda t: (t + 2) % 3

    def products(p, a0, lags, c, g, t, j0, j1, mark):
        if j0 == 0:
            part[t], part["u"] = [None, None], us[p.z + (UB + a0 + 1), c, g, t]
        acc = part[t]
        for j in range(j0, j1):
            kj = ks[(z0 if j < 10 else p.far) + j, c, g, slot_of(t)]
            if j == j0:
                kj = after(kj, mark)
            term = kj * part["u"]
            acc[1] = term if acc[1] is None else acc[1] + term
            if j < lags - 1:
                part["u"] = us[p.z + (UB + a0 - j), c, g, t]
                term = kj * part["u"]
                acc[0] = term if acc[0] is None else acc[0] + term
        if t < 2 or j1 < lags:
            return
        last = (pp[z0, c, g, 0], pp[z0, c, g, 1]) if lags > 2 else None
        for o in range(2):
            half = 0.5 * part[0][o]
            re, im = half - part[2][o], half + part[1][o]
            q = [re, im] if last is None else [re + last[1], im - last[0]]
            qs[p.z + (a0 + o), c, g] = pltpu.pack_elementwise(q, packed_dtype=bf16)
            last = (re, im)
        if lags < NC:
            pp[z0, c, g, 0] = last[0]
            pp[z0, c, g, 1] = last[1]

    def filter_dft(p, a, c, a0=0):
        taps = _rows(ssm_v[pl.ds(c * 64, 64), pl.ds(pl.multiple_of((a0 + a) * C, C), C)])
        kk = jax.lax.dot_general(_rows(fwd_v[:, 128:256]), taps, (((1,), (1,)), ((), ())),
                                 preferred_element_type=f32).reshape(NG, 2, 8, 128)
        ks[z0 + a0 + a, c, :, slot_of(0)] = kk[:, 1] - kk[:, 0]
        ks[z0 + a0 + a, c, :, slot_of(1)] = kk[:, 0]
        ks[z0 + a0 + a, c, :, slot_of(2)] = kk[:, 1]
        return [kk[i, 1] for i in range(NG)]

    def signal_dft(p, a, c):
        kv = _rows(kvb_v[a // 2 % 2][pl.ds(p.half + a * C // 2, C // 2), lanes(c)])
        uu = jnp.dot(_rows(fwd_v[:, 0:128]), kv, preferred_element_type=f32).reshape(NG, 2, 8, 128)
        us[p.z + (UB + a), c, :, 0] = uu[:, 0] + uu[:, 1]
        us[p.z + (UB + a), c, :, 1] = uu[:, 0]
        us[p.z + (UB + a), c, :, 2] = uu[:, 1]
        return [uu[i, 1] for i in range(NG)]

    def mlp_up(p, s, i, sync):
        f0 = i * 128
        n = min(128, F - f0)
        xn = _rows(xb_v[s % 2][pl.ds(p.half + s * TM // 2, TM // 2), :])
        h = jax.lax.dot_general(xn, _rows(w1_v[pl.ds(f0 // 2, 64), :]), (((1,), (1,)), ((), ())),
                                preferred_element_type=f32)
        sync()
        marks = [h[r:r + 8] for r in range(0, TM, 8)]
        h = h[:, :n] + b1_v[pl.ds(f0, n)].astype(f32)[None, :]
        c0 = np.float32(np.sqrt(2 / np.pi))
        c1 = np.float32(np.sqrt(2 / np.pi) * 0.044715)
        t = jnp.tanh(h * (c0 + c1 * (h * h)))
        g_v[s % 2, :, pl.ds(f0, n)] = _words((h + h * t).astype(bf16))
        return marks

    def mlp_down(p, s, c, m, sync):
        k0, k1 = KG[m] * 128, min(KG[m + 1] * 128, F)
        o = jnp.dot(_rows(g_v[s % 2, :, k0:k1]), _rows(w2_v[k0 // 2:k1 // 2, lanes(c)]), preferred_element_type=f32)
        sync()
        if m > 0:
            o = o + acc_v[z0]
        if m < NM - 1:
            acc_v[z0] = o
        else:
            ff_v[pl.ds(p.full + s * TM, TM), lanes(c)] = 0.5 * o + b2_v[lanes(c)].astype(f32)[None, :]
        return [o[r:r + 8] for r in range(0, TM, 8)]

    def finish(p, a, c):
        rr, rh = pl.ds(p.full + a * C, C), pl.ds(p.half + a * C // 2, C // 2)
        y = jnp.dot(_rows(inv_v[...]), _rows(qs[p.z + a, c].reshape(C, 128)), preferred_element_type=f32)
        x, xn, kv = (_rows(ref[rh, lanes(c)]).astype(f32) for ref in (x_v, xb_v[a // 2 % 2], kvb_v[a // 2 % 2]))
        r = xn * (y + kv * dd_v[lanes(c)].astype(f32)[None, :]) + x + ff_v[rr, lanes(c)]
        o_v[rh, lanes(c)] = _words(r.astype(bf16))
        return []

    up = lambda s: [(mlp_up, s, i) for i in range(NF)]
    down = lambda s: [(mlp_down, s, c, m) for c in range(NL) for m in range(NM)]
    tiles = lambda slot: 5 if slot[0] is mlp_up else KG[slot[3] + 1] - KG[slot[3]]

    def plan(slots, head, transforms, norms, outputs, spectra, density):
        at = {slot: t for t, slot in enumerate(slots)}
        mxu, side, done = {}, {}, {}
        for lo, hi, chunks, both in transforms:
            items = [(a, c) for c in range(NL) for a in chunks]
            for i, (a, c) in enumerate(items):
                t = int((lo + (hi - lo) * i / len(items)) * NP)
                mxu.setdefault(t, []).extend([(filter_dft, a, c)] * both + [(signal_dft, a, c)])
                done[a, c] = t
                for q in range(KQ):
                    side.setdefault(max(t - AHEAD - (q < KQ // 2), -1), []).append((short_conv, (a, c, q), 200 // KQ))
        for s, t0, span in norms:
            for h in range(TM // 16):
                for stage, cost in enumerate((25, 32, 40)):
                    side.setdefault(t0 + h * span // 16 + stage, []).append((layernorm, (s, h, stage), cost))
        for s, t0 in outputs:
            for c in range(NL):
                t = at[mlp_down, s, c, NM - 1] if t0 is None else t0 + c
                mxu[t] = [(finish, 2 * s, c), (finish, 2 * s + 1, c)] + mxu.get(t, [])
        queue = [(a0, lags, c, g) for a0, lags, cs in spectra for c in cs for g in range(NG)]
        credit = 0.0
        for t, slot in enumerate(slots):
            more = [it[0] for it in mxu.get(t, [])]
            if slot[0] is mlp_up:
                busy = 340 if slot[2] < NF - 1 else 170
            else:
                busy = 32 * tiles(slot) + 32 * (slot[3] == NM - 1)
            busy += sum(150 if fn is finish else 80 for fn in more) + sum(cost for _, _, cost in side.get(t, []))
            credit += max(0.0, density * 64 * (tiles(slot) + len(more)) - busy)
            due = [it[1:] for u in range(t, t + AHEAD + 1) for it in mxu.get(u, []) if it[0] is finish]
            while queue:
                a0, lags, c, g = queue[0]
                urgent = (a0, c) in due or t == len(slots) - 1
                if done.get((a0 + 1, c), -9) >= t - 1:
                    assert not urgent
                    credit = min(credit, 0.0)
                    break
                if credit <= 0 and not urgent:
                    break
                queue.pop(0)
                n = -(-lags // LAGS)
                cuts = [lags * i // n for i in range(n + 1)]
                side.setdefault(t, []).extend(
                    (products, (a0, lags, c, g, comp, j0, j1), 4 * (j1 - j0) + 12 * (comp == 2 and j1 == lags))
                    for comp in range(3) for j0, j1 in zip(cuts, cuts[1:]))
                credit -= 12 * lags + 6
        return slots, head, mxu, side

    def emit(p, timeline, syncs):
        slots, head, mxu, side = timeline
        for t, slot in enumerate([None] + slots, -1):
            if slot is None:
                groups = [(filter_dft(p, a, c, p.head), 1) for a in head for c in range(NL)]
            else:
                groups = [(slot[0](p, *slot[1:], syncs.get(t, lambda: None)), tiles(slot))]
                groups += [(it[0](p, *it[1:]), 1) for it in mxu.get(t, [])]
            marks = [(v, n / len(vals)) for vals, n in groups for v in vals]
            work = side.get(t, [])
            total, span = sum(cost for _, _, cost in work), sum(d for _, d in marks)
            spent, pos, j = 0.0, 0.0, 0
            for fn, args, cost in work:
                while j < len(marks) - 1 and pos < span * spent / total:
                    pos += marks[j][1]
                    j += 1
                fn(p, *args, marks[j][0])
                spent += cost

    every, lead, rest = range(NL), range(3), range(3, NL)
    opening = plan([(mlp_up, s, 2 * q + i) for q in range(NF // 2) for s in (0, 1) for i in (0, 1)]
                   + down(0) + down(1) + up(2), [],
                   [(1.42, 1.68, (0, 1), True), (1.71, 1.95, (2, 3), True), (1.95, 2.28, (4, 5), True)],
                   [(2, CONV_AT[1] + 1, 8)], [(0, 65), (1, 76)], [(0, 2, every), (2, 4, every), (4, 6, lead)], 2.45)
    middle = plan(down(0) + up(1) + down(1) + up(2), range(5),
                  [(0.03, 0.55, (2, 3), False), (0.85, 1.55, (4, 5), False)],
                  [(1, 0, 16), (2, NP, 16)], [(0, None), (1, None)], [(0, 10, rest), (2, 12, every), (4, 14, lead)], 2.47)
    closing = plan(down(6) + up(7) + down(7), [], [(0.12, 0.6, (14, 15), False)],
                   [(7, 0, 16)], [(6, None), (7, None)], [(12, 14, rest), (14, 16, every)], 2.5)
    for t in CONV_AT:
        opening[3].setdefault(t - 1, []).insert(0, (hold, (), 1))

    emit(Pos(0), opening, {t: (lambda ds=ds: [d.wait() for d in ds]) for t, ds in awaited.items()})
    outs = [store(0, 2), store(2, 4), store(4, 6), store(6, 7), store(7, NB, pl.ds(0, 384)), store(7, NB, pl.ds(384, D - 384))]

    def one_pass(it, carry):
        for i in range(2):
            @pl.when(it == i)
            def _():
                for d in per_pass[i]:
                    d.wait()
                outs[i].start()
        emit(Pos(2 * it + 2), middle, {})
        return carry

    jax.lax.fori_loop(0, 2, one_pass, 0)
    outs[2].start()
    emit(Pos(0), closing, {len(closing[0]) - 2 * NM + 1: lambda: [d.start() for d in outs[3:5]]})
    outs[5].start()
    for d in outs:
        d.wait()


@jax.jit
def pallas_parallel_sum__ssm_conv_h3__dense_activation_gelu__prompt_kernel(
        A_q, A_k, A_v, A_shift_k, A_ssm_k, A_ssm_D, B_x, B_w1, B_b1, B_w2, B_b2):
    del B_x
    vmem = pltpu.VMEM
    seq = vmem((S // 2, D), u32)
    hbm = pl.BlockSpec(memory_space=pl.ANY)
    out = pl.pallas_call(
        _kernel,
        in_specs=[hbm] * 13,
        out_specs=hbm,
        out_shape=jax.ShapeDtypeStruct((S, D), bf16),
        scratch_shapes=[
            seq, vmem((NL, S // 2 + 32, 128), u32), seq,
            vmem((D // 2, S), u32), vmem((NF * 64, D), u32), vmem((F // 2, D), u32), seq,
            seq, seq, seq, seq,
            vmem((S, D), f32), vmem((2, TM // 2, NF * 128), u32), vmem((1, TM, 128), f32),
            vmem((UB + NC, NL, NG, 3, 8, 128), f32), vmem((NC, NL, NG, 3, 8, 128), f32),
            vmem((NC, NL, NG, 8, 128), u32), vmem((1, NL, NG, 2, 8, 128), f32),
            vmem((C, 2 * C), u32), vmem((C // 2, 2 * C), u32), pltpu.SMEM((1,), jnp.int32),
            vmem((4, D), bf16), vmem((D,), bf16), vmem((F,), bf16), vmem((D,), bf16),
            pltpu.SemaphoreType.DMA((64,)),
        ],
        compiler_params=pltpu.CompilerParams(
            vmem_limit_bytes=110 * 1024 * 1024, flags={"XLA_TPU_RESCHEDULE_DMA_DONES": True}),
    )(jnp.asarray(np.zeros((1,), np.int32)), A_q.reshape(S, D), A_k.reshape(S, D), A_v.reshape(S, D), A_shift_k.T,
      A_ssm_k, A_ssm_D, B_w1.T, B_b1, B_w2, B_b2, *_dft_matrices())
    return out.reshape(1, S, D)
```

```python
import functools

import jax
import jax.numpy as jnp
import numpy as np
from jax.experimental import pallas as pl
from jax.experimental.pallas import tpu as pltpu

S, D, F = 2048, 640, 1728
C = 128
NC = S // C
TM = 256
NB = S // TM
NL = D // 128
NF = 14
NG = C // 8
KG = (0, 4, 8, 12, NF)
NM = len(KG) - 1
NP = NF + NL * NM
UB = 4
KP = 8
LAGS = 5
KQ = 8
AHEAD = 2

f32, bf16, u32 = jnp.float32, jnp.bfloat16, jnp.uint32


def _words(v):
    return pltpu.bitcast(v, u32)


def _rows(v):
    return pltpu.bitcast(v, bf16)


def _dft_matrices():
    theta = 2 * np.pi * (np.arange(C)[:, None] + 0.25) / C * np.arange(C)[None, :]
    co, si = np.cos(theta), np.sin(theta)
    by8 = lambda a, b: np.stack([a.reshape(NG, 8, C), b.reshape(NG, 8, C)], 1).reshape(2 * C, C)

    def words(m):
        b = m.astype(np.float32).astype(jnp.bfloat16).view(np.uint16).astype(np.uint32)
        return b[0::2] | (b[1::2] << 16)

    signal = by8(co, si)
    filt = by8(si - co, si + co)
    inverse = np.stack([co, si], 1).reshape(2 * C, C).T / C
    return np.concatenate([words(signal), words(filt)], 1), words(inverse)


def _kernel(z_h, x_h, k_h, v_h, sk_h, ssm_h, dd_h, w1_h, b1_h, w2_h, b2_h, fwd_h, inv_h, o_h,
            x_v, k_v, v_v, ssm_v, w1_v, w2_v, o_v, xb0, xb1, kvb0, kvb1, ff_v, g_v, acc_v, us, ks, qs, pp,
            b1t_v, fwd_v, inv_v, z_v, sk_v, dd_v, b1_v, b2_v, sems):
    def lanes(c):
        return pl.ds(c * 128, 128)

    xb_v, kvb_v = (xb0, xb1), (kvb0, kvb1)

    x_u, k_u, v_u, o_u, ssm_u, w1_u, w2_u = (r.bitcast(u32) for r in (x_h, k_h, v_h, o_h, ssm_h, w1_h, w2_h))
    copies = []

    def copy(src, dst):
        copies.append(pltpu.make_async_copy(src, dst, sems.at[len(copies)]))
        return copies[-1]

    def fetch_rows(src, dst, lo, hi):
        rr = pl.ds(lo, hi - lo)
        return copy(src.at[rr], dst.at[rr])

    def fetch_conv(x, kv, s):
        lo, hi = kv[0] * TM // 2, kv[1] * TM // 2
        cols = pl.ds(s[0] * C, (s[1] - s[0]) * C)
        return ([copy(k_u.at[pl.ds(lo, hi - lo), lanes(c)], k_v.at[c, pl.ds(KP + lo, hi - lo)]) for c in range(NL)]
                + [fetch_rows(v_u, v_v, lo, hi), copy(ssm_u.at[:, cols], ssm_v.at[:, cols])]
                + ([fetch_rows(x_u, x_v, x[0] * TM // 2, x[1] * TM // 2)] if x else []))

    def store(lo, hi, cols=slice(None)):
        rr = pl.ds(lo * TM // 2, (hi - lo) * TM // 2)
        return copy(o_v.at[rr, cols], o_u.at[rr, cols])

    CONV_AT = (44, 54)
    small = [copy(z_h, z_v), copy(b1_h, b1_v)]
    first_rows = [fetch_rows(x_u, x_v, s * TM // 2, (s + 1) * TM // 2) for s in range(2)]
    first_w1 = fetch_rows(w1_u, w1_v, 0, 128)
    awaited = {4 * q - 1: [fetch_rows(w1_u, w1_v, q * 128, min(q * 128 + 128, F // 2))] for q in range(1, NF // 2)}
    awaited[2 * NF - 1] = [copy(b2_h, b2_v), copy(w2_u.at[:, 0:256], w2_v.at[:, 0:256])]
    awaited[2 * NF - 1 + 2 * NM] = [copy(w2_u.at[:, 256:D], w2_v.at[:, 256:D])]
    awaited[CONV_AT[0]] = [copy(sk_h, sk_v), copy(dd_h, dd_v), copy(fwd_h, fwd_v), copy(inv_h, inv_v)]
    awaited[CONV_AT[0]] += fetch_conv(None, (0, 1), (0, 2))
    awaited[CONV_AT[1]] = fetch_conv((2, 3), (1, 3), (2, 6))
    per_pass = [fetch_conv((3, 5), (3, 5), (6, 11)), fetch_conv((5, NB), (5, NB), (11, NC))]
    for d in copies:
        d.start()

    k_v[:, 0:KP, :] = jnp.zeros((NL, KP, 128), u32)

    def clear(i, carry):
        us[i // NL, i % NL] = jnp.zeros(us.shape[2:], f32)
        return carry

    jax.lax.fori_loop(0, UB * NL, clear, 0)

    def normalize(i, carry):
        for s in range(2):
            pl.when(i == s)(first_rows[s].wait)
        rr = pl.ds(pl.multiple_of(i * (TM // 2), TM // 2), TM // 2)
        x = _rows(x_v[rr, :]).astype(f32)
        xc = x - jnp.sum(x, axis=-1, keepdims=True) * (1.0 / D)
        xn = xc * jax.lax.rsqrt(jnp.sum(xc * xc, axis=-1, keepdims=True) * (1.0 / D) + 1e-5)
        xb0[rr, :] = xb1[rr, :] = _words(xn.astype(bf16))
        return carry

    jax.lax.fori_loop(0, 2, normalize, 0)
    for d in small + [first_w1]:
        d.wait()

    b1t_v[...] = jnp.broadcast_to(b1_v[pl.ds(F - 64, 64)].astype(f32)[None, :], (128, 64)).T

    z0 = z_v[0]
    keep = jax.lax.broadcasted_iota(jnp.int32, (8, 128), 0) >= z0

    def after(v, mark):
        if v.dtype != f32:
            mark = pltpu.bitcast(mark, v.dtype)
        return jnp.where(keep, v, mark)

    def hold(p, mark):
        k_v[z0, pl.ds(KP + S // 2, 8), :] = pltpu.bitcast(mark, u32)

    class Pos:
        def __init__(self, blk):
            static = isinstance(blk, int)
            self.half = blk * (TM // 2) if static else pl.multiple_of(blk * (TM // 2), TM // 2)
            self.full = blk * TM if static else pl.multiple_of(blk * TM, TM)
            self.z = z0 + 2 * blk
            self.head = 0 if static else 1 + 5 * (blk // 2)
            self.far = z0 if static else z0 + 2 * (blk - 4)

    norm = {}

    def layernorm(p, s, h, stage, mark):
        r0 = s * TM + h * 16
        later = lambda v: after(v.reshape(2, 8, 128), mark[None]).reshape(16, 128)
        rowsum = lambda vs: jnp.broadcast_to(jnp.sum(functools.reduce(jnp.add, vs), axis=-1, keepdims=True), (16, 128))
        if stage == 0:
            xs = [x_v[pl.ds(p.half + r0 // 2, 8), lanes(c)] for c in range(NL)]
            xs = [_rows(after(v, mark)).astype(f32) for v in xs]
            norm[s, h] = xs, rowsum(xs)
        elif stage == 1:
            xs, total = norm[s, h]
            mean = later(total) * (1.0 / D)
            xc = [x - mean for x in xs]
            norm[s, h] = xc, rowsum([v * v for v in xc])
        else:
            xc, total = norm.pop((s, h))
            r = jax.lax.rsqrt(later(total) * (1.0 / D) + 1e-5)
            for c in range(NL):
                xb_v[s % 2][pl.ds(p.half + r0 // 2, 8), lanes(c)] = _words((xc[c] * r).astype(bf16))

    def short_conv(p, a, c, i, mark):
        n = C // 2 // KQ
        r0 = p.half + a * C // 2 + i * n
        even = lambda v: pltpu.unpack_elementwise(v, index=0, packed_dtype=bf16, unpacked_dtype=f32)
        odd = lambda v: pltpu.unpack_elementwise(v, index=1, packed_dtype=bf16, unpacked_dtype=f32)
        k0, k1, k2 = (k_v[c, pl.ds(r0 + (KP - d), n), :] for d in range(3))
        k0 = after(k0.reshape(n // 8, 8, 128), mark[None]).reshape(n, 128)
        w = sk_v[:, lanes(c)].astype(f32)
        e1, o1 = even(k1), odd(k1)
        ke = even(k0) * w[0:1] + o1 * w[1:2] + e1 * w[2:3] + odd(k2) * w[3:4]
        ko = odd(k0) * w[0:1] + even(k0) * w[1:2] + o1 * w[2:3] + e1 * w[3:4]
        v = v_v[pl.ds(r0, n), lanes(c)]
        kvb_v[a // 2 % 2][pl.ds(r0, n), lanes(c)] = pltpu.pack_elementwise(
            [ke * even(v), ko * odd(v)], packed_dtype=bf16)

    part = {}
    slot_of = lambda t: (t + 2) % 3

    def products(p, a0, lags, c, g, t, j0, j1, mark):
        if j0 == 0:
            part[t], part["u"] = [None, None], us[p.z + (UB + a0 + 1), c, g, t]
        acc = part[t]
        for j in range(j0, j1):
            kj = ks[(z0 if j < 10 else p.far) + j, c, g, slot_of(t)]
            if j == j0:
                kj = after(kj, mark)
            term = kj * part["u"]
            acc[1] = term if acc[1] is None else acc[1] + term
            if j < lags - 1:
                part["u"] = us[p.z + (UB + a0 - j), c, g, t]
                term = kj * part["u"]
                acc[0] = term if acc[0] is None else acc[0] + term
        if t < 2 or j1 < lags:
            return
        last = (pp[z0, c, g, 0], pp[z0, c, g, 1]) if lags > 2 else None
        for o in range(2):
            half = 0.5 * part[0][o]
            re, im = half - part[2][o], half + part[1][o]
            q = [re, im] if last is None else [re + last[1], im - last[0]]
            qs[p.z + (a0 + o), c, g] = pltpu.pack_elementwise(q, packed_dtype=bf16)
            last = (re, im)
        if lags < NC:
            pp[z0, c, g, 0] = last[0]
            pp[z0, c, g, 1] = last[1]

    def filter_dft(p, a, c, a0=0):
        taps = _rows(ssm_v[pl.ds(c * 64, 64), pl.ds(pl.multiple_of((a0 + a) * C, C), C)])
        kk = jax.lax.dot_general(_rows(fwd_v[:, 128:256]), taps, (((1,), (1,)), ((), ())),
                                 preferred_element_type=f32).reshape(NG, 2, 8, 128)
        ks[z0 + a0 + a, c, :, slot_of(0)] = kk[:, 1] - kk[:, 0]
        ks[z0 + a0 + a, c, :, slot_of(1)] = kk[:, 0]
        ks[z0 + a0 + a, c, :, slot_of(2)] = kk[:, 1]
        return [kk[i, 1] for i in range(NG)]

    def signal_dft(p, a, c):
        kv = _rows(kvb_v[a // 2 % 2][pl.ds(p.half + a * C // 2, C // 2), lanes(c)])
        uu = jnp.dot(_rows(fwd_v[:, 0:128]), kv, preferred_element_type=f32).reshape(NG, 2, 8, 128)
        us[p.z + (UB + a), c, :, 0] = uu[:, 0] + uu[:, 1]
        us[p.z + (UB + a), c, :, 1] = uu[:, 0]
        us[p.z + (UB + a), c, :, 2] = uu[:, 1]
        return [uu[i, 1] for i in range(NG)]

    def gelu2(h):
        c0 = np.float32(np.sqrt(2 / np.pi))
        c1 = np.float32(np.sqrt(2 / np.pi) * 0.044715)
        return h + h * jnp.tanh(h * (c0 + c1 * (h * h)))

    def mlp_up(p, s, i, sync):
        f0 = i * 128
        xn = _rows(xb_v[s % 2][pl.ds(p.half + s * TM // 2, TM // 2), :])
        nt = (((1,), (1,)), ((), ()))
        if i < NF - 1:
            h = jax.lax.dot_general(xn, _rows(w1_v[pl.ds(f0 // 2, 64), :]), nt, preferred_element_type=f32)
            sync()
            g_v[s % 2, :, lanes(i)] = _words(gelu2(h + b1_v[lanes(i)].astype(f32)[None, :]).astype(bf16))
            return [h[r:r + 8] for r in range(0, TM, 8)]
        h = jax.lax.dot_general(_rows(w1_v[pl.ds(f0 // 2, (F - f0) // 2), :]), xn, nt, preferred_element_type=f32)
        sync()
        g = gelu2(h + jnp.concatenate([b1t_v[...]] * (TM // 128), 1))
        g_v[s % 2, :, pl.ds(f0, F - f0)] = _words(g.T.astype(bf16))
        return [h[r:r + 8, q:q + 128] for q in range(0, TM, 128) for r in range(0, F - f0, 8)]

    def mlp_down(p, s, c, m, sync):
        k0, k1 = KG[m] * 128, min(KG[m + 1] * 128, F)
        o = jnp.dot(_rows(g_v[s % 2, :, k0:k1]), _rows(w2_v[k0 // 2:k1 // 2, lanes(c)]), preferred_element_type=f32)
        sync()
        if m > 0:
            o = o + acc_v[z0]
        if m < NM - 1:
            acc_v[z0] = o
        else:
            ff_v[pl.ds(p.full + s * TM, TM), lanes(c)] = 0.5 * o + b2_v[lanes(c)].astype(f32)[None, :]
        return [o[r:r + 8] for r in range(0, TM, 8)]

    def finish(p, a, c):
        rr, rh = pl.ds(p.full + a * C, C), pl.ds(p.half + a * C // 2, C // 2)
        y = jnp.dot(_rows(inv_v[...]), _rows(qs[p.z + a, c].reshape(C, 128)), preferred_element_type=f32)
        x, xn, kv = (_rows(ref[rh, lanes(c)]).astype(f32) for ref in (x_v, xb_v[a // 2 % 2], kvb_v[a // 2 % 2]))
        r = xn * (y + kv * dd_v[lanes(c)].astype(f32)[None, :]) + x + ff_v[rr, lanes(c)]
        o_v[rh, lanes(c)] = _words(r.astype(bf16))
        return []

    up = lambda s: [(mlp_up, s, i % NF) for i in range(-1, NF - 1)]
    down = lambda s: [(mlp_down, s, c, m) for c in range(NL) for m in range(NM)]
    tiles = lambda slot: (5 if slot[2] < NF - 1 else 2.5) if slot[0] is mlp_up else KG[slot[3] + 1] - KG[slot[3]]

    def plan(slots, head, transforms, norms, outputs, spectra, density):
        at = {slot: t for t, slot in enumerate(slots)}
        mxu, side, done = {}, {}, {}
        for lo, hi, chunks, both in transforms:
            items = [(a, c) for c in range(NL) for a in chunks]
            for i, (a, c) in enumerate(items):
                t = int((lo + (hi - lo) * i / len(items)) * NP)
                mxu.setdefault(t, []).extend([(filter_dft, a, c)] * both + [(signal_dft, a, c)])
                done[a, c] = t
                for q in range(KQ):
                    side.setdefault(max(t - AHEAD - (q < KQ // 2), -1), []).append((short_conv, (a, c, q), 200 // KQ))
        for s, t0, span in norms:
            for h in range(TM // 16):
                for stage, cost in enumerate((25, 32, 40)):
                    side.setdefault(t0 + h * span // 16 + stage, []).append((layernorm, (s, h, stage), cost))
        for s, t0 in outputs:
            for c in range(NL):
                t = at[mlp_down, s, c, NM - 1] if t0 is None else t0 + c
                mxu[t] = [(finish, 2 * s, c), (finish, 2 * s + 1, c)] + mxu.get(t, [])
        queue = [(a0, lags, c, g) for a0, lags, cs in spectra for c in cs for g in range(NG)]
        credit = 0.0
        for t, slot in enumerate(slots):
            more = [it[0] for it in mxu.get(t, [])]
            if slot[0] is mlp_up:
                busy = 340 if slot[2] < NF - 1 else 170
            else:
                busy = 32 * tiles(slot) + 32 * (slot[3] == NM - 1)
            busy += sum(150 if fn is finish else 80 for fn in more) + sum(cost for _, _, cost in side.get(t, []))
            credit += max(0.0, density * 64 * (tiles(slot) + len(more)) - busy)
            due = [it[1:] for u in range(t, t + AHEAD + 1) for it in mxu.get(u, []) if it[0] is finish]
            while queue:
                a0, lags, c, g = queue[0]
                urgent = (a0, c) in due or t == len(slots) - 1
                if done.get((a0 + 1, c), -9) >= t - 1:
                    assert not urgent
                    credit = min(credit, 0.0)
                    break
                if credit <= 0 and not urgent:
                    break
                queue.pop(0)
                n = -(-lags // LAGS)
                cuts = [lags * i // n for i in range(n + 1)]
                side.setdefault(t, []).extend(
                    (products, (a0, lags, c, g, comp, j0, j1), 4 * (j1 - j0) + 12 * (comp == 2 and j1 == lags))
                    for comp in range(3) for j0, j1 in zip(cuts, cuts[1:]))
                credit -= 12 * lags + 6
        return slots, head, mxu, side

    def emit(p, timeline, syncs):
        slots, head, mxu, side = timeline
        for t, slot in enumerate([None] + slots, -1):
            if slot is None:
                groups = [(filter_dft(p, a, c, p.head), 1) for a in head for c in range(NL)]
            else:
                groups = [(slot[0](p, *slot[1:], syncs.get(t, lambda: None)), tiles(slot))]
                groups += [(it[0](p, *it[1:]), 1) for it in mxu.get(t, [])]
            marks = [(v, n / len(vals)) for vals, n in groups for v in vals]
            work = side.get(t, [])
            total, span = sum(cost for _, _, cost in work), sum(d for _, d in marks)
            spent, pos, j = 0.0, 0.0, 0
            for fn, args, cost in work:
                while j < len(marks) - 1 and pos < span * spent / total:
                    pos += marks[j][1]
                    j += 1
                fn(p, *args, marks[j][0])
                spent += cost

    every, lead, rest = range(NL), range(3), range(3, NL)
    opening = plan([(mlp_up, s, 2 * q + i) for q in range(NF // 2) for s in (0, 1) for i in (0, 1)]
                   + down(0) + down(1) + up(2), [],
                   [(1.42, 1.66, (0, 1), True), (1.71, 1.9, (2, 3), True), (1.9, 2.15, (4, 5), True)],
                   [(2, CONV_AT[1] + 1, 8)], [(0, 65), (1, 77)], [(0, 2, every), (2, 4, every), (4, 6, lead)], 2.48)
    middle = plan(down(0) + up(1) + down(1) + up(2), range(5),
                  [(0.03, 0.55, (2, 3), False), (0.85, 1.55, (4, 5), False)],
                  [(1, 0, 16), (2, NP, 16)], [(0, None), (1, None)], [(0, 10, rest), (2, 12, every), (4, 14, lead)], 2.51)
    closing = plan(down(6) + up(7) + down(7), [], [(0.12, 0.6, (14, 15), False)],
                   [(7, 0, 16)], [(6, None), (7, None)], [(12, 14, rest), (14, 16, every)], 2.53)
    for t in CONV_AT:
        opening[3].setdefault(t - 1, []).insert(0, (hold, (), 1))

    emit(Pos(0), opening, {t: (lambda ds=ds: [d.wait() for d in ds]) for t, ds in awaited.items()})
    outs = [store(0, 2), store(2, 4), store(4, 6), store(6, 7), store(7, NB, pl.ds(0, 384)), store(7, NB, pl.ds(384, D - 384))]

    def one_pass(it, carry):
        for i in range(2):
            @pl.when(it == i)
            def _():
                for d in per_pass[i]:
                    d.wait()
                outs[i].start()
        emit(Pos(2 * it + 2), middle, {})
        return carry

    jax.lax.fori_loop(0, 2, one_pass, 0)
    outs[2].start()
    emit(Pos(0), closing, {len(closing[0]) - 2 * NM + 1: lambda: [d.start() for d in outs[3:5]]})
    outs[5].start()
    for d in outs:
        d.wait()


@jax.jit
def pallas_parallel_sum__ssm_conv_h3__dense_activation_gelu__prompt_kernel(
        A_q, A_k, A_v, A_shift_k, A_ssm_k, A_ssm_D, B_x, B_w1, B_b1, B_w2, B_b2):
    del B_x
    vmem = pltpu.VMEM
    seq = vmem((S // 2, D), u32)
    hbm = pl.BlockSpec(memory_space=pl.ANY)
    out = pl.pallas_call(
        _kernel,
        in_specs=[hbm] * 13,
        out_specs=hbm,
        out_shape=jax.ShapeDtypeStruct((S, D), bf16),
        scratch_shapes=[
            seq, vmem((NL, S // 2 + 32, 128), u32), seq,
            vmem((D // 2, S), u32), vmem((F // 2, D), u32), vmem((F // 2, D), u32), seq,
            seq, seq, seq, seq,
            vmem((S, D), f32), vmem((2, TM // 2, NF * 128), u32), vmem((1, TM, 128), f32),
            vmem((UB + NC, NL, NG, 3, 8, 128), f32), vmem((NC, NL, NG, 3, 8, 128), f32),
            vmem((NC, NL, NG, 8, 128), u32), vmem((1, NL, NG, 2, 8, 128), f32),
            vmem((64, 128), f32), vmem((C, 2 * C), u32), vmem((C // 2, 2 * C), u32), pltpu.SMEM((1,), jnp.int32),
            vmem((4, D), bf16), vmem((D,), bf16), vmem((F,), bf16), vmem((D,), bf16),
            pltpu.SemaphoreType.DMA((64,)),
        ],
        compiler_params=pltpu.CompilerParams(
            vmem_limit_bytes=110 * 1024 * 1024, flags={"XLA_TPU_RESCHEDULE_DMA_DONES": True}),
    )(jnp.asarray(np.zeros((1,), np.int32)), A_q.reshape(S, D), A_k.reshape(S, D), A_v.reshape(S, D), A_shift_k.T,
      A_ssm_k, A_ssm_D, B_w1.T, B_b1, B_w2, B_b2, *_dft_matrices())
    return out.reshape(1, S, D)
```

```python
import functools

import jax
import jax.numpy as jnp
import numpy as np
from jax.experimental import pallas as pl
from jax.experimental.pallas import tpu as pltpu

S, D, F = 2048, 640, 1728
C = 128
NC = S // C
TM = 256
NB = S // TM
NL = D // 128
NF = 14
NG = C // 8
KG = (0, 4, 8, 12, NF)
NM = len(KG) - 1
NP = NF + NL * NM
UB = 4
KP = 8
LAGS = 5
KQ = 8
AHEAD = 2

f32, bf16, u32 = jnp.float32, jnp.bfloat16, jnp.uint32


def _words(v):
    return pltpu.bitcast(v, u32)


def _rows(v):
    return pltpu.bitcast(v, bf16)


def _dft_matrices():
    theta = 2 * np.pi * (np.arange(C)[:, None] + 0.25) / C * np.arange(C)[None, :]
    co, si = np.cos(theta), np.sin(theta)
    by8 = lambda a, b: np.stack([a.reshape(NG, 8, C), b.reshape(NG, 8, C)], 1).reshape(2 * C, C)

    def words(m):
        b = m.astype(np.float32).astype(jnp.bfloat16).view(np.uint16).astype(np.uint32)
        return b[0::2] | (b[1::2] << 16)

    signal = by8(co, si)
    filt = by8(si - co, si + co)
    inverse = np.stack([co, si], 1).reshape(2 * C, C).T / C
    return np.concatenate([words(signal), words(filt)], 1), words(inverse)


def _kernel(z_h, x_h, k_h, v_h, sk_h, ssm_h, dd_h, w1_h, b1_h, w2_h, b2_h, fwd_h, inv_h, o_h,
            x_v, k_v, v_v, ssm_v, w1_v, w2_v, o_v, xb0, xb1, kvb0, kvb1, ff_v, g_v, acc_v, us, ks, qs, pp,
            b1t_v, fwd_v, inv_v, z_v, sk_v, dd_v, b1_v, b2_v, sems):
    def lanes(c):
        return pl.ds(c * 128, 128)

    xb_v, kvb_v = (xb0, xb1), (kvb0, kvb1)

    x_u, k_u, v_u, o_u, ssm_u, w1_u, w2_u = (r.bitcast(u32) for r in (x_h, k_h, v_h, o_h, ssm_h, w1_h, w2_h))
    copies = []

    def copy(src, dst):
        copies.append(pltpu.make_async_copy(src, dst, sems.at[len(copies)]))
        return copies[-1]

    def fetch_rows(src, dst, lo, hi):
        rr = pl.ds(lo, hi - lo)
        return copy(src.at[rr], dst.at[rr])

    def fetch_conv(x, kv, s):
        lo, hi = kv[0] * TM // 2, kv[1] * TM // 2
        cols = pl.ds(s[0] * C, (s[1] - s[0]) * C)
        return ([copy(k_u.at[pl.ds(lo, hi - lo), lanes(c)], k_v.at[c, pl.ds(KP + lo, hi - lo)]) for c in range(NL)]
                + [fetch_rows(v_u, v_v, lo, hi), copy(ssm_u.at[:, cols], ssm_v.at[:, cols])]
                + ([fetch_rows(x_u, x_v, x[0] * TM // 2, x[1] * TM // 2)] if x else []))

    def store(lo, hi, cols=slice(None)):
        rr = pl.ds(lo * TM // 2, (hi - lo) * TM // 2)
        return copy(o_v.at[rr, cols], o_u.at[rr, cols])

    LEAD_IN = 6
    CONV_AT = (44 + LEAD_IN, 54 + LEAD_IN)
    small = [copy(z_h, z_v), copy(b1_h, b1_v)]
    x_piece = lambda i: fetch_rows(x_u, x_v, i * C // 2, (i + 1) * C // 2)
    w1_piece = lambda q: fetch_rows(w1_u, w1_v, q * 128, min(q * 128 + 128, F // 2))
    first = [fetch_rows(x_u, x_v, 0, TM // 2), w1_piece(0)]
    awaited = {1: [x_piece(2)], 5: [w1_piece(1)], 6: [x_piece(3)]}
    awaited.update({LEAD_IN + 4 * q - 1: [w1_piece(q)] for q in range(2, NF // 2)})
    awaited[LEAD_IN + 2 * NF - 1] = [copy(b2_h, b2_v), copy(w2_u.at[:, 0:256], w2_v.at[:, 0:256])]
    awaited[LEAD_IN + 2 * NF - 1 + 2 * NM] = [copy(w2_u.at[:, 256:D], w2_v.at[:, 256:D])]
    awaited[CONV_AT[0]] = [copy(sk_h, sk_v), copy(dd_h, dd_v), copy(fwd_h, fwd_v), copy(inv_h, inv_v)]
    awaited[CONV_AT[0]] += fetch_conv(None, (0, 1), (0, 2))
    awaited[CONV_AT[1]] = fetch_conv((2, 3), (1, 3), (2, 6))
    per_pass = [fetch_conv((3, 5), (3, 5), (6, 11)), fetch_conv((5, NB), (5, NB), (11, NC))]
    for d in copies:
        d.start()

    k_v[:, 0:KP, :] = jnp.zeros((NL, KP, 128), u32)

    def clear(i, carry):
        us[i // NL, i % NL] = jnp.zeros(us.shape[2:], f32)
        return carry

    jax.lax.fori_loop(0, UB * NL, clear, 0)

    first[0].wait()
    x = _rows(x_v[0:TM // 2, :]).astype(f32)
    xc = x - jnp.sum(x, axis=-1, keepdims=True) * (1.0 / D)
    xn = xc * jax.lax.rsqrt(jnp.sum(xc * xc, axis=-1, keepdims=True) * (1.0 / D) + 1e-5)
    xb0[0:TM // 2, :] = _words(xn.astype(bf16))
    for d in small + [first[1]]:
        d.wait()

    b1t_v[...] = jnp.broadcast_to(b1_v[pl.ds(F - 64, 64)].astype(f32)[None, :], (128, 64)).T

    z0 = z_v[0]
    keep = jax.lax.broadcasted_iota(jnp.int32, (8, 128), 0) >= z0

    def after(v, mark):
        if v.dtype != f32:
            mark = pltpu.bitcast(mark, v.dtype)
        return jnp.where(keep, v, mark)

    def hold(p, mark):
        k_v[z0, pl.ds(KP + S // 2, 8), :] = pltpu.bitcast(mark, u32)

    class Pos:
        def __init__(self, blk):
            static = isinstance(blk, int)
            self.half = blk * (TM // 2) if static else pl.multiple_of(blk * (TM // 2), TM // 2)
            self.full = blk * TM if static else pl.multiple_of(blk * TM, TM)
            self.z = z0 + 2 * blk
            self.head = 0 if static else 1 + 5 * (blk // 2)
            self.far = z0 if static else z0 + 2 * (blk - 4)

    norm = {}

    def layernorm(p, s, h, stage, mark):
        r0 = s * TM + h * 16
        later = lambda v: after(v.reshape(2, 8, 128), mark[None]).reshape(16, 128)
        rowsum = lambda vs: jnp.broadcast_to(jnp.sum(functools.reduce(jnp.add, vs), axis=-1, keepdims=True), (16, 128))
        if stage == 0:
            xs = [x_v[pl.ds(p.half + r0 // 2, 8), lanes(c)] for c in range(NL)]
            xs = [_rows(after(v, mark)).astype(f32) for v in xs]
            norm[s, h] = xs, rowsum(xs)
        elif stage == 1:
            xs, total = norm[s, h]
            mean = later(total) * (1.0 / D)
            xc = [x - mean for x in xs]
            norm[s, h] = xc, rowsum([v * v for v in xc])
        else:
            xc, total = norm.pop((s, h))
            r = jax.lax.rsqrt(later(total) * (1.0 / D) + 1e-5)
            for c in range(NL):
                xb_v[s % 2][pl.ds(p.half + r0 // 2, 8), lanes(c)] = _words((xc[c] * r).astype(bf16))

    def short_conv(p, a, c, i, mark):
        n = C // 2 // KQ
        r0 = p.half + a * C // 2 + i * n
        even = lambda v: pltpu.unpack_elementwise(v, index=0, packed_dtype=bf16, unpacked_dtype=f32)
        odd = lambda v: pltpu.unpack_elementwise(v, index=1, packed_dtype=bf16, unpacked_dtype=f32)
        k0, k1, k2 = (k_v[c, pl.ds(r0 + (KP - d), n), :] for d in range(3))
        k0 = after(k0.reshape(n // 8, 8, 128), mark[None]).reshape(n, 128)
        w = sk_v[:, lanes(c)].astype(f32)
        e1, o1 = even(k1), odd(k1)
        ke = even(k0) * w[0:1] + o1 * w[1:2] + e1 * w[2:3] + odd(k2) * w[3:4]
        ko = odd(k0) * w[0:1] + even(k0) * w[1:2] + o1 * w[2:3] + e1 * w[3:4]
        v = v_v[pl.ds(r0, n), lanes(c)]
        kvb_v[a // 2 % 2][pl.ds(r0, n), lanes(c)] = pltpu.pack_elementwise(
            [ke * even(v), ko * odd(v)], packed_dtype=bf16)

    part = {}
    slot_of = lambda t: (t + 2) % 3

    def products(p, a0, lags, c, g, t, j0, j1, mark):
        if j0 == 0:
            part[t], part["u"] = [None, None], us[p.z + (UB + a0 + 1), c, g, t]
        acc = part[t]
        for j in range(j0, j1):
            kj = ks[(z0 if j < 10 else p.far) + j, c, g, slot_of(t)]
            if j == j0:
                kj = after(kj, mark)
            term = kj * part["u"]
            acc[1] = term if acc[1] is None else acc[1] + term
            if j < lags - 1:
                part["u"] = us[p.z + (UB + a0 - j), c, g, t]
                term = kj * part["u"]
                acc[0] = term if acc[0] is None else acc[0] + term
        if t < 2 or j1 < lags:
            return
        last = (pp[z0, c, g, 0], pp[z0, c, g, 1]) if lags > 2 else None
        for o in range(2):
            half = 0.5 * part[0][o]
            re, im = half - part[2][o], half + part[1][o]
            q = [re, im] if last is None else [re + last[1], im - last[0]]
            qs[p.z + (a0 + o), c, g] = pltpu.pack_elementwise(q, packed_dtype=bf16)
            last = (re, im)
        if lags < NC:
            pp[z0, c, g, 0] = last[0]
            pp[z0, c, g, 1] = last[1]

    def filter_dft(p, a, c, a0=0):
        taps = _rows(ssm_v[pl.ds(c * 64, 64), pl.ds(pl.multiple_of((a0 + a) * C, C), C)])
        kk = jax.lax.dot_general(_rows(fwd_v[:, 128:256]), taps, (((1,), (1,)), ((), ())),
                                 preferred_element_type=f32).reshape(NG, 2, 8, 128)
        ks[z0 + a0 + a, c, :, slot_of(0)] = kk[:, 1] - kk[:, 0]
        ks[z0 + a0 + a, c, :, slot_of(1)] = kk[:, 0]
        ks[z0 + a0 + a, c, :, slot_of(2)] = kk[:, 1]
        return [kk[i, 1] for i in range(NG)]

    def signal_dft(p, a, c):
        kv = _rows(kvb_v[a // 2 % 2][pl.ds(p.half + a * C // 2, C // 2), lanes(c)])
        uu = jnp.dot(_rows(fwd_v[:, 0:128]), kv, preferred_element_type=f32).reshape(NG, 2, 8, 128)
        us[p.z + (UB + a), c, :, 0] = uu[:, 0] + uu[:, 1]
        us[p.z + (UB + a), c, :, 1] = uu[:, 0]
        us[p.z + (UB + a), c, :, 2] = uu[:, 1]
        return [uu[i, 1] for i in range(NG)]

    def gelu2(h):
        c0 = np.float32(np.sqrt(2 / np.pi))
        c1 = np.float32(np.sqrt(2 / np.pi) * 0.044715)
        return h + h * jnp.tanh(h * (c0 + c1 * (h * h)))

    def mlp_up(p, s, i, r0, n, sync):
        f0 = i * 128
        xn = _rows(xb_v[s % 2][pl.ds(p.half + (s * TM + r0) // 2, n // 2), :])
        nt = (((1,), (1,)), ((), ()))
        if i < NF - 1:
            h = jax.lax.dot_general(xn, _rows(w1_v[pl.ds(f0 // 2, 64), :]), nt, preferred_element_type=f32)
            sync()
            g_v[s % 2, pl.ds(r0 // 2, n // 2), lanes(i)] = _words(gelu2(h + b1_v[lanes(i)].astype(f32)[None, :]).astype(bf16))
            return [h[r:r + 8] for r in range(0, n, 8)]
        h = jax.lax.dot_general(_rows(w1_v[pl.ds(f0 // 2, (F - f0) // 2), :]), xn, nt, preferred_element_type=f32)
        sync()
        g = gelu2(h + jnp.concatenate([b1t_v[...]] * (TM // 128), 1))
        g_v[s % 2, :, pl.ds(f0, F - f0)] = _words(g.T.astype(bf16))
        return [h[r:r + 8, q:q + 128] for q in range(0, TM, 128) for r in range(0, F - f0, 8)]

    def mlp_down(p, s, c, m, sync):
        k0, k1 = KG[m] * 128, min(KG[m + 1] * 128, F)
        o = jnp.dot(_rows(g_v[s % 2, :, k0:k1]), _rows(w2_v[k0 // 2:k1 // 2, lanes(c)]), preferred_element_type=f32)
        sync()
        if m > 0:
            o = o + acc_v[z0]
        if m < NM - 1:
            acc_v[z0] = o
        else:
            ff_v[pl.ds(p.full + s * TM, TM), lanes(c)] = 0.5 * o + b2_v[lanes(c)].astype(f32)[None, :]
        return [o[r:r + 8] for r in range(0, TM, 8)]

    def finish(p, a, c):
        rr, rh = pl.ds(p.full + a * C, C), pl.ds(p.half + a * C // 2, C // 2)
        y = jnp.dot(_rows(inv_v[...]), _rows(qs[p.z + a, c].reshape(C, 128)), preferred_element_type=f32)
        x, xn, kv = (_rows(ref[rh, lanes(c)]).astype(f32) for ref in (x_v, xb_v[a // 2 % 2], kvb_v[a // 2 % 2]))
        r = xn * (y + kv * dd_v[lanes(c)].astype(f32)[None, :]) + x + ff_v[rr, lanes(c)]
        o_v[rh, lanes(c)] = _words(r.astype(bf16))
        return []

    up = lambda s: [(mlp_up, s, i % NF, 0, TM) for i in range(-1, NF - 1)]
    down = lambda s: [(mlp_down, s, c, m) for c in range(NL) for m in range(NM)]
    tiles = lambda slot: (5 * slot[4] / TM if slot[2] < NF - 1 else 2.5) if slot[0] is mlp_up else KG[slot[3] + 1] - KG[slot[3]]

    def plan(slots, head, transforms, norms, outputs, spectra, density):
        at = {slot: t for t, slot in enumerate(slots)}
        mxu, side, done = {}, {}, {}
        for lo, hi, chunks, both in transforms:
            items = [(a, c) for c in range(NL) for a in chunks]
            for i, (a, c) in enumerate(items):
                t = int((lo + (hi - lo) * i / len(items)) * NP)
                mxu.setdefault(t, []).extend([(filter_dft, a, c)] * both + [(signal_dft, a, c)])
                done[a, c] = t
                for q in range(KQ):
                    side.setdefault(max(t - AHEAD - (q < KQ // 2), -1), []).append((short_conv, (a, c, q), 200 // KQ))
        for s, t0, span in norms:
            for h in range(TM // 16):
                for stage, cost in enumerate((25, 32, 40)):
                    side.setdefault(t0 + h * span // 16 + stage, []).append((layernorm, (s, h, stage), cost))
        for s, t0 in outputs:
            for c in range(NL):
                t = at[mlp_down, s, c, NM - 1] if t0 is None else t0 + c
                mxu[t] = [(finish, 2 * s, c), (finish, 2 * s + 1, c)] + mxu.get(t, [])
        queue = [(a0, lags, c, g) for a0, lags, cs in spectra for c in cs for g in range(NG)]
        credit = 0.0
        for t, slot in enumerate(slots):
            more = [it[0] for it in mxu.get(t, [])]
            if slot[0] is mlp_up:
                busy = 340 if slot[2] < NF - 1 else 170
            else:
                busy = 32 * tiles(slot) + 32 * (slot[3] == NM - 1)
            busy += sum(150 if fn is finish else 80 for fn in more) + sum(cost for _, _, cost in side.get(t, []))
            credit += max(0.0, density * 64 * (tiles(slot) + len(more)) - busy)
            due = [it[1:] for u in range(t, t + AHEAD + 1) for it in mxu.get(u, []) if it[0] is finish]
            while queue:
                a0, lags, c, g = queue[0]
                urgent = (a0, c) in due or t == len(slots) - 1
                if done.get((a0 + 1, c), -9) >= t - 1:
                    assert not urgent
                    credit = min(credit, 0.0)
                    break
                if credit <= 0 and not urgent:
                    break
                queue.pop(0)
                n = -(-lags // LAGS)
                cuts = [lags * i // n for i in range(n + 1)]
                side.setdefault(t, []).extend(
                    (products, (a0, lags, c, g, comp, j0, j1), 4 * (j1 - j0) + 12 * (comp == 2 and j1 == lags))
                    for comp in range(3) for j0, j1 in zip(cuts, cuts[1:]))
                credit -= 12 * lags + 6
        return slots, head, mxu, side

    def emit(p, timeline, syncs):
        slots, head, mxu, side = timeline
        for t, slot in enumerate([None] + slots, -1):
            if slot is None:
                groups = [(filter_dft(p, a, c, p.head), 1) for a in head for c in range(NL)]
            else:
                groups = [(slot[0](p, *slot[1:], syncs.get(t, lambda: None)), tiles(slot))]
                groups += [(it[0](p, *it[1:]), 1) for it in mxu.get(t, [])]
            marks = [(v, n / len(vals)) for vals, n in groups for v in vals]
            work = side.get(t, [])
            total, span = sum(cost for _, _, cost in work), sum(d for _, d in marks)
            spent, pos, j = 0.0, 0.0, 0
            for fn, args, cost in work:
                while j < len(marks) - 1 and pos < span * spent / total:
                    pos += marks[j][1]
                    j += 1
                fn(p, *args, marks[j][0])
                spent += cost

    every, lead, rest = range(NL), range(3), range(3, NL)
    lead_in = ([(mlp_up, 0, i, r0, C) for r0 in (0, C) for i in (0, 1)] + [(mlp_up, 1, i, 0, C) for i in (0, 1)]
               + [(mlp_up, 0, i, 0, TM) for i in (2, 3)] + [(mlp_up, 1, i, 0, C) for i in (2, 3)]
               + [(mlp_up, 1, i, C, C) for i in range(4)])
    off = LEAD_IN / NP
    opening = plan(lead_in + [(mlp_up, s, 2 * q + i, 0, TM) for q in range(2, NF // 2) for s in (0, 1) for i in (0, 1)]
                   + down(0) + down(1) + up(2), [],
                   [(1.42 + off, 1.66 + off, (0, 1), True), (1.71 + off, 1.9 + off, (2, 3), True),
                    (1.9 + off, 2.15 + off, (4, 5), True)],
                   [(2, CONV_AT[1] + 1, 8)], [(0, 65 + LEAD_IN), (1, 77 + LEAD_IN)], [(0, 2, every), (2, 4, every), (4, 6, lead)], 2.48)
    middle = plan(down(0) + up(1) + down(1) + up(2), range(5),
                  [(0.03, 0.55, (2, 3), False), (0.85, 1.55, (4, 5), False)],
                  [(1, 0, 16), (2, NP, 16)], [(0, None), (1, None)], [(0, 10, rest), (2, 12, every), (4, 14, lead)], 2.51)
    closing = plan(down(6) + up(7) + down(7), [], [(0.12, 0.6, (14, 15), False)],
                   [(7, 0, 16)], [(6, None), (7, None)], [(12, 14, rest), (14, 16, every)], 2.53)
    for t in CONV_AT:
        opening[3].setdefault(t - 1, []).insert(0, (hold, (), 1))

    for h in range(TM // 16):
        for stage in range(3):
            opening[3].setdefault((1 if h < 8 else 6) + stage, []).append((layernorm, (1, h, stage), 32))
    syncs = {t: (lambda ds=ds: [d.wait() for d in ds]) for t, ds in awaited.items()}
    emit(Pos(0), opening, syncs)
    outs = [store(0, 2), store(2, 4), store(4, 6), store(6, 7), store(7, NB, pl.ds(0, 384)), store(7, NB, pl.ds(384, D - 384))]

    def one_pass(it, carry):
        for i in range(2):
            @pl.when(it == i)
            def _():
                for d in per_pass[i]:
                    d.wait()
                outs[i].start()
        emit(Pos(2 * it + 2), middle, {})
        return carry

    jax.lax.fori_loop(0, 2, one_pass, 0)
    outs[2].start()
    emit(Pos(0), closing, {len(closing[0]) - 2 * NM + 1: lambda: [d.start() for d in outs[3:5]]})
    outs[5].start()
    for d in outs:
        d.wait()


@jax.jit
def pallas_parallel_sum__ssm_conv_h3__dense_activation_gelu__prompt_kernel(
        A_q, A_k, A_v, A_shift_k, A_ssm_k, A_ssm_D, B_x, B_w1, B_b1, B_w2, B_b2):
    del B_x
    vmem = pltpu.VMEM
    seq = vmem((S // 2, D), u32)
    hbm = pl.BlockSpec(memory_space=pl.ANY)
    out = pl.pallas_call(
        _kernel,
        in_specs=[hbm] * 13,
        out_specs=hbm,
        out_shape=jax.ShapeDtypeStruct((S, D), bf16),
        scratch_shapes=[
            seq, vmem((NL, S // 2 + 32, 128), u32), seq,
            vmem((D // 2, S), u32), vmem((F // 2, D), u32), vmem((F // 2, D), u32), seq,
            seq, seq, seq, seq,
            vmem((S, D), f32), vmem((2, TM // 2, NF * 128), u32), vmem((1, TM, 128), f32),
            vmem((UB + NC, NL, NG, 3, 8, 128), f32), vmem((NC, NL, NG, 3, 8, 128), f32),
            vmem((NC, NL, NG, 8, 128), u32), vmem((1, NL, NG, 2, 8, 128), f32),
            vmem((64, 128), f32), vmem((C, 2 * C), u32), vmem((C // 2, 2 * C), u32), pltpu.SMEM((1,), jnp.int32),
            vmem((4, D), bf16), vmem((D,), bf16), vmem((F,), bf16), vmem((D,), bf16),
            pltpu.SemaphoreType.DMA((64,)),
        ],
        compiler_params=pltpu.CompilerParams(
            vmem_limit_bytes=110 * 1024 * 1024, flags={"XLA_TPU_RESCHEDULE_DMA_DONES": True}),
    )(jnp.asarray(np.zeros((1,), np.int32)), A_q.reshape(S, D), A_k.reshape(S, D), A_v.reshape(S, D), A_shift_k.T,
      A_ssm_k, A_ssm_D, B_w1.T, B_b1, B_w2, B_b2, *_dft_matrices())
    return out.reshape(1, S, D)
```

```python
import functools

import jax
import jax.numpy as jnp
import numpy as np
from jax.experimental import pallas as pl
from jax.experimental.pallas import tpu as pltpu

S, D, F = 2048, 640, 1728
C = 128
NC = S // C
TM = 256
NB = S // TM
NL = D // 128
NF = 14
NG = C // 8
KG = (0, 4, 8, 12, NF)
NM = len(KG) - 1
NP = NF + NL * NM
UB = 4
KP = 8
LAGS = 5
KQ = 8
AHEAD = 2

f32, bf16, u32 = jnp.float32, jnp.bfloat16, jnp.uint32


def _words(v):
    return pltpu.bitcast(v, u32)


def _rows(v):
    return pltpu.bitcast(v, bf16)


def _dft_matrices():
    theta = 2 * np.pi * (np.arange(C)[:, None] + 0.25) / C * np.arange(C)[None, :]
    co, si = np.cos(theta), np.sin(theta)
    by8 = lambda a, b: np.stack([a.reshape(NG, 8, C), b.reshape(NG, 8, C)], 1).reshape(2 * C, C)

    def words(m):
        b = m.astype(np.float32).astype(jnp.bfloat16).view(np.uint16).astype(np.uint32)
        return b[0::2] | (b[1::2] << 16)

    signal = by8(co, si)
    filt = by8(si - co, si + co)
    inverse = np.stack([co, si], 1).reshape(2 * C, C).T / C
    return np.concatenate([words(signal), words(filt)], 1), words(inverse)


def _kernel(z_h, x_h, k_h, v_h, sk_h, ssm_h, dd_h, w1_h, b1_h, w2_h, b2_h, fwd_h, inv_h, o_h,
            x_v, k_v, v_v, ssm_v, w1_v, w2_v, o_v, xb0, xb1, kvb0, kvb1, ff_v, g_v, acc_v, us, ks, qs, pp,
            b1t_v, fwd_v, inv_v, z_v, sk_v, dd_v, b1_v, b2_v, sems):
    def lanes(c):
        return pl.ds(c * 128, 128)

    xb_v, kvb_v = (xb0, xb1), (kvb0, kvb1)

    x_u, k_u, v_u, o_u, ssm_u, w1_u, w2_u = (r.bitcast(u32) for r in (x_h, k_h, v_h, o_h, ssm_h, w1_h, w2_h))
    copies = []

    def copy(src, dst):
        copies.append(pltpu.make_async_copy(src, dst, sems.at[len(copies)]))
        return copies[-1]

    def fetch_rows(src, dst, lo, hi):
        rr = pl.ds(lo, hi - lo)
        return copy(src.at[rr], dst.at[rr])

    def fetch_conv(x, kv, s):
        lo, hi = kv[0] * TM // 2, kv[1] * TM // 2
        cols = pl.ds(s[0] * C, (s[1] - s[0]) * C)
        return ([copy(k_u.at[pl.ds(lo, hi - lo), lanes(c)], k_v.at[c, pl.ds(KP + lo, hi - lo)]) for c in range(NL)]
                + [fetch_rows(v_u, v_v, lo, hi), copy(ssm_u.at[:, cols], ssm_v.at[:, cols])]
                + ([fetch_rows(x_u, x_v, x[0] * TM // 2, x[1] * TM // 2)] if x else []))

    def store(lo, hi, cols=slice(None)):
        rr = pl.ds(lo * TM // 2, (hi - lo) * TM // 2)
        return copy(o_v.at[rr, cols], o_u.at[rr, cols])

    LEAD_IN = 6
    CONV_AT = (44 + LEAD_IN, 54 + LEAD_IN)
    small = [copy(z_h, z_v), copy(b1_h, b1_v)]
    x_piece = lambda i: fetch_rows(x_u, x_v, i * C // 2, (i + 1) * C // 2)
    w1_piece = lambda q: fetch_rows(w1_u, w1_v, q * 128, min(q * 128 + 128, F // 2))
    first = [fetch_rows(x_u, x_v, 0, TM // 2), w1_piece(0)]
    awaited = {1: [x_piece(2)], 5: [w1_piece(1)], 6: [x_piece(3)]}
    awaited.update({LEAD_IN + 4 * q - 1: [w1_piece(q)] for q in range(2, NF // 2)})
    awaited[LEAD_IN + 2 * NF - 1] = [copy(b2_h, b2_v), copy(w2_u.at[:, 0:256], w2_v.at[:, 0:256])]
    awaited[LEAD_IN + 2 * NF - 1 + 2 * NM] = [copy(w2_u.at[:, 256:D], w2_v.at[:, 256:D])]
    awaited[CONV_AT[0]] = [copy(sk_h, sk_v), copy(dd_h, dd_v), copy(fwd_h, fwd_v), copy(inv_h, inv_v)]
    awaited[CONV_AT[0]] += fetch_conv(None, (0, 1), (0, 2))
    awaited[CONV_AT[1]] = fetch_conv((2, 3), (1, 3), (2, 6))
    per_pass = [fetch_conv((3, 5), (3, 5), (6, 11)), fetch_conv((5, NB), (5, NB), (11, NC))]
    for d in copies:
        d.start()

    k_v[:, 0:KP, :] = jnp.zeros((NL, KP, 128), u32)

    def clear(i, carry):
        us[i // NL, i % NL] = jnp.zeros(us.shape[2:], f32)
        return carry

    jax.lax.fori_loop(0, UB * NL, clear, 0)

    first[0].wait()
    x = _rows(x_v[0:TM // 2, :]).astype(f32)
    xc = x - jnp.sum(x, axis=-1, keepdims=True) * (1.0 / D)
    xn = xc * jax.lax.rsqrt(jnp.sum(xc * xc, axis=-1, keepdims=True) * (1.0 / D) + 1e-5)
    xb0[0:TM // 2, :] = _words(xn.astype(bf16))
    for d in small + [first[1]]:
        d.wait()

    b1t_v[...] = jnp.broadcast_to(b1_v[pl.ds(F - 64, 64)].astype(f32)[None, :], (128, 64)).T

    z0 = z_v[0]
    keep = jax.lax.broadcasted_iota(jnp.int32, (8, 128), 0) >= z0

    def after(v, mark):
        if v.dtype != f32:
            mark = pltpu.bitcast(mark, v.dtype)
        return jnp.where(keep, v, mark)

    def hold(p, mark):
        k_v[z0, pl.ds(KP + S // 2, 8), :] = pltpu.bitcast(mark, u32)

    class Pos:
        def __init__(self, blk):
            static = isinstance(blk, int)
            self.half = blk * (TM // 2) if static else pl.multiple_of(blk * (TM // 2), TM // 2)
            self.full = blk * TM if static else pl.multiple_of(blk * TM, TM)
            self.z = z0 + 2 * blk
            self.head = 0 if static else 1 + 5 * (blk // 2)
            self.far = z0 if static else z0 + 2 * (blk - 4)

    norm = {}

    def layernorm(p, s, h, stage, mark):
        r0 = s * TM + h * 16
        later = lambda v: after(v.reshape(2, 8, 128), mark[None]).reshape(16, 128)
        rowsum = lambda vs: jnp.broadcast_to(jnp.sum(functools.reduce(jnp.add, vs), axis=-1, keepdims=True), (16, 128))
        if stage == 0:
            xs = [x_v[pl.ds(p.half + r0 // 2, 8), lanes(c)] for c in range(NL)]
            xs = [_rows(after(v, mark)).astype(f32) for v in xs]
            norm[s, h] = xs, rowsum(xs)
        elif stage == 1:
            xs, total = norm[s, h]
            mean = later(total) * (1.0 / D)
            xc = [x - mean for x in xs]
            norm[s, h] = xc, rowsum([v * v for v in xc])
        else:
            xc, total = norm.pop((s, h))
            r = jax.lax.rsqrt(later(total) * (1.0 / D) + 1e-5)
            for c in range(NL):
                xb_v[s % 2][pl.ds(p.half + r0 // 2, 8), lanes(c)] = _words((xc[c] * r).astype(bf16))

    def short_conv(p, a, c, i, mark):
        n = C // 2 // KQ
        r0 = p.half + a * C // 2 + i * n
        even = lambda v: pltpu.unpack_elementwise(v, index=0, packed_dtype=bf16, unpacked_dtype=f32)
        odd = lambda v: pltpu.unpack_elementwise(v, index=1, packed_dtype=bf16, unpacked_dtype=f32)
        k0, k1, k2 = (k_v[c, pl.ds(r0 + (KP - d), n), :] for d in range(3))
        k0 = after(k0.reshape(n // 8, 8, 128), mark[None]).reshape(n, 128)
        w = sk_v[:, lanes(c)].astype(f32)
        e1, o1 = even(k1), odd(k1)
        ke = even(k0) * w[0:1] + o1 * w[1:2] + e1 * w[2:3] + odd(k2) * w[3:4]
        ko = odd(k0) * w[0:1] + even(k0) * w[1:2] + o1 * w[2:3] + e1 * w[3:4]
        v = v_v[pl.ds(r0, n), lanes(c)]
        kvb_v[a // 2 % 2][pl.ds(r0, n), lanes(c)] = pltpu.pack_elementwise(
            [ke * even(v), ko * odd(v)], packed_dtype=bf16)

    part = {}
    slot_of = lambda t: (t + 2) % 3

    def products(p, a0, lags, c, g, t, j0, j1, mark):
        if j0 == 0:
            part[t], part["u"] = [None, None], us[p.z + (UB + a0 + 1), c, g, t]
        acc = part[t]
        for j in range(j0, j1):
            kj = ks[(z0 if j < 10 else p.far) + j, c, g, slot_of(t)]
            if j == j0:
                kj = after(kj, mark)
            term = kj * part["u"]
            acc[1] = term if acc[1] is None else acc[1] + term
            if j < lags - 1:
                part["u"] = us[p.z + (UB + a0 - j), c, g, t]
                term = kj * part["u"]
                acc[0] = term if acc[0] is None else acc[0] + term
        if t < 2 or j1 < lags:
            return
        last = (pp[z0, c, g, 0], pp[z0, c, g, 1]) if lags > 2 else None
        for o in range(2):
            half = 0.5 * part[0][o]
            re, im = half - part[2][o], half + part[1][o]
            q = [re, im] if last is None else [re + last[1], im - last[0]]
            qs[p.z + (a0 + o), c, g] = pltpu.pack_elementwise(q, packed_dtype=bf16)
            last = (re, im)
        if lags < NC:
            pp[z0, c, g, 0] = last[0]
            pp[z0, c, g, 1] = last[1]

    def filter_dft(p, a, c, a0=0):
        taps = _rows(ssm_v[pl.ds(c * 64, 64), pl.ds(pl.multiple_of((a0 + a) * C, C), C)])
        kk = jax.lax.dot_general(_rows(fwd_v[:, 128:256]), taps, (((1,), (1,)), ((), ())),
                                 preferred_element_type=f32).reshape(NG, 2, 8, 128)
        ks[z0 + a0 + a, c, :, slot_of(0)] = kk[:, 1] - kk[:, 0]
        ks[z0 + a0 + a, c, :, slot_of(1)] = kk[:, 0]
        ks[z0 + a0 + a, c, :, slot_of(2)] = kk[:, 1]
        return [kk[i, 1] for i in range(NG)]

    def signal_dft(p, a, c):
        kv = _rows(kvb_v[a // 2 % 2][pl.ds(p.half + a * C // 2, C // 2), lanes(c)])
        uu = jnp.dot(_rows(fwd_v[:, 0:128]), kv, preferred_element_type=f32).reshape(NG, 2, 8, 128)
        us[p.z + (UB + a), c, :, 0] = uu[:, 0] + uu[:, 1]
        us[p.z + (UB + a), c, :, 1] = uu[:, 0]
        us[p.z + (UB + a), c, :, 2] = uu[:, 1]
        return [uu[i, 1] for i in range(NG)]

    def gelu2(h):
        c0 = np.float32(np.sqrt(2 / np.pi))
        c1 = np.float32(np.sqrt(2 / np.pi) * 0.044715)
        return h + h * jnp.tanh(h * (c0 + c1 * (h * h)))

    def mlp_up(p, s, i, r0, n, sync):
        f0 = i * 128
        xn = _rows(xb_v[s % 2][pl.ds(p.half + (s * TM + r0) // 2, n // 2), :])
        nt = (((1,), (1,)), ((), ()))
        if i < NF - 1:
            h = jax.lax.dot_general(xn, _rows(w1_v[pl.ds(f0 // 2, 64), :]), nt, preferred_element_type=f32)
            sync()
            g_v[s % 2, pl.ds(r0 // 2, n // 2), lanes(i)] = _words(gelu2(h + b1_v[lanes(i)].astype(f32)[None, :]).astype(bf16))
            return [h[r:r + 8] for r in range(0, n, 8)]
        h = jax.lax.dot_general(_rows(w1_v[pl.ds(f0 // 2, (F - f0) // 2), :]), xn, nt, preferred_element_type=f32)
        sync()
        g = gelu2(h + jnp.concatenate([b1t_v[...]] * (TM // 128), 1))
        g_v[s % 2, :, pl.ds(f0, F - f0)] = _words(g.T.astype(bf16))
        return [h[r:r + 8, q:q + 128] for q in range(0, TM, 128) for r in range(0, F - f0, 8)]

    def mlp_down(p, s, c, m, sync):
        k0, k1 = KG[m] * 128, min(KG[m + 1] * 128, F)
        o = jnp.dot(_rows(g_v[s % 2, :, k0:k1]), _rows(w2_v[k0 // 2:k1 // 2, lanes(c)]), preferred_element_type=f32)
        sync()
        if m > 0:
            o = o + acc_v[z0]
        if m < NM - 1:
            acc_v[z0] = o
        else:
            ff_v[pl.ds(p.full + s * TM, TM), lanes(c)] = 0.5 * o + b2_v[lanes(c)].astype(f32)[None, :]
        return [o[r:r + 8] for r in range(0, TM, 8)]

    def finish(p, a, c):
        rr, rh = pl.ds(p.full + a * C, C), pl.ds(p.half + a * C // 2, C // 2)
        y = jnp.dot(_rows(inv_v[...]), _rows(qs[p.z + a, c].reshape(C, 128)), preferred_element_type=f32)
        x, xn, kv = (_rows(ref[rh, lanes(c)]).astype(f32) for ref in (x_v, xb_v[a // 2 % 2], kvb_v[a // 2 % 2]))
        r = xn * (y + kv * dd_v[lanes(c)].astype(f32)[None, :]) + x + ff_v[rr, lanes(c)]
        o_v[rh, lanes(c)] = _words(r.astype(bf16))
        return []

    up = lambda s: [(mlp_up, s, i % NF, 0, TM) for i in range(-1, NF - 1)]
    down = lambda s: [(mlp_down, s, c, m) for c in range(NL) for m in range(NM)]
    tiles = lambda slot: (5 * slot[4] / TM if slot[2] < NF - 1 else 2.5) if slot[0] is mlp_up else KG[slot[3] + 1] - KG[slot[3]]

    def plan(slots, head, transforms, norms, outputs, spectra, density):
        at = {slot: t for t, slot in enumerate(slots)}
        mxu, side, done = {}, {}, {}
        for lo, hi, chunks, both in transforms:
            items = [(a, c) for c in range(NL) for a in chunks]
            for i, (a, c) in enumerate(items):
                t = int((lo + (hi - lo) * i / len(items)) * NP)
                mxu.setdefault(t, []).extend([(filter_dft, a, c)] * both + [(signal_dft, a, c)])
                done[a, c] = t
                for q in range(KQ):
                    side.setdefault(max(t - AHEAD - (q < KQ // 2), -1), []).append((short_conv, (a, c, q), 200 // KQ))
        for s, t0, span in norms:
            for h in range(TM // 16):
                for stage, cost in enumerate((25, 32, 40)):
                    side.setdefault(t0 + h * span // 16 + stage, []).append((layernorm, (s, h, stage), cost))
        for s, t0 in outputs:
            for c in range(NL):
                t = at[mlp_down, s, c, NM - 1] if t0 is None else t0 + c
                mxu[t] = [(finish, 2 * s, c), (finish, 2 * s + 1, c)] + mxu.get(t, [])
        queue = [(a0, lags, c, g) for a0, lags, cs in spectra for c in cs for g in range(NG)]
        credit = 0.0
        for t, slot in enumerate(slots):
            more = [it[0] for it in mxu.get(t, [])]
            if slot[0] is mlp_up:
                busy = 340 if slot[2] < NF - 1 else 170
            else:
                busy = 32 * tiles(slot) + 32 * (slot[3] == NM - 1)
            busy += sum(150 if fn is finish else 80 for fn in more) + sum(cost for _, _, cost in side.get(t, []))
            credit += max(0.0, density * 64 * (tiles(slot) + len(more)) - busy)
            due = [it[1:] for u in range(t, t + AHEAD + 1) for it in mxu.get(u, []) if it[0] is finish]
            while queue:
                a0, lags, c, g = queue[0]
                urgent = (a0, c) in due or t == len(slots) - 1
                if done.get((a0 + 1, c), -9) >= t - 1:
                    assert not urgent
                    credit = min(credit, 0.0)
                    break
                if credit <= 0 and not urgent:
                    break
                queue.pop(0)
                n = -(-lags // LAGS)
                cuts = [lags * i // n for i in range(n + 1)]
                side.setdefault(t, []).extend(
                    (products, (a0, lags, c, g, comp, j0, j1), 4 * (j1 - j0) + 12 * (comp == 2 and j1 == lags))
                    for comp in range(3) for j0, j1 in zip(cuts, cuts[1:]))
                credit -= 12 * lags + 6
        return slots, head, mxu, side

    def emit(p, timeline, syncs):
        slots, head, mxu, side = timeline
        for t, slot in enumerate([None] + slots, -1):
            if slot is None:
                groups = [(filter_dft(p, a, c, p.head), 1) for a in head for c in range(NL)]
            else:
                groups = [(slot[0](p, *slot[1:], syncs.get(t, lambda: None)), tiles(slot))]
                groups += [(it[0](p, *it[1:]), 1) for it in mxu.get(t, [])]
            marks = [(v, n / len(vals)) for vals, n in groups for v in vals]
            work = side.get(t, [])
            total, span = sum(cost for _, _, cost in work), sum(d for _, d in marks)
            spent, pos, j = 0.0, 0.0, 0
            for fn, args, cost in work:
                while j < len(marks) - 1 and pos < span * spent / total:
                    pos += marks[j][1]
                    j += 1
                fn(p, *args, marks[j][0])
                spent += cost

    every, lead, rest = range(NL), range(3), range(3, NL)
    lead_in = ([(mlp_up, 0, i, r0, C) for r0 in (0, C) for i in (0, 1)] + [(mlp_up, 1, i, 0, C) for i in (0, 1)]
               + [(mlp_up, 0, i, 0, TM) for i in (2, 3)] + [(mlp_up, 1, i, 0, C) for i in (2, 3)]
               + [(mlp_up, 1, i, C, C) for i in range(4)])
    off = LEAD_IN / NP
    opening = plan(lead_in + [(mlp_up, s, 2 * q + i, 0, TM) for q in range(2, NF // 2) for s in (0, 1) for i in (0, 1)]
                   + down(0) + down(1) + up(2), [],
                   [(1.42 + off, 1.66 + off, (0, 1), True), (1.71 + off, 1.9 + off, (2, 3), True),
                    (1.9 + off, 2.15 + off, (4, 5), True)],
                   [(2, CONV_AT[1] + 1, 8)], [(0, 65 + LEAD_IN), (1, 77 + LEAD_IN)], [(0, 2, every), (2, 4, every), (4, 6, lead)], 2.48)
    middle = plan(down(0) + up(1) + down(1) + up(2), range(5),
                  [(0.03, 0.55, (2, 3), False), (0.85, 1.55, (4, 5), False)],
                  [(1, 0, 16), (2, NP, 16)], [(0, None), (1, None)], [(0, 10, rest), (2, 12, every), (4, 14, lead)], 2.51)
    closing = plan(down(6) + up(7) + down(7), [], [(0.12, 0.6, (14, 15), False)],
                   [(7, 0, 16)], [(6, None), (7, None)], [(12, 14, rest), (14, 16, every)], 2.53)
    for t in CONV_AT:
        opening[3].setdefault(t - 1, []).insert(0, (hold, (), 1))

    for h in range(TM // 16):
        for stage in range(3):
            opening[3].setdefault((1 if h < 8 else 6) + stage, []).append((layernorm, (1, h, stage), 32))
    syncs = {t: (lambda ds=ds: [d.wait() for d in ds]) for t, ds in awaited.items()}
    emit(Pos(0), opening, syncs)
    outs = [store(0, 2), store(2, 4), store(4, 6), store(6, 7), store(7, NB, pl.ds(0, 384)),
            store(7, NB, lanes(3)), store(7, NB, lanes(4))]

    def one_pass(it, carry):
        for i in range(2):
            @pl.when(it == i)
            def _():
                for d in per_pass[i]:
                    d.wait()
                outs[i].start()
        emit(Pos(2 * it + 2), middle, {})
        return carry

    jax.lax.fori_loop(0, 2, one_pass, 0)
    outs[2].start()
    emit(Pos(0), closing, {len(closing[0]) - 2 * NM + 1: lambda: [d.start() for d in outs[3:5]],
                           len(closing[0]) - NM + 1: outs[5].start})
    outs[6].start()
    for d in outs:
        d.wait()


@jax.jit
def pallas_parallel_sum__ssm_conv_h3__dense_activation_gelu__prompt_kernel(
        A_q, A_k, A_v, A_shift_k, A_ssm_k, A_ssm_D, B_x, B_w1, B_b1, B_w2, B_b2):
    del B_x
    vmem = pltpu.VMEM
    seq = vmem((S // 2, D), u32)
    hbm = pl.BlockSpec(memory_space=pl.ANY)
    out = pl.pallas_call(
        _kernel,
        in_specs=[hbm] * 13,
        out_specs=hbm,
        out_shape=jax.ShapeDtypeStruct((S, D), bf16),
        scratch_shapes=[
            seq, vmem((NL, S // 2 + 32, 128), u32), seq,
            vmem((D // 2, S), u32), vmem((F // 2, D), u32), vmem((F // 2, D), u32), seq,
            seq, seq, seq, seq,
            vmem((S, D), f32), vmem((2, TM // 2, NF * 128), u32), vmem((1, TM, 128), f32),
            vmem((UB + NC, NL, NG, 3, 8, 128), f32), vmem((NC, NL, NG, 3, 8, 128), f32),
            vmem((NC, NL, NG, 8, 128), u32), vmem((1, NL, NG, 2, 8, 128), f32),
            vmem((64, 128), f32), vmem((C, 2 * C), u32), vmem((C // 2, 2 * C), u32), pltpu.SMEM((1,), jnp.int32),
            vmem((4, D), bf16), vmem((D,), bf16), vmem((F,), bf16), vmem((D,), bf16),
            pltpu.SemaphoreType.DMA((64,)),
        ],
        compiler_params=pltpu.CompilerParams(
            vmem_limit_bytes=110 * 1024 * 1024, flags={"XLA_TPU_RESCHEDULE_DMA_DONES": True}),
    )(jnp.asarray(np.zeros((1,), np.int32)), A_q.reshape(S, D), A_k.reshape(S, D), A_v.reshape(S, D), A_shift_k.T,
      A_ssm_k, A_ssm_D, B_w1.T, B_b1, B_w2, B_b2, *_dft_matrices())
    return out.reshape(1, S, D)
```

```python
import functools

import jax
import jax.numpy as jnp
import numpy as np
from jax.experimental import pallas as pl
from jax.experimental.pallas import tpu as pltpu

S, D, F = 2048, 640, 1728
C = 128
NC = S // C
TM = 256
NB = S // TM
NL = D // 128
NF = 14
NG = C // 8
KG = (0, 4, 8, 12, NF)
NM = len(KG) - 1
NP = NF + NL * NM
UB = 4
KP = 8
LAGS = 4
KQ = 8
AHEAD = 2

f32, bf16, u32 = jnp.float32, jnp.bfloat16, jnp.uint32


def _words(v):
    return pltpu.bitcast(v, u32)


def _rows(v):
    return pltpu.bitcast(v, bf16)


def _dft_matrices():
    theta = 2 * np.pi * (np.arange(C)[:, None] + 0.25) / C * np.arange(C)[None, :]
    co, si = np.cos(theta), np.sin(theta)
    by8 = lambda a, b: np.stack([a.reshape(NG, 8, C), b.reshape(NG, 8, C)], 1).reshape(2 * C, C)

    def words(m):
        b = m.astype(np.float32).astype(jnp.bfloat16).view(np.uint16).astype(np.uint32)
        return b[0::2] | (b[1::2] << 16)

    signal = by8(co, si)
    filt = by8(si - co, si + co)
    inverse = np.stack([co, si], 1).reshape(2 * C, C).T / C
    return np.concatenate([words(signal), words(filt)], 1), words(inverse)


def _kernel(z_h, x_h, k_h, v_h, sk_h, ssm_h, dd_h, w1_h, b1_h, w2_h, b2_h, fwd_h, inv_h, o_h,
            x_v, k_v, v_v, ssm_v, w1_v, w2_v, o_v, xb0, xb1, kvb0, kvb1, ff_v, g_v, acc_v, us, ks, qs, pp,
            b1t_v, fwd_v, inv_v, z_v, sk_v, dd_v, b1_v, b2_v, sems):
    def lanes(c):
        return pl.ds(c * 128, 128)

    xb_v, kvb_v = (xb0, xb1), (kvb0, kvb1)

    x_u, k_u, v_u, o_u, ssm_u, w1_u, w2_u = (r.bitcast(u32) for r in (x_h, k_h, v_h, o_h, ssm_h, w1_h, w2_h))
    copies = []

    def copy(src, dst):
        copies.append(pltpu.make_async_copy(src, dst, sems.at[len(copies)]))
        return copies[-1]

    def fetch_rows(src, dst, lo, hi):
        rr = pl.ds(lo, hi - lo)
        return copy(src.at[rr], dst.at[rr])

    def fetch_conv(x, kv, s):
        lo, hi = kv[0] * TM // 2, kv[1] * TM // 2
        cols = pl.ds(s[0] * C, (s[1] - s[0]) * C)
        return ([copy(k_u.at[pl.ds(lo, hi - lo), lanes(c)], k_v.at[c, pl.ds(KP + lo, hi - lo)]) for c in range(NL)]
                + [fetch_rows(v_u, v_v, lo, hi), copy(ssm_u.at[:, cols], ssm_v.at[:, cols])]
                + ([fetch_rows(x_u, x_v, x[0] * TM // 2, x[1] * TM // 2)] if x else []))

    def store(lo, hi, cols=slice(None)):
        rr = pl.ds(lo * TM // 2, (hi - lo) * TM // 2)
        return copy(o_v.at[rr, cols], o_u.at[rr, cols])

    LEAD_IN = 6
    CONV_AT = (44 + LEAD_IN, 54 + LEAD_IN)
    small = [copy(z_h, z_v), copy(b1_h, b1_v)]
    x_piece = lambda i: fetch_rows(x_u, x_v, i * C // 2, (i + 1) * C // 2)
    w1_piece = lambda q: fetch_rows(w1_u, w1_v, q * 128, min(q * 128 + 128, F // 2))
    first = [fetch_rows(x_u, x_v, 0, TM // 2), w1_piece(0)]
    awaited = {1: [x_piece(2)], 5: [w1_piece(1)], 6: [x_piece(3)]}
    awaited.update({LEAD_IN + 4 * q - 1: [w1_piece(q)] for q in range(2, NF // 2)})
    awaited[LEAD_IN + 2 * NF - 1] = [copy(b2_h, b2_v), copy(w2_u.at[:, 0:256], w2_v.at[:, 0:256])]
    awaited[LEAD_IN + 2 * NF - 1 + 2 * NM] = [copy(w2_u.at[:, 256:D], w2_v.at[:, 256:D])]
    awaited[CONV_AT[0]] = [copy(sk_h, sk_v), copy(dd_h, dd_v), copy(fwd_h, fwd_v), copy(inv_h, inv_v)]
    awaited[CONV_AT[0]] += fetch_conv(None, (0, 1), (0, 2))
    awaited[CONV_AT[1]] = fetch_conv((2, 3), (1, 3), (2, 6))
    per_pass = [fetch_conv((3, 5), (3, 5), (6, 11)), fetch_conv((5, NB), (5, NB), (11, NC))]
    for d in copies:
        d.start()

    k_v[:, 0:KP, :] = jnp.zeros((NL, KP, 128), u32)

    def clear(i, carry):
        us[i // NL, i % NL] = jnp.zeros(us.shape[2:], f32)
        return carry

    jax.lax.fori_loop(0, UB * NL, clear, 0)

    first[0].wait()
    x = _rows(x_v[0:TM // 2, :]).astype(f32)
    xc = x - jnp.sum(x, axis=-1, keepdims=True) * (1.0 / D)
    xn = xc * jax.lax.rsqrt(jnp.sum(xc * xc, axis=-1, keepdims=True) * (1.0 / D) + 1e-5)
    xb0[0:TM // 2, :] = _words(xn.astype(bf16))
    for d in small + [first[1]]:
        d.wait()

    b1t_v[...] = jnp.broadcast_to(b1_v[pl.ds(F - 64, 64)].astype(f32)[None, :], (128, 64)).T

    z0 = z_v[0]
    keep = jax.lax.broadcasted_iota(jnp.int32, (8, 128), 0) >= z0

    def after(v, mark):
        if v.dtype != f32:
            mark = pltpu.bitcast(mark, v.dtype)
        return jnp.where(keep, v, mark)

    def hold(p, mark):
        k_v[z0, pl.ds(KP + S // 2, 8), :] = pltpu.bitcast(mark, u32)

    class Pos:
        def __init__(self, blk):
            static = isinstance(blk, int)
            self.half = blk * (TM // 2) if static else pl.multiple_of(blk * (TM // 2), TM // 2)
            self.full = blk * TM if static else pl.multiple_of(blk * TM, TM)
            self.z = z0 + 2 * blk
            self.head = 0 if static else 1 + 5 * (blk // 2)
            self.far = z0 if static else z0 + 2 * (blk - 4)

    norm = {}

    def layernorm(p, s, h, stage, mark):
        r0 = s * TM + h * 16
        later = lambda v: after(v.reshape(2, 8, 128), mark[None]).reshape(16, 128)
        rowsum = lambda vs: jnp.broadcast_to(jnp.sum(functools.reduce(jnp.add, vs), axis=-1, keepdims=True), (16, 128))
        if stage == 0:
            xs = [x_v[pl.ds(p.half + r0 // 2, 8), lanes(c)] for c in range(NL)]
            xs = [_rows(after(v, mark)).astype(f32) for v in xs]
            norm[s, h] = xs, rowsum(xs)
        elif stage == 1:
            xs, total = norm[s, h]
            mean = later(total) * (1.0 / D)
            xc = [x - mean for x in xs]
            norm[s, h] = xc, rowsum([v * v for v in xc])
        else:
            xc, total = norm.pop((s, h))
            r = jax.lax.rsqrt(later(total) * (1.0 / D) + 1e-5)
            for c in range(NL):
                xb_v[s % 2][pl.ds(p.half + r0 // 2, 8), lanes(c)] = _words((xc[c] * r).astype(bf16))

    def short_conv(p, a, c, i, mark):
        n = C // 2 // KQ
        r0 = p.half + a * C // 2 + i * n
        even = lambda v: pltpu.unpack_elementwise(v, index=0, packed_dtype=bf16, unpacked_dtype=f32)
        odd = lambda v: pltpu.unpack_elementwise(v, index=1, packed_dtype=bf16, unpacked_dtype=f32)
        k0, k1, k2 = (k_v[c, pl.ds(r0 + (KP - d), n), :] for d in range(3))
        k0 = after(k0.reshape(n // 8, 8, 128), mark[None]).reshape(n, 128)
        w = sk_v[:, lanes(c)].astype(f32)
        e1, o1 = even(k1), odd(k1)
        ke = even(k0) * w[0:1] + o1 * w[1:2] + e1 * w[2:3] + odd(k2) * w[3:4]
        ko = odd(k0) * w[0:1] + even(k0) * w[1:2] + o1 * w[2:3] + e1 * w[3:4]
        v = v_v[pl.ds(r0, n), lanes(c)]
        kvb_v[a // 2 % 2][pl.ds(r0, n), lanes(c)] = pltpu.pack_elementwise(
            [ke * even(v), ko * odd(v)], packed_dtype=bf16)

    part = {}
    slot_of = lambda t: (t + 2) % 3

    def products(p, a0, lags, c, g, t, j0, j1, mark):
        if j0 == 0:
            part[t], part["u"] = [None, None], us[p.z + (UB + a0 + 1), c, g, t]
        acc = part[t]
        for j in range(j0, j1):
            kj = ks[(z0 if j < 10 else p.far) + j, c, g, slot_of(t)]
            if j == j0:
                kj = after(kj, mark)
            term = kj * part["u"]
            acc[1] = term if acc[1] is None else acc[1] + term
            if j < lags - 1:
                part["u"] = us[p.z + (UB + a0 - j), c, g, t]
                term = kj * part["u"]
                acc[0] = term if acc[0] is None else acc[0] + term
        if t < 2 or j1 < lags:
            return
        last = (pp[z0, c, g, 0], pp[z0, c, g, 1]) if lags > 2 else None
        for o in range(2):
            half = 0.5 * part[0][o]
            re, im = half - part[2][o], half + part[1][o]
            q = [re, im] if last is None else [re + last[1], im - last[0]]
            qs[p.z + (a0 + o), c, g] = pltpu.pack_elementwise(q, packed_dtype=bf16)
            last = (re, im)
        if lags < NC:
            pp[z0, c, g, 0] = last[0]
            pp[z0, c, g, 1] = last[1]

    def filter_dft(p, a, c, a0=0):
        taps = _rows(ssm_v[pl.ds(c * 64, 64), pl.ds(pl.multiple_of((a0 + a) * C, C), C)])
        kk = jax.lax.dot_general(_rows(fwd_v[:, 128:256]), taps, (((1,), (1,)), ((), ())),
                                 preferred_element_type=f32).reshape(NG, 2, 8, 128)
        ks[z0 + a0 + a, c, :, slot_of(0)] = kk[:, 1] - kk[:, 0]
        ks[z0 + a0 + a, c, :, slot_of(1)] = kk[:, 0]
        ks[z0 + a0 + a, c, :, slot_of(2)] = kk[:, 1]
        return [kk[i, 1] for i in range(NG)]

    def signal_dft(p, a, c):
        kv = _rows(kvb_v[a // 2 % 2][pl.ds(p.half + a * C // 2, C // 2), lanes(c)])
        uu = jnp.dot(_rows(fwd_v[:, 0:128]), kv, preferred_element_type=f32).reshape(NG, 2, 8, 128)
        us[p.z + (UB + a), c, :, 0] = uu[:, 0] + uu[:, 1]
        us[p.z + (UB + a), c, :, 1] = uu[:, 0]
        us[p.z + (UB + a), c, :, 2] = uu[:, 1]
        return [uu[i, 1] for i in range(NG)]

    def gelu2(h):
        c0 = np.float32(np.sqrt(2 / np.pi))
        c1 = np.float32(np.sqrt(2 / np.pi) * 0.044715)
        return h + h * jnp.tanh(h * (c0 + c1 * (h * h)))

    def mlp_up(p, s, i, r0, n, sync):
        f0 = i * 128
        xn = _rows(xb_v[s % 2][pl.ds(p.half + (s * TM + r0) // 2, n // 2), :])
        nt = (((1,), (1,)), ((), ()))
        if i < NF - 1:
            h = jax.lax.dot_general(xn, _rows(w1_v[pl.ds(f0 // 2, 64), :]), nt, preferred_element_type=f32)
            sync()
            g_v[s % 2, pl.ds(r0 // 2, n // 2), lanes(i)] = _words(gelu2(h + b1_v[lanes(i)].astype(f32)[None, :]).astype(bf16))
            return [h[r:r + 8] for r in range(0, n, 8)]
        h = jax.lax.dot_general(_rows(w1_v[pl.ds(f0 // 2, (F - f0) // 2), :]), xn, nt, preferred_element_type=f32)
        sync()
        g = gelu2(h + jnp.concatenate([b1t_v[...]] * (TM // 128), 1))
        g_v[s % 2, :, pl.ds(f0, F - f0)] = _words(g.T.astype(bf16))
        return [h[r:r + 8, q:q + 128] for q in range(0, TM, 128) for r in range(0, F - f0, 8)]

    def mlp_down(p, s, c, m, sync):
        k0, k1 = KG[m] * 128, min(KG[m + 1] * 128, F)
        o = jnp.dot(_rows(g_v[s % 2, :, k0:k1]), _rows(w2_v[k0 // 2:k1 // 2, lanes(c)]), preferred_element_type=f32)
        sync()
        if m > 0:
            o = o + acc_v[z0]
        if m < NM - 1:
            acc_v[z0] = o
        else:
            ff_v[pl.ds(p.full + s * TM, TM), lanes(c)] = 0.5 * o + b2_v[lanes(c)].astype(f32)[None, :]
        return [o[r:r + 8] for r in range(0, TM, 8)]

    def finish(p, a, c):
        rr, rh = pl.ds(p.full + a * C, C), pl.ds(p.half + a * C // 2, C // 2)
        y = jnp.dot(_rows(inv_v[...]), _rows(qs[p.z + a, c].reshape(C, 128)), preferred_element_type=f32)
        x, xn, kv = (_rows(ref[rh, lanes(c)]).astype(f32) for ref in (x_v, xb_v[a // 2 % 2], kvb_v[a // 2 % 2]))
        r = xn * (y + kv * dd_v[lanes(c)].astype(f32)[None, :]) + x + ff_v[rr, lanes(c)]
        o_v[rh, lanes(c)] = _words(r.astype(bf16))
        return []

    up = lambda s: [(mlp_up, s, i % NF, 0, TM) for i in range(-1, NF - 1)]
    down = lambda s: [(mlp_down, s, c, m) for c in range(NL) for m in range(NM)]
    tiles = lambda slot: (5 * slot[4] / TM if slot[2] < NF - 1 else 2.5) if slot[0] is mlp_up else KG[slot[3] + 1] - KG[slot[3]]

    def plan(slots, head, transforms, norms, outputs, spectra, density):
        at = {slot: t for t, slot in enumerate(slots)}
        mxu, side, done = {}, {}, {}
        for lo, hi, chunks, both in transforms:
            items = [(a, c) for c in range(NL) for a in chunks]
            for i, (a, c) in enumerate(items):
                t = int((lo + (hi - lo) * i / len(items)) * NP)
                mxu.setdefault(t, []).extend([(filter_dft, a, c)] * both + [(signal_dft, a, c)])
                done[a, c] = t
                for q in range(KQ):
                    side.setdefault(max(t - AHEAD - (q < KQ // 2), -1), []).append((short_conv, (a, c, q), 200 // KQ))
        for s, t0, span in norms:
            for h in range(TM // 16):
                for stage, cost in enumerate((25, 32, 40)):
                    side.setdefault(t0 + h * span // 16 + 3 * stage, []).append((layernorm, (s, h, stage), cost))
        for s, t0 in outputs:
            for c in range(NL):
                t = at[mlp_down, s, c, NM - 1] if t0 is None else t0 + c
                mxu[t] = [(finish, 2 * s, c), (finish, 2 * s + 1, c)] + mxu.get(t, [])
        queue = [(a0, lags, c, g) for a0, lags, cs in spectra for c in cs for g in range(NG)]
        credit = 0.0
        for t, slot in enumerate(slots):
            more = [it[0] for it in mxu.get(t, [])]
            if slot[0] is mlp_up:
                busy = 340 if slot[2] < NF - 1 else 170
            else:
                busy = 32 * tiles(slot) + 32 * (slot[3] == NM - 1)
            busy += sum(150 if fn is finish else 80 for fn in more) + sum(cost for _, _, cost in side.get(t, []))
            credit += max(0.0, density * 64 * (tiles(slot) + len(more)) - busy)
            due = [it[1:] for u in range(t, t + AHEAD + 1) for it in mxu.get(u, []) if it[0] is finish]
            while queue:
                a0, lags, c, g = queue[0]
                urgent = (a0, c) in due or t == len(slots) - 1
                if done.get((a0 + 1, c), -9) >= t - 1:
                    assert not urgent
                    credit = min(credit, 0.0)
                    break
                if credit <= 0 and not urgent:
                    break
                queue.pop(0)
                n = -(-lags // LAGS)
                cuts = [lags * i // n for i in range(n + 1)]
                side.setdefault(t, []).extend(
                    (products, (a0, lags, c, g, comp, j0, j1), 4 * (j1 - j0) + 12 * (comp == 2 and j1 == lags))
                    for comp in range(3) for j0, j1 in zip(cuts, cuts[1:]))
                credit -= 12 * lags + 6
        return slots, head, mxu, side

    def emit(p, timeline, syncs):
        slots, head, mxu, side = timeline
        for t, slot in enumerate([None] + slots, -1):
            if slot is None:
                groups = [(filter_dft(p, a, c, p.head), 1) for a in head for c in range(NL)]
            else:
                groups = [(slot[0](p, *slot[1:], syncs.get(t, lambda: None)), tiles(slot))]
                groups += [(it[0](p, *it[1:]), 1) for it in mxu.get(t, [])]
            marks = [(v, n / len(vals)) for vals, n in groups for v in vals]
            work = side.get(t, [])
            total, span = sum(cost for _, _, cost in work), sum(d for _, d in marks)
            spent, pos, j = 0.0, 0.0, 0
            for fn, args, cost in work:
                while j < len(marks) - 1 and pos < span * spent / total:
                    pos += marks[j][1]
                    j += 1
                fn(p, *args, marks[j][0])
                spent += cost

    every, lead, rest = range(NL), range(3), range(3, NL)
    lead_in = ([(mlp_up, 0, i, r0, C) for r0 in (0, C) for i in (0, 1)] + [(mlp_up, 1, i, 0, C) for i in (0, 1)]
               + [(mlp_up, 0, i, 0, TM) for i in (2, 3)] + [(mlp_up, 1, i, 0, C) for i in (2, 3)]
               + [(mlp_up, 1, i, C, C) for i in range(4)])
    off = LEAD_IN / NP
    opening = plan(lead_in + [(mlp_up, s, 2 * q + i, 0, TM) for q in range(2, NF // 2) for s in (0, 1) for i in (0, 1)]
                   + down(0) + down(1) + up(2), [],
                   [(1.42 + off, 1.66 + off, (0, 1), True), (1.71 + off, 1.9 + off, (2, 3), True),
                    (1.9 + off, 2.15 + off, (4, 5), True)],
                   [(2, CONV_AT[1] + 1, 5)], [(0, 65 + LEAD_IN), (1, 77 + LEAD_IN)], [(0, 2, every), (2, 4, every), (4, 6, lead)], 2.48)
    middle = plan(down(0) + up(1) + down(1) + up(2), range(5),
                  [(0.03, 0.55, (2, 3), False), (0.85, 1.55, (4, 5), False)],
                  [(1, 0, 12), (2, NP, 12)], [(0, None), (1, None)], [(0, 10, rest), (2, 12, every), (4, 14, lead)], 2.51)
    closing = plan(down(6) + up(7) + down(7), [], [(0.12, 0.6, (14, 15), False)],
                   [(7, 0, 12)], [(6, None), (7, None)], [(12, 14, rest), (14, 16, every)], 2.53)
    for t in CONV_AT:
        opening[3].setdefault(t - 1, []).insert(0, (hold, (), 1))

    for h in range(TM // 16):
        for stage in range(3):
            opening[3].setdefault((1 if h < 8 else 6) + stage, []).append((layernorm, (1, h, stage), 32))
    syncs = {t: (lambda ds=ds: [d.wait() for d in ds]) for t, ds in awaited.items()}
    emit(Pos(0), opening, syncs)
    outs = [store(0, 2), store(2, 4), store(4, 6), store(6, 7), store(7, NB, pl.ds(0, 384)),
            store(7, NB, lanes(3)), store(7, NB, lanes(4))]

    def one_pass(it, carry):
        for i in range(2):
            @pl.when(it == i)
            def _():
                for d in per_pass[i]:
                    d.wait()
                outs[i].start()
        emit(Pos(2 * it + 2), middle, {})
        return carry

    jax.lax.fori_loop(0, 2, one_pass, 0)
    outs[2].start()
    emit(Pos(0), closing, {len(closing[0]) - 2 * NM + 1: lambda: [d.start() for d in outs[3:5]],
                           len(closing[0]) - NM + 1: outs[5].start})
    outs[6].start()
    for d in outs:
        d.wait()


@jax.jit
def pallas_parallel_sum__ssm_conv_h3__dense_activation_gelu__prompt_kernel(
        A_q, A_k, A_v, A_shift_k, A_ssm_k, A_ssm_D, B_x, B_w1, B_b1, B_w2, B_b2):
    del B_x
    vmem = pltpu.VMEM
    seq = vmem((S // 2, D), u32)
    hbm = pl.BlockSpec(memory_space=pl.ANY)
    out = pl.pallas_call(
        _kernel,
        in_specs=[hbm] * 13,
        out_specs=hbm,
        out_shape=jax.ShapeDtypeStruct((S, D), bf16),
        scratch_shapes=[
            seq, vmem((NL, S // 2 + 32, 128), u32), seq,
            vmem((D // 2, S), u32), vmem((F // 2, D), u32), vmem((F // 2, D), u32), seq,
            seq, seq, seq, seq,
            vmem((S, D), f32), vmem((2, TM // 2, NF * 128), u32), vmem((1, TM, 128), f32),
            vmem((UB + NC, NL, NG, 3, 8, 128), f32), vmem((NC, NL, NG, 3, 8, 128), f32),
            vmem((NC, NL, NG, 8, 128), u32), vmem((1, NL, NG, 2, 8, 128), f32),
            vmem((64, 128), f32), vmem((C, 2 * C), u32), vmem((C // 2, 2 * C), u32), pltpu.SMEM((1,), jnp.int32),
            vmem((4, D), bf16), vmem((D,), bf16), vmem((F,), bf16), vmem((D,), bf16),
            pltpu.SemaphoreType.DMA((64,)),
        ],
        compiler_params=pltpu.CompilerParams(
            vmem_limit_bytes=110 * 1024 * 1024, flags={"XLA_TPU_RESCHEDULE_DMA_DONES": True}),
    )(jnp.asarray(np.zeros((1,), np.int32)), A_q.reshape(S, D), A_k.reshape(S, D), A_v.reshape(S, D), A_shift_k.T,
      A_ssm_k, A_ssm_D, B_w1.T, B_b1, B_w2, B_b2, *_dft_matrices())
    return out.reshape(1, S, D)
```

```python
import functools

import jax
import jax.numpy as jnp
import numpy as np
from jax.experimental import pallas as pl
from jax.experimental.pallas import tpu as pltpu

S, D, F = 2048, 640, 1728
C = 128
NC = S // C
TM = 256
NB = S // TM
NL = D // 128
NF = 14
NG = C // 8
KG = (0, 4, 8, 12, NF)
NM = len(KG) - 1
NP = NF + NL * NM
UB = 4
KP = 8
LAGS = 4
KQ = C // 16
AHEAD = 2

f32, bf16, u32 = jnp.float32, jnp.bfloat16, jnp.uint32


def _words(v):
    return pltpu.bitcast(v, u32)


def _rows(v):
    return pltpu.bitcast(v, bf16)


def _dft_matrices():
    theta = 2 * np.pi * (np.arange(C)[:, None] + 0.25) / C * np.arange(C)[None, :]
    co, si = np.cos(theta), np.sin(theta)
    by8 = lambda a, b: np.stack([a.reshape(NG, 8, C), b.reshape(NG, 8, C)], 1).reshape(2 * C, C)

    def words(m):
        b = m.astype(np.float32).astype(jnp.bfloat16).view(np.uint16).astype(np.uint32)
        return b[0::2] | (b[1::2] << 16)

    steps = np.arange(C).reshape(C // 16, 8, 2).transpose(0, 2, 1).reshape(C)
    signal = by8(co, si)[:, steps]
    filt = by8(si - co, si + co)
    inverse = by8(co, si).T / C
    return np.concatenate([words(signal), words(filt)], 1), words(inverse)


def _kernel(z_h, x_h, k_h, v_h, sk_h, ssm_h, dd_h, w1_h, b1_h, w2_h, b2_h, fwd_h, inv_h, o_h,
            x_v, k_v, v_v, ssm_v, w1_v, w2_v, o_v, xb0, xb1, kvb0, kvb1, ff_v, g_v, acc_v, us, ks, qs, pp,
            b1t_v, fwd_v, inv_v, z_v, sk_v, dd_v, b1_v, b2_v, sems):
    def lanes(c):
        return pl.ds(c * 128, 128)

    xb_v, kvb_v = (xb0, xb1), (kvb0, kvb1)

    x_u, k_u, v_u, o_u, ssm_u, w1_u, w2_u = (r.bitcast(u32) for r in (x_h, k_h, v_h, o_h, ssm_h, w1_h, w2_h))
    copies = []

    def copy(src, dst):
        copies.append(pltpu.make_async_copy(src, dst, sems.at[len(copies)]))
        return copies[-1]

    def fetch_rows(src, dst, lo, hi):
        rr = pl.ds(lo, hi - lo)
        return copy(src.at[rr], dst.at[rr])

    def fetch_conv(x, kv, s):
        lo, hi = kv[0] * TM // 2, kv[1] * TM // 2
        cols = pl.ds(s[0] * C, (s[1] - s[0]) * C)
        return ([copy(k_u.at[pl.ds(lo, hi - lo), lanes(c)], k_v.at[c, pl.ds(KP + lo, hi - lo)]) for c in range(NL)]
                + [fetch_rows(v_u, v_v, lo, hi), copy(ssm_u.at[:, cols], ssm_v.at[:, cols])]
                + ([fetch_rows(x_u, x_v, x[0] * TM // 2, x[1] * TM // 2)] if x else []))

    def store(lo, hi, cols=slice(None)):
        rr = pl.ds(lo * TM // 2, (hi - lo) * TM // 2)
        return copy(o_v.at[rr, cols], o_u.at[rr, cols])

    LEAD_IN = 6
    CONV_AT = (44 + LEAD_IN, 54 + LEAD_IN)
    small = [copy(z_h, z_v), copy(b1_h, b1_v)]
    x_piece = lambda i: fetch_rows(x_u, x_v, i * C // 2, (i + 1) * C // 2)
    w1_piece = lambda q: fetch_rows(w1_u, w1_v, q * 128, min(q * 128 + 128, F // 2))
    first = [fetch_rows(x_u, x_v, 0, TM // 2), w1_piece(0)]
    awaited = {1: [x_piece(2)], 5: [w1_piece(1)], 6: [x_piece(3)]}
    awaited.update({LEAD_IN + 4 * q - 1: [w1_piece(q)] for q in range(2, NF // 2)})
    awaited[LEAD_IN + 2 * NF - 1] = [copy(b2_h, b2_v), copy(w2_u.at[:, 0:256], w2_v.at[:, 0:256])]
    awaited[LEAD_IN + 2 * NF - 1 + 2 * NM] = [copy(w2_u.at[:, 256:D], w2_v.at[:, 256:D])]
    awaited[CONV_AT[0]] = [copy(sk_h, sk_v), copy(dd_h, dd_v), copy(fwd_h, fwd_v), copy(inv_h, inv_v)]
    awaited[CONV_AT[0]] += fetch_conv(None, (0, 1), (0, 2))
    awaited[CONV_AT[1]] = fetch_conv((2, 3), (1, 3), (2, 6))
    per_pass = [fetch_conv((3, 5), (3, 5), (6, 11)), fetch_conv((5, NB), (5, NB), (11, NC))]
    for d in copies:
        d.start()

    k_v[:, 0:KP, :] = jnp.zeros((NL, KP, 128), u32)

    def clear(i, carry):
        us[i // NL, i % NL] = jnp.zeros(us.shape[2:], f32)
        return carry

    jax.lax.fori_loop(0, UB * NL, clear, 0)

    first[0].wait()
    x = _rows(x_v[0:TM // 2, :]).astype(f32)
    xc = x - jnp.sum(x, axis=-1, keepdims=True) * (1.0 / D)
    xn = xc * jax.lax.rsqrt(jnp.sum(xc * xc, axis=-1, keepdims=True) * (1.0 / D) + 1e-5)
    xb0[0:TM // 2, :] = _words(xn.astype(bf16))
    for d in small + [first[1]]:
        d.wait()

    b1t_v[...] = jnp.broadcast_to(b1_v[pl.ds(F - 64, 64)].astype(f32)[None, :], (128, 64)).T

    z0 = z_v[0]
    keep = jax.lax.broadcasted_iota(jnp.int32, (8, 128), 0) >= z0

    def after(v, mark):
        if v.dtype != f32:
            mark = pltpu.bitcast(mark, v.dtype)
        return jnp.where(keep, v, mark)

    def hold(p, mark):
        k_v[z0, pl.ds(KP + S // 2, 8), :] = pltpu.bitcast(mark, u32)

    class Pos:
        def __init__(self, blk):
            static = isinstance(blk, int)
            self.half = blk * (TM // 2) if static else pl.multiple_of(blk * (TM // 2), TM // 2)
            self.full = blk * TM if static else pl.multiple_of(blk * TM, TM)
            self.z = z0 + 2 * blk
            self.head = 0 if static else 1 + 5 * (blk // 2)
            self.far = z0 if static else z0 + 2 * (blk - 4)

    norm = {}

    def layernorm(p, s, h, stage, mark):
        r0 = s * TM + h * 16
        later = lambda v: after(v.reshape(2, 8, 128), mark[None]).reshape(16, 128)
        rowsum = lambda vs: jnp.broadcast_to(jnp.sum(functools.reduce(jnp.add, vs), axis=-1, keepdims=True), (16, 128))
        if stage == 0:
            xs = [x_v[pl.ds(p.half + r0 // 2, 8), lanes(c)] for c in range(NL)]
            xs = [_rows(after(v, mark)).astype(f32) for v in xs]
            norm[s, h] = xs, rowsum(xs)
        elif stage == 1:
            xs, total = norm[s, h]
            mean = later(total) * (1.0 / D)
            xc = [x - mean for x in xs]
            norm[s, h] = xc, rowsum([v * v for v in xc])
        else:
            xc, total = norm.pop((s, h))
            r = jax.lax.rsqrt(later(total) * (1.0 / D) + 1e-5)
            for c in range(NL):
                xb_v[s % 2][pl.ds(p.half + r0 // 2, 8), lanes(c)] = _words((xc[c] * r).astype(bf16))

    def short_conv(p, a, c, i, mark):
        n = C // 2 // KQ
        r0 = p.half + a * C // 2 + i * n
        even = lambda v: pltpu.bitcast(v << 16, f32)
        odd = lambda v: pltpu.bitcast(v & np.uint32(0xFFFF0000), f32)
        k0, k1, k2 = (k_v[c, pl.ds(r0 + (KP - d), n), :] for d in range(3))
        k0 = after(k0.reshape(n // 8, 8, 128), mark[None]).reshape(n, 128)
        w = sk_v[:, lanes(c)].astype(f32)
        e1, o1 = even(k1), odd(k1)
        ke = even(k0) * w[0:1] + o1 * w[1:2] + e1 * w[2:3] + odd(k2) * w[3:4]
        ko = odd(k0) * w[0:1] + even(k0) * w[1:2] + o1 * w[2:3] + e1 * w[3:4]
        v = v_v[pl.ds(r0, n), lanes(c)]
        kv = jnp.concatenate([ke * even(v), ko * odd(v)], 0)
        kvb_v[a // 2 % 2][pl.ds(r0, n), lanes(c)] = _words(kv.astype(bf16))

    part = {}
    slot_of = lambda t: (t + 2) % 3

    def products(p, a0, lags, c, g, t, j0, j1, mark):
        if j0 == 0:
            part[t], part["u"] = [None, None], us[p.z + (UB + a0 + 1), c, g, t]
        acc = part[t]
        for j in range(j0, j1):
            kj = ks[(z0 if j < 10 else p.far) + j, c, g, slot_of(t)]
            if j == j0:
                kj = after(kj, mark)
            term = kj * part["u"]
            acc[1] = term if acc[1] is None else acc[1] + term
            if j < lags - 1:
                part["u"] = us[p.z + (UB + a0 - j), c, g, t]
                term = kj * part["u"]
                acc[0] = term if acc[0] is None else acc[0] + term
        if t < 2 or j1 < lags:
            return
        last = (pp[z0, c, g, 0], pp[z0, c, g, 1]) if lags > 2 else None
        for o in range(2):
            half = 0.5 * part[0][o]
            re, im = half - part[2][o], half + part[1][o]
            q = [re, im] if last is None else [re + last[1], im - last[0]]
            qs[p.z + (a0 + o), pl.ds(g * 8, 8), lanes(c)] = _words(jnp.concatenate(q, 0).astype(bf16))
            last = (re, im)
        if lags < NC:
            pp[z0, c, g, 0] = last[0]
            pp[z0, c, g, 1] = last[1]

    def filter_dft(p, a, c, a0=0):
        taps = _rows(ssm_v[pl.ds(c * 64, 64), pl.ds(pl.multiple_of((a0 + a) * C, C), C)])
        kk = jax.lax.dot_general(_rows(fwd_v[:, 128:256]), taps, (((1,), (1,)), ((), ())),
                                 preferred_element_type=f32).reshape(NG, 2, 8, 128)
        minus, plus = kk[:, 0], kk[:, 1]
        if isinstance(a0, int) and a0 + a == 0:
            skip = dd_v[lanes(c)].astype(f32)[None, None, :]
            minus, plus = minus - skip, plus + skip
        ks[z0 + a0 + a, c, :, slot_of(0)] = plus - minus
        ks[z0 + a0 + a, c, :, slot_of(1)] = minus
        ks[z0 + a0 + a, c, :, slot_of(2)] = plus
        return [kk[i, 1] for i in range(NG)]

    def signal_dft(p, a, c):
        kv = _rows(kvb_v[a // 2 % 2][pl.ds(p.half + a * C // 2, C // 2), lanes(c)])
        uu = jnp.dot(_rows(fwd_v[:, 0:128]), kv, preferred_element_type=f32).reshape(NG, 2, 8, 128)
        us[p.z + (UB + a), c, :, 0] = uu[:, 0] + uu[:, 1]
        us[p.z + (UB + a), c, :, 1] = uu[:, 0]
        us[p.z + (UB + a), c, :, 2] = uu[:, 1]
        return [uu[i, 1] for i in range(NG)]

    def gelu2(h):
        c0 = np.float32(np.sqrt(2 / np.pi))
        c1 = np.float32(np.sqrt(2 / np.pi) * 0.044715)
        return h + h * jnp.tanh(h * (c0 + c1 * (h * h)))

    def mlp_up(p, s, i, r0, n, sync):
        f0 = i * 128
        xn = _rows(xb_v[s % 2][pl.ds(p.half + (s * TM + r0) // 2, n // 2), :])
        nt = (((1,), (1,)), ((), ()))
        if i < NF - 1:
            h = jax.lax.dot_general(xn, _rows(w1_v[pl.ds(f0 // 2, 64), :]), nt, preferred_element_type=f32)
            sync()
            g_v[s % 2, pl.ds(r0 // 2, n // 2), lanes(i)] = _words(gelu2(h + b1_v[lanes(i)].astype(f32)[None, :]).astype(bf16))
            return [h[r:r + 8] for r in range(0, n, 8)]
        h = jax.lax.dot_general(_rows(w1_v[pl.ds(f0 // 2, (F - f0) // 2), :]), xn, nt, preferred_element_type=f32)
        sync()
        g = gelu2(h + jnp.concatenate([b1t_v[...]] * (TM // 128), 1))
        g_v[s % 2, :, pl.ds(f0, F - f0)] = _words(g.T.astype(bf16))
        return [h[r:r + 8, q:q + 128] for q in range(0, TM, 128) for r in range(0, F - f0, 8)]

    def mlp_down(p, s, c, m, sync):
        k0, k1 = KG[m] * 128, min(KG[m + 1] * 128, F)
        o = jnp.dot(_rows(g_v[s % 2, :, k0:k1]), _rows(w2_v[k0 // 2:k1 // 2, lanes(c)]), preferred_element_type=f32)
        sync()
        if m > 0:
            o = o + acc_v[z0]
        if m < NM - 1:
            acc_v[z0] = o
        else:
            ff_v[pl.ds(p.full + s * TM, TM), lanes(c)] = 0.5 * o + b2_v[lanes(c)].astype(f32)[None, :]
        return [o[r:r + 8] for r in range(0, TM, 8)]

    def finish(p, a, c):
        rr, rh = pl.ds(p.full + a * C, C), pl.ds(p.half + a * C // 2, C // 2)
        y = jnp.dot(_rows(inv_v[...]), _rows(qs[p.z + a, :, lanes(c)]), preferred_element_type=f32)
        x, xn = (_rows(ref[rh, lanes(c)]).astype(f32) for ref in (x_v, xb_v[a // 2 % 2]))
        r = xn * y + x + ff_v[rr, lanes(c)]
        o_v[rh, lanes(c)] = _words(r.astype(bf16))
        return []

    up = lambda s: [(mlp_up, s, i % NF, 0, TM) for i in range(-1, NF - 1)]
    down = lambda s: [(mlp_down, s, c, m) for c in range(NL) for m in range(NM)]
    tiles = lambda slot: (5 * slot[4] / TM if slot[2] < NF - 1 else 2.5) if slot[0] is mlp_up else KG[slot[3] + 1] - KG[slot[3]]

    def plan(slots, head, transforms, norms, outputs, spectra, density):
        at = {slot: t for t, slot in enumerate(slots)}
        mxu, side, done = {}, {}, {}
        for lo, hi, chunks, both in transforms:
            items = [(a, c) for c in range(NL) for a in chunks]
            for i, (a, c) in enumerate(items):
                t = int((lo + (hi - lo) * i / len(items)) * NP)
                mxu.setdefault(t, []).extend([(filter_dft, a, c)] * both + [(signal_dft, a, c)])
                done[a, c] = t
                for q in range(KQ):
                    side.setdefault(max(t - AHEAD - (q < KQ // 2), -1), []).append((short_conv, (a, c, q), 200 // KQ))
        for s, t0, span in norms:
            for h in range(TM // 16):
                for stage, cost in enumerate((25, 32, 40)):
                    side.setdefault(t0 + h * span // 16 + 4 * stage, []).append((layernorm, (s, h, stage), cost))
        for s, t0 in outputs:
            for c in range(NL):
                t = at[mlp_down, s, c, NM - 1] if t0 is None else t0 + c
                mxu[t] = [(finish, 2 * s, c), (finish, 2 * s + 1, c)] + mxu.get(t, [])
        queue = [(a0, lags, c, g) for a0, lags, cs in spectra for c in cs for g in range(NG)]
        credit = 0.0
        for t, slot in enumerate(slots):
            more = [it[0] for it in mxu.get(t, [])]
            if slot[0] is mlp_up:
                busy = 340 if slot[2] < NF - 1 else 170
            else:
                busy = 32 * tiles(slot) + 32 * (slot[3] == NM - 1)
            busy += sum(150 if fn is finish else 80 for fn in more) + sum(cost for _, _, cost in side.get(t, []))
            credit += max(0.0, density * 64 * (tiles(slot) + len(more)) - busy)
            due = [it[1:] for u in range(t, t + AHEAD + 1) for it in mxu.get(u, []) if it[0] is finish]
            while queue:
                a0, lags, c, g = queue[0]
                urgent = (a0, c) in due or t == len(slots) - 1
                if done.get((a0 + 1, c), -9) >= t - 1:
                    assert not urgent
                    credit = min(credit, 0.0)
                    break
                if credit <= 0 and not urgent:
                    break
                queue.pop(0)
                n = -(-lags // LAGS)
                cuts = [lags * i // n for i in range(n + 1)]
                side.setdefault(t, []).extend(
                    (products, (a0, lags, c, g, comp, j0, j1), 4 * (j1 - j0) + 12 * (comp == 2 and j1 == lags))
                    for comp in range(3) for j0, j1 in zip(cuts, cuts[1:]))
                credit -= 12 * lags + 6
        return slots, head, mxu, side

    def emit(p, timeline, syncs):
        slots, head, mxu, side = timeline
        for t, slot in enumerate([None] + slots, -1):
            if slot is None:
                groups = [(filter_dft(p, a, c, p.head), 1) for a in head for c in range(NL)]
            else:
                groups = [(slot[0](p, *slot[1:], syncs.get(t, lambda: None)), tiles(slot))]
                groups += [(it[0](p, *it[1:]), 1) for it in mxu.get(t, [])]
            marks = [(v, n / len(vals)) for vals, n in groups for v in vals]
            work = side.get(t, [])
            total, span = sum(cost for _, _, cost in work), sum(d for _, d in marks)
            spent, pos, j = 0.0, 0.0, 0
            for fn, args, cost in work:
                while j < len(marks) - 1 and pos < span * spent / total:
                    pos += marks[j][1]
                    j += 1
                fn(p, *args, marks[j][0])
                spent += cost

    every, lead, rest = range(NL), range(3), range(3, NL)
    lead_in = ([(mlp_up, 0, i, r0, C) for r0 in (0, C) for i in (0, 1)] + [(mlp_up, 1, i, 0, C) for i in (0, 1)]
               + [(mlp_up, 0, i, 0, TM) for i in (2, 3)] + [(mlp_up, 1, i, 0, C) for i in (2, 3)]
               + [(mlp_up, 1, i, C, C) for i in range(4)])
    off = LEAD_IN / NP
    opening = plan(lead_in + [(mlp_up, s, 2 * q + i, 0, TM) for q in range(2, NF // 2) for s in (0, 1) for i in (0, 1)]
                   + down(0) + down(1) + up(2), [],
                   [(1.42 + off, 1.66 + off, (0, 1), True), (1.71 + off, 1.9 + off, (2, 3), True),
                    (1.9 + off, 2.15 + off, (4, 5), True)],
                   [(2, CONV_AT[1] + 1, 4)], [(0, 65 + LEAD_IN), (1, 77 + LEAD_IN)], [(0, 2, every), (2, 4, every), (4, 6, lead)], 2.48)
    middle = plan(down(0) + up(1) + down(1) + up(2), range(5),
                  [(0.03, 0.55, (2, 3), False), (0.85, 1.55, (4, 5), False)],
                  [(1, 0, 10), (2, NP, 10)], [(0, None), (1, None)], [(0, 10, rest), (2, 12, every), (4, 14, lead)], 2.5)
    closing = plan(down(6) + up(7) + down(7), [], [(0.12, 0.6, (14, 15), False)],
                   [(7, 0, 10)], [(6, None), (7, None)], [(12, 14, rest), (14, 16, every)], 2.53)
    for t in CONV_AT:
        opening[3].setdefault(t - 1, []).insert(0, (hold, (), 1))

    for h in range(TM // 16):
        for stage in range(3):
            opening[3].setdefault((1 if h < 8 else 6) + stage, []).append((layernorm, (1, h, stage), 32))
    syncs = {t: (lambda ds=ds: [d.wait() for d in ds]) for t, ds in awaited.items()}
    emit(Pos(0), opening, syncs)
    outs = [store(0, 2), store(2, 4), store(4, 6), store(6, 7), store(7, NB, pl.ds(0, 384)),
            store(7, NB, lanes(3)), store(7, NB, lanes(4))]

    def one_pass(it, carry):
        for i in range(2):
            @pl.when(it == i)
            def _():
                for d in per_pass[i]:
                    d.wait()
                outs[i].start()
        emit(Pos(2 * it + 2), middle, {})
        return carry

    jax.lax.fori_loop(0, 2, one_pass, 0)
    outs[2].start()
    emit(Pos(0), closing, {len(closing[0]) - 2 * NM + 1: lambda: [d.start() for d in outs[3:5]],
                           len(closing[0]) - NM + 1: outs[5].start})
    outs[6].start()
    for d in outs:
        d.wait()


@jax.jit
def pallas_parallel_sum__ssm_conv_h3__dense_activation_gelu__prompt_kernel(
        A_q, A_k, A_v, A_shift_k, A_ssm_k, A_ssm_D, B_x, B_w1, B_b1, B_w2, B_b2):
    del B_x
    vmem = pltpu.VMEM
    seq = vmem((S // 2, D), u32)
    hbm = pl.BlockSpec(memory_space=pl.ANY)
    out = pl.pallas_call(
        _kernel,
        in_specs=[hbm] * 13,
        out_specs=hbm,
        out_shape=jax.ShapeDtypeStruct((S, D), bf16),
        scratch_shapes=[
            seq, vmem((NL, S // 2 + 32, 128), u32), seq,
            vmem((D // 2, S), u32), vmem((F // 2, D), u32), vmem((F // 2, D), u32), seq,
            seq, seq, seq, seq,
            vmem((S, D), f32), vmem((2, TM // 2, NF * 128), u32), vmem((1, TM, 128), f32),
            vmem((UB + NC, NL, NG, 3, 8, 128), f32), vmem((NC, NL, NG, 3, 8, 128), f32),
            vmem((NC, C, D), u32), vmem((1, NL, NG, 2, 8, 128), f32),
            vmem((64, 128), f32), vmem((C, 2 * C), u32), vmem((C // 2, 2 * C), u32), pltpu.SMEM((1,), jnp.int32),
            vmem((4, D), bf16), vmem((D,), bf16), vmem((F,), bf16), vmem((D,), bf16),
            pltpu.SemaphoreType.DMA((64,)),
        ],
        compiler_params=pltpu.CompilerParams(
            vmem_limit_bytes=110 * 1024 * 1024, flags={"XLA_TPU_RESCHEDULE_DMA_DONES": True}),
    )(jnp.asarray(np.zeros((1,), np.int32)), A_q.reshape(S, D), A_k.reshape(S, D), A_v.reshape(S, D), A_shift_k.T,
      A_ssm_k, A_ssm_D, B_w1.T, B_b1, B_w2, B_b2, *_dft_matrices())
    return out.reshape(1, S, D)
```
